```python
import jax
import jax.numpy as jnp

def _softmax(x, axis=-1):
    return jax.nn.softmax(x, axis=axis)

def _gelu(x):
    return jax.nn.gelu(x, approximate=True)

def _silu(x):
    return jax.nn.silu(x)

def _sigmoid(x):
    return jax.nn.sigmoid(x)

def _layernorm(x, axis=-1, eps=1e-05):
    m = jnp.mean(x, axis=axis, keepdims=True)
    v = jnp.var(x, axis=axis, keepdims=True)
    return (x - m) / jnp.sqrt(v + eps)

def _scatter_add(tgt, idx, src, axis=0):
    return tgt.at[idx].add(src)

def _segment_sum(src, seg, n):
    return jax.ops.segment_sum(src, seg, n)

class _Rng:

    def __init__(self, key):
        self._k = key

    def _next(self):
        self._k, sub = jax.random.split(self._k)
        return sub

    def normal(self, shape):
        return jax.random.normal(self._next(), shape, dtype=jnp.bfloat16)

    def randint(self, lo, hi, shape):
        return jax.random.randint(self._next(), shape, lo, hi, dtype=jnp.int32)

    def uniform(self, shape, lo=0.0, hi=1.0):
        return jax.random.uniform(self._next(), shape, jnp.bfloat16, lo, hi)

    def permutation(self, n):
        return jax.random.permutation(self._next(), n)
kernel_name = 'interleave_layers__memory_aug_recurrent_mem_tr__moe_arch_mod__prompt'

def setup_inputs():
    _rng = _Rng(jax.random.key(int.from_bytes(__import__("os").urandom(4), "little")))
    _w = lambda a: (lambda t: t.astype(jnp.bfloat16) if jnp.issubdtype(t.dtype, jnp.floating) else t)(jnp.asarray(a))

    def _A_setup():
        B, S, Dm = (1, 2048, 512)
        H, Dh = (32, 128)
        M, seg = (8, 32)
        seg = min(seg, S)
        S = S // seg * seg
        return {'x': _w((lambda *s: _rng.normal(s) * 0.05)(B, S, Dm)), 'mem0': _w((lambda *s: _rng.normal(s) * 0.05)(B, M, Dm)), 'Wq': _w((lambda *s: _rng.normal(s) * 0.05)(Dm, H, Dh) * Dm ** (-0.5)), 'Wk': _w((lambda *s: _rng.normal(s) * 0.05)(Dm, H, Dh) * Dm ** (-0.5)), 'Wv': _w((lambda *s: _rng.normal(s) * 0.05)(Dm, H, Dh) * Dm ** (-0.5)), 'Wo': _w((lambda *s: _rng.normal(s) * 0.05)(H, Dh, Dm) * (H * Dh) ** (-0.5)), 'seg_len': seg}
    _A_in = _A_setup()

    def _B_setup():
        B, S, D, F, C = (1, 2048, 512, 1792, 1)
        return {'x': _w((lambda *s: _rng.normal(s) * 0.05)(B, S, D)), 'w_r': _w((lambda *s: _rng.normal(s) * 0.05)(D)), 'w_gate': _w((lambda *s: _rng.normal(s) * 0.05)(D, F)), 'w_up': _w((lambda *s: _rng.normal(s) * 0.05)(D, F)), 'w_down': _w((lambda *s: _rng.normal(s) * 0.05)(F, D))}
    _B_in = _B_setup()
    return {'A_x': _A_in['x'], 'A_mem0': _A_in['mem0'], 'A_Wq': _A_in['Wq'], 'A_Wk': _A_in['Wk'], 'A_Wv': _A_in['Wv'], 'A_Wo': _A_in['Wo'], 'A_seg_len': _A_in['seg_len'], 'B_x': _B_in['x'], 'B_w_r': _B_in['w_r'], 'B_w_gate': _B_in['w_gate'], 'B_w_up': _B_in['w_up'], 'B_w_down': _B_in['w_down']}

def reference(A_x, A_mem0, A_Wq, A_Wk, A_Wv, A_Wo, A_seg_len, B_x, B_w_r, B_w_gate, B_w_up, B_w_down):

    def _A_ref(x, mem0, Wq, Wk, Wv, Wo, seg_len):
        B, S, Dm = x.shape
        H, Dh = (Wq.shape[1], Wq.shape[2])
        M = mem0.shape[1]
        scale = Dh ** (-0.5)
        n_seg = S // seg_len
        L = M + seg_len
        idx = jnp.arange(L)
        mask = (idx[:, None] < M) | (idx[:, None] >= idx[None, :])
        mem = mem0
        outs = []
        for s in range(n_seg):
            xs = x[:, s * seg_len:(s + 1) * seg_len, :].copy()
            h = jnp.concatenate([mem, xs], axis=1)
            q = jnp.einsum('btd,dhe->bhte', h, Wq)
            k = jnp.einsum('btd,dhe->bhte', h, Wk)
            v = jnp.einsum('btd,dhe->bhte', h, Wv)
            scores = jnp.einsum('bhqe,bhke->bhqk', q, k) * scale
            scores = jnp.where(mask[None, None], scores, -1000000000.0)
            p = _softmax(scores, axis=-1)
            o = jnp.einsum('bhqk,bhke->bhqe', p, v)
            o = jnp.einsum('bhte,hed->btd', o, Wo)
            mem = o[:, :M, :].copy()
            outs.append(o[:, M:, :])
        return jnp.concatenate(outs, axis=1)

    def _B_ref(x, w_r, w_gate, w_up, w_down):
        B, S, D = x.shape
        C = 1
        r = x @ w_r
        idx = jnp.argsort(-r, axis=-1)[:, :C]
        idx_e = jnp.repeat(idx.reshape(B, C, 1), D, axis=2)
        x_sel = jnp.take_along_axis(x, idx_e, axis=1)
        g = _silu(x_sel @ w_gate)
        u = x_sel @ w_up
        y = g * u @ w_down
        r_sel = _sigmoid(jnp.take_along_axis(r, idx, axis=1))
        y = y * r_sel.reshape(B, C, 1)
        b_off = (jnp.arange(B) * S).reshape(B, 1)
        flat_idx = (idx + b_off).reshape(B * C)
        zero = (x * 0.0).reshape(B * S, D)
        upd = _scatter_add(zero, flat_idx, y.reshape(B * C, D), axis=0)
        return x + upd.reshape(B, S, D)
    x = A_x
    x = x + _A_ref(_layernorm(x, axis=-1), A_mem0, A_Wq, A_Wk, A_Wv, A_Wo, A_seg_len)
    x = x + _B_ref(_layernorm(x, axis=-1), B_w_r, B_w_gate, B_w_up, B_w_down)
    x = x + _A_ref(_layernorm(x, axis=-1), A_mem0, A_Wq, A_Wk, A_Wv, A_Wo, A_seg_len)
    x = x + _B_ref(_layernorm(x, axis=-1), B_w_r, B_w_gate, B_w_up, B_w_down)
    return x
```

```python
import functools

import jax
import jax.numpy as jnp
from jax import lax
import jax.experimental.pallas as pl
import jax.experimental.pallas.tpu as pltpu

F32 = jnp.float32
BF16 = jnp.bfloat16
LANES = 128
GROUP = 4
EPS_BF16 = 1.0013580322265625e-05


def _rnd(x):
    return x.astype(BF16).astype(F32)


def _layernorm(x):
    inv_d = 1.0 / x.shape[-1]
    m = jnp.sum(x, axis=-1, keepdims=True) * inv_d
    c = x - m
    v = jnp.sum(c * c, axis=-1, keepdims=True) * inv_d
    sd = _rnd(jnp.sqrt(_rnd(_rnd(v) + EPS_BF16)))
    return _rnd(_rnd(x - _rnd(m)) / sd)


def _dot(a, b):
    return jnp.dot(a, b, preferred_element_type=F32)


def _kernel(x_hbm, mem0_ref, wq_hbm, wk_hbm, wv_hbm, wo_hbm, wr_ref, wg_hbm, wu_hbm, wd_hbm,
            out_hbm,
            raw_ref, wqkv_ref, wo_ref, wg_ref, wu_ref, wd_ref, xr_ref, xm_ref, n_ref, a_ref, sems,
            *, seg, n_heads, unroll, n_chunks):
    S, D = xr_ref.shape
    M = mem0_ref.shape[0]
    Dh = LANES
    n_seg = S // seg
    L = M + seg
    G = n_heads // GROUP
    GW = GROUP * Dh
    scale = Dh ** -0.5

    rows = D * n_heads // n_chunks
    w_hbm = (wq_hbm, wk_hbm, wv_hbm)

    def w_copy(i, c):
        return pltpu.make_async_copy(w_hbm[i].at[pl.ds(c * rows, rows)],
                                     raw_ref.at[i, pl.ds(c * rows, rows)],
                                     sems.at[5 + i * n_chunks + c])

    x_copy = pltpu.make_async_copy(x_hbm, xr_ref, sems.at[0])
    wo_copy = pltpu.make_async_copy(wo_hbm, wo_ref, sems.at[1])
    ffn_copies = [pltpu.make_async_copy(src, dst, sems.at[2 + i])
                  for i, (src, dst) in enumerate(((wg_hbm, wg_ref), (wu_hbm, wu_ref), (wd_hbm, wd_ref)))]
    x_copy.start()
    for i in range(3):
        for c in range(n_chunks):
            w_copy(i, c).start()
    wo_copy.start()

    x_copy.wait()

    def ln_body(i, carry):
        r0 = pl.multiple_of(i * 64, 64)
        n_ref[pl.ds(r0, 64), :] = _layernorm(xr_ref[pl.ds(r0, 64), :].astype(F32))
        return carry

    lax.fori_loop(0, S // 64, ln_body, 0)

    raw32 = raw_ref.bitcast(jnp.uint32)
    hp = n_heads // 2
    d_chunk = D // n_chunks
    for i in range(3):
        for c in range(n_chunks):
            w_copy(i, c).wait()

            def relayout(b, carry, i=i, c=c):
                d0 = pl.multiple_of(c * d_chunk + b * 16, 16)
                blk = raw32.at[i, pl.ds(pl.multiple_of(d0 * hp, 16 * hp), 16 * hp)]
                for j in range(hp):
                    even = blk[pl.ds(j, 8, stride=2 * hp), :]
                    odd = blk[pl.ds(hp + j, 8, stride=2 * hp), :]
                    lo = (even & jnp.uint32(0xFFFF)) | (odd << 16)
                    hi = (even >> 16) | (odd & jnp.uint32(0xFFFF0000))
                    wqkv_ref[i, pl.ds(d0, 16), pl.ds(2 * j * Dh, Dh)] = pltpu.bitcast(lo, BF16)
                    wqkv_ref[i, pl.ds(d0, 16), pl.ds((2 * j + 1) * Dh, Dh)] = pltpu.bitcast(hi, BF16)
                return carry

            lax.fori_loop(0, d_chunk // 16, relayout, 0)
    wo_copy.wait()
    for cp in ffn_copies:
        cp.start()

    def attend(s, mem):
        tok = n_ref[pl.ds(pl.multiple_of(s * seg, seg), seg), :]
        h = jnp.concatenate([tok, mem], axis=0)
        qi = lax.broadcasted_iota(jnp.int32, (L, L), 0)
        ki = lax.broadcasted_iota(jnp.int32, (L, L), 1)
        visible = (qi >= seg) | (ki >= seg) | (qi >= ki)
        q, k, v, e, inv, o = {}, {}, {}, {}, {}, {}
        acc = [None] * (D // LANES)

        def proj(i, g):
            return _dot(h, wqkv_ref[i, :, g * GW:(g + 1) * GW])

        def scores(g):
            for j in range(GROUP):
                c = slice(j * Dh, (j + 1) * Dh)
                sc = lax.dot_general(q[g][:, c], k[g][:, c], (((1,), (1,)), ((), ())),
                                     preferred_element_type=F32)
                sc = jnp.where(visible, sc * scale, -1e9)
                p = jnp.exp(sc - jnp.max(sc, axis=-1, keepdims=True))
                e[g, j] = p
                inv[g, j] = pl.reciprocal(jnp.sum(p, axis=-1, keepdims=True), approx=True)

        def values(g):
            og = jnp.concatenate([_dot(e[g, j], v[g][:, j * Dh:(j + 1) * Dh]) * inv[g, j]
                                  for j in range(GROUP)], axis=1)
            o[g] = jnp.concatenate([og[seg:], og[:seg]], axis=0)

        def out(n, groups):
            for g in groups:
                t = _dot(o[g], wo_ref[g * GW:(g + 1) * GW, n * LANES:(n + 1) * LANES])
                acc[n] = t if acc[n] is None else acc[n] + t

        for g in range(G):
            k[g] = proj(1, g).astype(BF16)
            q[g] = proj(0, g)
            v[g] = proj(2, g).astype(BF16)
            scores(g)
            if g:
                values(g - 1)
        out(0, range(0, G - 2))
        values(G - 1)
        out(1, range(0, G - 2))
        out(0, range(G - 2, G))
        out(1, range(G - 2, G))
        for n in range(2, D // LANES):
            out(n, range(G))
        res = _rnd(jnp.concatenate(acc, axis=1))
        return res[M:], res[:M]

    def router(n):
        return _rnd(jnp.sum(n * wr_ref[...].astype(F32), axis=-1, keepdims=True))

    def finish(s, a, best):
        rs = pl.ds(pl.multiple_of(s * seg, seg), seg)
        x1 = _rnd(xr_ref[rs, :].astype(F32) + a)
        n1 = _layernorm(x1)
        x2 = _rnd(x1 + n1)
        xm_ref[rs, :] = x1.astype(BF16)
        xr_ref[rs, :] = x2.astype(BF16)
        n_ref[rs, :] = _layernorm(x2)
        r = jnp.broadcast_to(router(n1), (seg, LANES))
        best_r, best_i = best
        sub = lax.broadcasted_iota(jnp.int32, (8, LANES), 0)
        for b in range(seg // 8):
            rb = r[b * 8:(b + 1) * 8]
            better = rb > best_r
            best_r = jnp.where(better, rb, best_r)
            best_i = jnp.where(better, sub + (s * seg + b * 8), best_i)
        return best_r, best_i

    def layer(l, carry):
        def steps(it, c):
            mem, best = c
            for u in range(unroll):
                s = it * unroll + u
                a, mem = attend(s, mem)
                best = finish(s, a, best)
            return mem, best

        best0 = (jnp.full((8, LANES), -jnp.inf, F32), lax.broadcasted_iota(jnp.int32, (8, LANES), 0))
        _, (best_r, best_i) = lax.fori_loop(0, n_seg // unroll, steps, (mem0_ref[...].astype(F32), best0))

        @pl.when(l == 0)
        def _():
            for cp in ffn_copies:
                cp.wait()

        top = jnp.max(best_r, axis=0, keepdims=True)
        idx = jnp.min(jnp.where(best_r == top, best_i, S - 1))
        base = pl.multiple_of(jnp.clip(idx // 16 * 16, 0, S - 16), 16)
        rs = pl.ds(base, 16)
        x1 = xm_ref[rs, :].astype(F32)
        n1 = _layernorm(x1)
        nb = n1.astype(BF16)
        gate = _rnd(_dot(nb, wg_ref[...]))
        gate = _rnd(gate * jax.nn.sigmoid(gate))
        up = _rnd(_dot(nb, wu_ref[...]))
        y = _rnd(_dot((gate * up).astype(BF16), wd_ref[...]))
        y = _rnd(y * _rnd(jax.nn.sigmoid(router(n1))))
        chosen = lax.broadcasted_iota(jnp.int32, (16, D), 0) == idx - base
        x2 = _rnd(x1 + _rnd(n1 + jnp.where(chosen, y, 0.0)))
        xr_ref[rs, :] = x2.astype(BF16)
        n_ref[rs, :] = _layernorm(x2)
        return carry

    lax.fori_loop(0, 2, layer, 0)
    out_copy = pltpu.make_async_copy(xr_ref, out_hbm, sems.at[0])
    out_copy.start()
    out_copy.wait()


@functools.partial(jax.jit, static_argnames=("A_seg_len",))
def pallas_interleave_layers__memory_aug_recurrent_mem_tr__moe_arch_mod__prompt_kernel(
    A_x, A_mem0, A_Wq, A_Wk, A_Wv, A_Wo, A_seg_len, B_x, B_w_r, B_w_gate, B_w_up, B_w_down,
):
    del B_x
    B, S, D = A_x.shape
    _, H, Dh = A_Wq.shape
    M = A_mem0.shape[1]
    F = B_w_gate.shape[1]
    seg = int(A_seg_len)
    assert B == 1 and Dh == LANES and S % seg == 0 and seg % 16 == 0 and M % 8 == 0
    n_chunks = 4
    hbm = pl.BlockSpec(memory_space=pl.ANY)
    vmem = pl.BlockSpec(memory_space=pltpu.VMEM)
    out = pl.pallas_call(
        functools.partial(_kernel, seg=seg, n_heads=H, unroll=1, n_chunks=n_chunks),
        out_shape=jax.ShapeDtypeStruct((S, D), A_x.dtype),
        in_specs=[hbm, vmem, hbm, hbm, hbm, hbm, vmem, hbm, hbm, hbm],
        out_specs=hbm,
        scratch_shapes=[
            pltpu.VMEM((3, D * H, Dh), BF16),
            pltpu.VMEM((3, D, H * Dh), BF16),
            pltpu.VMEM((H * Dh, D), BF16),
            pltpu.VMEM((D, F), BF16),
            pltpu.VMEM((D, F), BF16),
            pltpu.VMEM((F, D), BF16),
            pltpu.VMEM((S, D), BF16),
            pltpu.VMEM((S, D), BF16),
            pltpu.VMEM((S, D), F32),
            pltpu.VMEM((seg, D), F32),
            pltpu.SemaphoreType.DMA((5 + 3 * n_chunks,)),
        ],
        compiler_params=pltpu.CompilerParams(vmem_limit_bytes=100 * 1024 * 1024),
        name="rmt_mod",
    )(A_x.reshape(S, D), A_mem0.reshape(M, D), A_Wq.reshape(D * H, Dh), A_Wk.reshape(D * H, Dh),
      A_Wv.reshape(D * H, Dh), A_Wo.reshape(H * Dh, D), B_w_r.reshape(1, D), B_w_gate, B_w_up, B_w_down)
    return out.reshape(B, S, D)
```

```python
import functools

import jax
import jax.numpy as jnp
from jax import lax
import jax.experimental.pallas as pl
import jax.experimental.pallas.tpu as pltpu

F32 = jnp.float32
BF16 = jnp.bfloat16
LANES = 128
GROUP = 4
EPS_BF16 = 1.0013580322265625e-05


def _rnd(x):
    return x.astype(BF16).astype(F32)


def _layernorm(x):
    inv_d = 1.0 / x.shape[-1]
    m = jnp.sum(x, axis=-1, keepdims=True) * inv_d
    c = x - m
    v = jnp.sum(c * c, axis=-1, keepdims=True) * inv_d
    sd = _rnd(jnp.sqrt(_rnd(_rnd(v) + EPS_BF16)))
    return _rnd(_rnd(x - _rnd(m)) / sd)


def _dot(a, b):
    return jnp.dot(a, b, preferred_element_type=F32)


def _kernel(x_hbm, mem0_ref, wq_hbm, wk_hbm, wv_hbm, wo_hbm, wr_ref, wg_hbm, wu_hbm, wd_hbm,
            out_hbm,
            raw_ref, wqkv_ref, wo_ref, wg_ref, wu_ref, wd_ref, xr_ref, xm_ref, n_ref, a_ref, sems,
            *, seg, n_heads, unroll, n_chunks):
    S, D = x_hbm.shape
    M = mem0_ref.shape[0]
    Dh = LANES
    n_seg = S // seg
    L = M + seg
    G = n_heads // GROUP
    GW = GROUP * Dh
    scale = Dh ** -0.5

    rows = D * n_heads // n_chunks
    w_hbm = (wq_hbm, wk_hbm, wv_hbm)

    def w_copy(i, c):
        return pltpu.make_async_copy(w_hbm[i].at[pl.ds(c * rows, rows)],
                                     raw_ref.at[i, pl.ds(c * rows, rows)],
                                     sems.at[5 + i * n_chunks + c])

    x_copy = pltpu.make_async_copy(x_hbm, xr_ref.at[pl.ds(0, S)], sems.at[0])
    wo_copy = pltpu.make_async_copy(wo_hbm, wo_ref.bitcast(BF16), sems.at[1])
    ffn_copies = [pltpu.make_async_copy(src, dst, sems.at[2 + i])
                  for i, (src, dst) in enumerate(((wg_hbm, wg_ref), (wu_hbm, wu_ref), (wd_hbm, wd_ref)))]
    x_copy.start()
    for i in range(3):
        for c in range(n_chunks):
            w_copy(i, c).start()
    wo_copy.start()

    x_copy.wait()

    def ln_body(i, carry):
        r0 = pl.multiple_of(i * 64, 64)
        n_ref[pl.ds(r0, 64), :] = _layernorm(xr_ref[pl.ds(r0, 64), :].astype(F32))
        return carry

    lax.fori_loop(0, S // 64, ln_body, 0)

    raw32 = raw_ref.bitcast(jnp.uint32)
    hp = n_heads // 2
    d_chunk = D // n_chunks
    for i in range(3):
        for c in range(n_chunks):
            w_copy(i, c).wait()

            def relayout(b, carry, i=i, c=c):
                d0 = pl.multiple_of(c * d_chunk + b * 16, 16)
                dst = pl.ds(pl.multiple_of(d0 // 2, 8), 8)
                blk = raw32.at[i, pl.ds(pl.multiple_of(d0 * hp, 16 * hp), 16 * hp)]
                for j in range(hp):
                    even = blk[pl.ds(j, 8, stride=2 * hp), :]
                    odd = blk[pl.ds(hp + j, 8, stride=2 * hp), :]
                    lo = (even & jnp.uint32(0xFFFF)) | (odd << 16)
                    hi = (even >> 16) | (odd & jnp.uint32(0xFFFF0000))
                    wqkv_ref[i, dst, pl.ds(2 * j * Dh, Dh)] = lo
                    wqkv_ref[i, dst, pl.ds((2 * j + 1) * Dh, Dh)] = hi
                return carry

            lax.fori_loop(0, d_chunk // 16, relayout, 0)
    wo_copy.wait()
    for cp in ffn_copies:
        cp.start()

    def attend(tok, mem):
        h = jnp.concatenate([tok, mem], axis=0)
        qi = lax.broadcasted_iota(jnp.int32, (L, L), 0)
        ki = lax.broadcasted_iota(jnp.int32, (L, L), 1)
        visible = (qi >= seg) | (ki >= seg) | (qi >= ki)
        q, k, v, e, inv, o = {}, {}, {}, {}, {}, {}
        acc = [None] * (D // LANES)

        def proj(i, g):
            return _dot(h, pltpu.bitcast(wqkv_ref[i, :, g * GW:(g + 1) * GW], BF16))

        def scores(g):
            for j in range(GROUP):
                c = slice(j * Dh, (j + 1) * Dh)
                sc = lax.dot_general(q[g][:, c], k[g][:, c], (((1,), (1,)), ((), ())),
                                     preferred_element_type=F32)
                sc = jnp.where(visible, sc * scale, -1e9)
                p = jnp.exp(sc - jnp.max(sc, axis=-1, keepdims=True))
                e[g, j] = p
                inv[g, j] = pl.reciprocal(jnp.sum(p, axis=-1, keepdims=True), approx=True)

        def values(g):
            og = jnp.concatenate([_dot(e[g, j], v[g][:, j * Dh:(j + 1) * Dh]) * inv[g, j]
                                  for j in range(GROUP)], axis=1)
            o[g] = jnp.concatenate([og[seg:], og[:seg]], axis=0)

        def out(n, groups):
            for g in groups:
                w = wo_ref[g * GW // 2:(g + 1) * GW // 2, n * LANES:(n + 1) * LANES]
                t = _dot(o[g], pltpu.bitcast(w, BF16))
                acc[n] = t if acc[n] is None else acc[n] + t

        for g in range(G):
            k[g] = proj(1, g).astype(BF16)
            q[g] = proj(0, g)
            v[g] = proj(2, g).astype(BF16)
            scores(g)
            if g:
                values(g - 1)
        out(0, range(0, G - 2))
        values(G - 1)
        out(1, range(0, G - 2))
        out(0, range(G - 2, G))
        out(1, range(G - 2, G))
        for n in range(2, D // LANES):
            out(n, range(G))
        res = _rnd(jnp.concatenate(acc, axis=1))
        return res[M:], res[:M]

    def router(n):
        return _rnd(jnp.sum(n * wr_ref[...].astype(F32), axis=-1, keepdims=True))

    def finish(s, a, best):
        src = pl.ds(pl.multiple_of(jnp.maximum(s, 0) * seg, seg), seg)
        rs = pl.ds(pl.multiple_of(jnp.where(s < 0, n_seg, s) * seg, seg), seg)
        x1 = _rnd(xr_ref[src, :].astype(F32) + a)
        n1 = _layernorm(x1)
        x2 = _rnd(x1 + n1)
        xm_ref[rs, :] = x1.astype(BF16)
        xr_ref[rs, :] = x2.astype(BF16)
        n_ref[rs, :] = _layernorm(x2)
        r = jnp.where(s < 0, -jnp.inf, jnp.broadcast_to(router(n1), (seg, LANES)))
        best_r, best_i = best
        sub = lax.broadcasted_iota(jnp.int32, (8, LANES), 0)
        for b in range(seg // 8):
            rb = r[b * 8:(b + 1) * 8]
            better = rb > best_r
            best_r = jnp.where(better, rb, best_r)
            best_i = jnp.where(better, sub + (s * seg + b * 8), best_i)
        return best_r, best_i

    def layer(l, carry):
        def steps(it, c):
            mem, best = c
            for u in range(unroll):
                s = it * unroll + u
                tok = n_ref[pl.ds(pl.multiple_of(s * seg, seg), seg), :]
                best = finish(s - 1, a_ref[...], best)
                a_ref[...], mem = attend(tok, mem)
            return mem, best

        best0 = (jnp.full((8, LANES), -jnp.inf, F32), lax.broadcasted_iota(jnp.int32, (8, LANES), 0))
        _, best = lax.fori_loop(0, n_seg // unroll, steps, (mem0_ref[...].astype(F32), best0))
        best_r, best_i = finish(n_seg - 1, a_ref[...], best)

        @pl.when(l == 0)
        def _():
            for cp in ffn_copies:
                cp.wait()

        top = jnp.max(best_r, axis=0, keepdims=True)
        idx = jnp.min(jnp.where(best_r == top, best_i, S - 1))
        base = pl.multiple_of(jnp.clip(idx // 16 * 16, 0, S - 16), 16)
        rs = pl.ds(base, 16)
        x1 = xm_ref[rs, :].astype(F32)
        n1 = _layernorm(x1)
        nb = n1.astype(BF16)
        gate = _rnd(_dot(nb, wg_ref[...]))
        gate = _rnd(gate * jax.nn.sigmoid(gate))
        up = _rnd(_dot(nb, wu_ref[...]))
        y = _rnd(_dot((gate * up).astype(BF16), wd_ref[...]))
        y = _rnd(y * _rnd(jax.nn.sigmoid(router(n1))))
        chosen = lax.broadcasted_iota(jnp.int32, (16, D), 0) == idx - base
        x2 = _rnd(x1 + _rnd(n1 + jnp.where(chosen, y, 0.0)))
        xr_ref[rs, :] = x2.astype(BF16)
        n_ref[rs, :] = _layernorm(x2)
        return carry

    a_ref[...] = jnp.zeros_like(a_ref)
    lax.fori_loop(0, 2, layer, 0)
    out_copy = pltpu.make_async_copy(xr_ref.at[pl.ds(0, S)], out_hbm, sems.at[0])
    out_copy.start()
    out_copy.wait()


@functools.partial(jax.jit, static_argnames=("A_seg_len",))
def pallas_interleave_layers__memory_aug_recurrent_mem_tr__moe_arch_mod__prompt_kernel(
    A_x, A_mem0, A_Wq, A_Wk, A_Wv, A_Wo, A_seg_len, B_x, B_w_r, B_w_gate, B_w_up, B_w_down,
):
    del B_x
    B, S, D = A_x.shape
    _, H, Dh = A_Wq.shape
    M = A_mem0.shape[1]
    F = B_w_gate.shape[1]
    seg = int(A_seg_len)
    assert B == 1 and Dh == LANES and S % seg == 0 and seg % 16 == 0 and M % 8 == 0
    n_chunks = 4
    hbm = pl.BlockSpec(memory_space=pl.ANY)
    vmem = pl.BlockSpec(memory_space=pltpu.VMEM)
    out = pl.pallas_call(
        functools.partial(_kernel, seg=seg, n_heads=H, unroll=1, n_chunks=n_chunks),
        out_shape=jax.ShapeDtypeStruct((S, D), A_x.dtype),
        in_specs=[hbm, vmem, hbm, hbm, hbm, hbm, vmem, hbm, hbm, hbm],
        out_specs=hbm,
        scratch_shapes=[
            pltpu.VMEM((3, D * H, Dh), BF16),
            pltpu.VMEM((3, D // 2, H * Dh), jnp.uint32),
            pltpu.VMEM((H * Dh // 2, D), jnp.uint32),
            pltpu.VMEM((D, F), BF16),
            pltpu.VMEM((D, F), BF16),
            pltpu.VMEM((F, D), BF16),
            pltpu.VMEM((S + seg, D), BF16),
            pltpu.VMEM((S + seg, D), BF16),
            pltpu.VMEM((S + seg, D), F32),
            pltpu.VMEM((seg, D), F32),
            pltpu.SemaphoreType.DMA((5 + 3 * n_chunks,)),
        ],
        compiler_params=pltpu.CompilerParams(vmem_limit_bytes=100 * 1024 * 1024),
        name="rmt_mod",
    )(A_x.reshape(S, D), A_mem0.reshape(M, D), A_Wq.reshape(D * H, Dh), A_Wk.reshape(D * H, Dh),
      A_Wv.reshape(D * H, Dh), A_Wo.reshape(H * Dh, D), B_w_r.reshape(1, D), B_w_gate, B_w_up, B_w_down)
    return out.reshape(B, S, D)
```

```python
import functools

import jax
import jax.numpy as jnp
from jax import lax
import jax.experimental.pallas as pl
import jax.experimental.pallas.tpu as pltpu

F32 = jnp.float32
BF16 = jnp.bfloat16
U32 = jnp.uint32
LANES = 128
UW = 2 * LANES
EPS_BF16 = 1.0013580322265625e-05
Q, K, V = 0, 1, 2


def _rnd(x):
    return x.astype(BF16).astype(F32)


def _layernorm(x):
    inv_d = 1.0 / x.shape[-1]
    m = jnp.sum(x, axis=-1, keepdims=True) * inv_d
    c = x - m
    v = jnp.sum(c * c, axis=-1, keepdims=True) * inv_d
    sd = _rnd(jnp.sqrt(_rnd(_rnd(v) + EPS_BF16)))
    return _rnd(_rnd(x - _rnd(m)) / sd)


def _dot(a, b):
    return jnp.dot(a, b, preferred_element_type=F32)


def _rows(*xs):
    return xs[0] if len(xs) == 1 else jnp.concatenate(xs, axis=0)


def _cols(*xs):
    return jnp.concatenate(xs, axis=1)


def _right(b11, b12, b21, b22):
    return {1: b11 + b22, 2: b11, 3: b12 - b22, 4: b21 - b11, 5: b22, 6: b11 + b12, 7: b21 + b22}


def _left(i, a11, a12, a21, a22):
    return {1: lambda: a11 + a22, 2: lambda: a21 + a22, 3: lambda: a11, 4: lambda: a22,
            5: lambda: a11 + a12, 6: lambda: a21 - a11, 7: lambda: a12 - a22}[i]()


SET_A, SET_B, SET_C = (1, 3, 5, 7), (1, 2, 4, 6), (2, 3, 4, 5)
HALVES = {SET_A: {1: "x", 3: "x", 5: "x", 7: "xy"},
          SET_B: {1: "y", 2: "x", 4: "x", 6: "xy"},
          SET_C: {2: "y", 3: "y", 4: "y", 5: "y"}}


def _direct_left(ops, a1, a2):
    both = a1 + a2
    return {1: a1 if ops == SET_A else a2, 2: both, 3: a1, 4: a2, 5: both, 6: a1, 7: a2}


def _direct_out(ops, p):
    c1 = p[1] - p[5] + p[7] if ops == SET_A else p[2] + p[4]
    c2 = p[1] - p[2] + p[6] if ops == SET_B else p[3] + p[5]
    return c1, c2


def _kernel(x_hbm, mem0_ref, wq_hbm, wk_hbm, wv_hbm, wo_hbm, wr_ref, wg_hbm, wu_hbm, wd_hbm,
            out_hbm,
            raw_ref, rawo_ref, win_ref, wout_ref, wg_ref, wu_ref, wd_ref,
            xr_ref, xm_ref, n_ref, px_ref, py_ref, left_ref, o_ref, onext_ref, a_ref, sems,
            *, seg, n_heads, n_chunks):
    S, D = x_hbm.shape
    M = mem0_ref.shape[0]
    Dh = LANES
    n_seg = S // seg
    L = M + seg
    G = n_heads // 4
    HD = D // 2
    P = 3 * seg
    R = P // 4
    n_per = (n_seg - 1) // 3
    scale = Dh ** -0.5

    rows = HD * n_heads // n_chunks
    w_hbm = (wq_hbm, wk_hbm, wv_hbm)

    def w_copy(i, c, half):
        r = pl.ds((half * n_chunks + c) * rows, rows)
        return pltpu.make_async_copy(w_hbm[i].at[r], raw_ref.at[i, r],
                                     sems.at[5 + (i * n_chunks + c) * 2 + half])

    x_copy = pltpu.make_async_copy(x_hbm, xr_ref.at[pl.ds(0, S)], sems.at[0])
    wo_copy = pltpu.make_async_copy(wo_hbm, rawo_ref, sems.at[1])
    ffn_copies = [pltpu.make_async_copy(src, dst, sems.at[2 + i])
                  for i, (src, dst) in enumerate(((wg_hbm, wg_ref), (wu_hbm, wu_ref), (wd_hbm, wd_ref)))]
    x_copy.start()
    for i in range(3):
        for c in range(n_chunks):
            w_copy(i, c, 0).start()
            w_copy(i, c, 1).start()
    wo_copy.start()

    a_ref[...] = jnp.zeros_like(a_ref)
    x_copy.wait()

    def ln_body(i, carry):
        r0 = pl.multiple_of(i * 64, 64)
        n_ref[pl.ds(r0, 64), :] = _layernorm(xr_ref[pl.ds(r0, 64), :].astype(F32))
        return carry

    lax.fori_loop(0, S // 64, ln_body, 0)

    def pack(x):
        return pltpu.bitcast(x.astype(BF16), U32)

    raw32 = raw_ref.bitcast(U32)
    hp = n_heads // 2
    d_chunk = HD // n_chunks
    for i in range(3):
        for c in range(n_chunks):
            w_copy(i, c, 0).wait()
            w_copy(i, c, 1).wait()

            def prep_in(b, carry, i=i, c=c):
                d0 = c * d_chunk + b * 16
                dst = pl.ds(pl.multiple_of(d0 // 2, 8), 8)
                src = [raw32.at[i, pl.ds(pl.multiple_of((d0 + half * HD) * hp, 16 * hp), 16 * hp)]
                       for half in range(2)]
                for j in range(hp):
                    w1, w2 = (s[pl.ds(j, 16, stride=hp), :] for s in src)
                    blocks = [pltpu.bitcast(w, F32) for w in
                              (w1 << 16, w1 & U32(0xFFFF0000), w2 << 16, w2 & U32(0xFFFF0000))]
                    for op, w in _right(*blocks).items():
                        win_ref[op - 1, i, dst, pl.ds(j * Dh, Dh)] = pack(w)
                return carry

            lax.fori_loop(0, d_chunk // 16, prep_in, 0)

    def prep_out(j, carry):
        even = rawo_ref[pl.ds(pl.multiple_of(2 * j * Dh, Dh), Dh), :].astype(F32)
        odd = rawo_ref[pl.ds(pl.multiple_of((2 * j + 1) * Dh, Dh), Dh), :].astype(F32)
        dst = pl.ds(pl.multiple_of(j * (Dh // 2), Dh // 2), Dh // 2)
        for op, w in _right(even[:, :HD], even[:, HD:], odd[:, :HD], odd[:, HD:]).items():
            wout_ref[op - 1, dst, :] = pack(w)
        return carry

    def token_left(ops, t0):
        def block(r):
            t = n_ref[pl.ds(pl.multiple_of(t0 + r * R, 8), R), :]
            return t[:, :HD], t[:, HD:]

        used = "".join(HALVES[ops].values())
        blocks = {h: block(r) + block(r + 1) for h, r in (("x", 0), ("y", 2)) if h in used}
        return {i: [_left(i, *blocks[h]) for h in HALVES[ops][i]] for i in ops}

    def split(ops, i, prod, n_direct):
        parts = {h: prod[t * R:(t + 1) * R] for t, h in enumerate(HALVES[ops][i])}
        if n_direct:
            parts["d"] = prod[-n_direct:]
        return parts

    def in_tokens(ops, mat, g, m):
        c = slice(g * UW, (g + 1) * UW)
        if ops == SET_A:
            own = left_ref[0, mat, :, c], left_ref[1, mat, :, c]
            px_ref[0, mat, :, c] = m[1]["x"] - m[5]["x"] + m[7]["x"]
            px_ref[1, mat, :, c] = m[3]["x"] + m[5]["x"]
            px_ref[2, mat, :, c] = m[1]["x"] + m[3]["x"]
            px_ref[3, mat, :, c] = m[7]["y"]
            return own
        if ops == SET_B:
            even = _rows(px_ref[0, mat, :, c] + m[4]["x"], m[2]["x"] + m[4]["x"])
            odd = _rows(px_ref[1, mat, :, c], px_ref[2, mat, :, c] - m[2]["x"] + m[6]["x"])
            py_ref[0, mat, :, c] = px_ref[3, mat, :, c] + m[1]["y"]
            py_ref[1, mat, :, c] = m[1]["y"] + m[6]["y"]
            left_ref[0, mat, :2 * R - seg, c] = even[seg:]
            left_ref[1, mat, :2 * R - seg, c] = odd[seg:]
            return even[:seg], odd[:seg]
        even = _rows(left_ref[0, mat, :2 * R - seg, c],
                     py_ref[0, mat, :, c] + m[4]["y"] - m[5]["y"], m[2]["y"] + m[4]["y"])
        odd = _rows(left_ref[1, mat, :2 * R - seg, c],
                    m[3]["y"] + m[5]["y"], py_ref[1, mat, :, c] - m[2]["y"] + m[3]["y"])
        left_ref[0, mat, :, c] = even[seg:]
        left_ref[1, mat, :, c] = odd[seg:]
        return even[:seg], odd[:seg]

    def w_in(i, mat, r, c):
        return pltpu.bitcast(win_ref[i - 1, mat, r, c], BF16)

    def attend(ops, t0, direct, o_dst, o_row, tail):
        nd = direct.shape[0]
        dl = _direct_left(ops, direct[:, :HD], direct[:, HD:])
        tl = {i: [] for i in ops} if t0 is None else token_left(ops, t0)
        lhs = {i: _rows(*tl[i], dl[i]) for i in ops}
        qi = lax.broadcasted_iota(jnp.int32, (L, L), 0)
        ki = lax.broadcasted_iota(jnp.int32, (L, L), 1)
        visible = (qi >= seg) | (ki >= seg) | (qi >= ki)
        qkv, e, inv, o_mem = {}, {}, {}, {}

        early = {i: _dot(lhs[i][:, :LANES], w_in(i, K, slice(0, LANES // 2), slice(0, 2 * UW))) for i in ops}
        early = {i: early[i] + _dot(lhs[i][:, LANES:], w_in(i, K, slice(LANES // 2, LANES), slice(0, 2 * UW)))
                 for i in ops}

        def project(mat, g):
            c = slice(g * UW, (g + 1) * UW)
            if mat == K and g < 2:
                prod = {i: early[i][:, c] for i in ops}
            else:
                prod = {i: _dot(lhs[i], w_in(i, mat, slice(None), c)) for i in ops}
            halves = _direct_out(ops, {i: prod[i][-nd:] for i in ops})
            if t0 is not None:
                own = in_tokens(ops, mat, g, {i: split(ops, i, prod[i], 0) for i in ops})
                halves = [_rows(t, d) for t, d in zip(own, halves)]
            for p, x in enumerate(halves):
                x = x if mat == Q else x.astype(BF16)
                for j in range(2):
                    qkv[mat, g, p, j] = x[:, j * Dh:(j + 1) * Dh]

        heads = [(p, j) for p in range(2) for j in range(2)]

        def scores(g):
            for p, j in heads:
                sc = lax.dot_general(qkv[Q, g, p, j], qkv[K, g, p, j], (((1,), (1,)), ((), ())),
                                     preferred_element_type=F32)
                sc = jnp.where(visible, sc * scale, -1e9)
                w = jnp.exp(sc - jnp.max(sc, axis=-1, keepdims=True))
                e[g, p, j] = w
                inv[g, p, j] = pl.reciprocal(jnp.sum(w, axis=-1, keepdims=True), approx=True)

        def values(g):
            for p, j in heads:
                o = _dot(e[g, p, j], qkv[V, g, p, j]) * inv[g, p, j]
                o_dst[p, o_row:o_row + seg, (2 * g + j) * Dh:(2 * g + j + 1) * Dh] = o[:seg]
                o_mem[p, 2 * g + j] = o[seg:]

        project(K, 0)
        project(K, 1)
        for g in range(G):
            if g > 1:
                project(K, g)
            project(Q, g)
            project(V, g)
            scores(g)
            if g:
                values(g - 1)
        return tail(o_mem, lambda: values(G - 1))

    def project_out(ops, with_tokens, direct, midway=None):
        n_k = hp // 4
        lhs, acc = {}, {}

        def run(n, kk):
            c = slice(kk * 4 * Dh, (kk + 1) * 4 * Dh)
            if kk not in lhs:
                dl = _direct_left(ops, *direct(kk))
                block = lambda r: (o_ref[0, r * R:(r + 1) * R, c], o_ref[1, r * R:(r + 1) * R, c])
                used = "".join(HALVES[ops].values()) if with_tokens else ""
                blocks = {h: block(r) + block(r + 1) for h, r in (("y", 0), ("x", 2)) if h in used}
                lhs[kk] = {i: _rows(dl[i], *[_left(i, *blocks[h]) for h in HALVES[ops][i] if h in used])
                           for i in ops}
            for i in ops:
                w = wout_ref[i - 1, kk * 2 * Dh:(kk + 1) * 2 * Dh, n * LANES:(n + 1) * LANES]
                t = _dot(lhs[kk][i], pltpu.bitcast(w, BF16))
                acc[i, n] = acc[i, n] + t if kk else t

        for n in range(HD // LANES):
            for kk in range(n_k):
                if midway is not None and n == 0 and kk == n_k - 2:
                    midway()
                run(n, kk)
        prod = {i: _cols(*[acc[i, n] for n in range(HD // LANES)]) for i in ops}
        nd = direct(0)[0].shape[0]
        res = _rnd(_cols(*_direct_out(ops, {i: prod[i][:nd] for i in ops})))
        return res, {i: split(ops, i, prod[i][nd:], 0) for i in ops} if with_tokens else None

    def mem_rows(o_mem):
        return lambda kk: tuple(_cols(*[o_mem[p, 4 * kk + t] for t in range(4)]) for p in range(2))

    def router(n):
        return _rnd(jnp.sum(n * wr_ref[...].astype(F32), axis=-1, keepdims=True))

    def finish(s, a, best):
        src = pl.ds(pl.multiple_of(jnp.maximum(s, 0) * seg, seg), seg)
        rs = pl.ds(pl.multiple_of(jnp.where(s < 0, n_seg, s) * seg, seg), seg)
        x1 = _rnd(xr_ref[src, :].astype(F32) + a)
        n1 = _layernorm(x1)
        x2 = _rnd(x1 + n1)
        xm_ref[rs, :] = x1.astype(BF16)
        xr_ref[rs, :] = x2.astype(BF16)
        n_ref[rs, :] = _layernorm(x2)
        r = jnp.where(s < 0, -jnp.inf, jnp.broadcast_to(router(n1), (seg, LANES)))
        best_r, best_i = best
        sub = lax.broadcasted_iota(jnp.int32, (8, LANES), 0)
        for b in range(seg // 8):
            rb = r[b * 8:(b + 1) * 8]
            better = rb > best_r
            best_r = jnp.where(better, rb, best_r)
            best_i = jnp.where(better, sub + (s * seg + b * 8), best_i)
        return best_r, best_i

    def period(it, carry):
        mem, best = carry
        t0 = seg + it * P
        t1 = jnp.where(it == n_per - 1, seg, t0 + P)
        o_ref[:, :seg, :] = onext_ref[...]
        m = {}
        for u, (ops_in, t, ops_out, dst, row) in enumerate(((SET_B, t0, SET_C, o_ref, seg),
                                                           (SET_C, t0, SET_B, o_ref, 2 * seg),
                                                           (SET_A, t1, SET_A, onext_ref, 0))):
            def tail(o_mem, last_values, u=u, ops_out=ops_out):
                new_best = finish(3 * (it - 1) + u, a_ref[u * seg:(u + 1) * seg, :], best)
                return project_out(ops_out, True, mem_rows(o_mem), last_values), new_best

            (mem, prods), best = attend(ops_in, t, mem, dst, row, tail)
            for i in ops_out:
                for h, x in prods[i].items():
                    m[i, h] = x
        for t, h in enumerate("yx"):
            top = _cols(m[1, h] + m[4, h] - m[5, h] + m[7, h], m[3, h] + m[5, h])
            bottom = _cols(m[2, h] + m[4, h], m[1, h] - m[2, h] + m[3, h] + m[6, h])
            a_ref[2 * t * R:2 * (t + 1) * R, :] = _rnd(_rows(top, bottom))
        return mem, best

    def layer(l, stale):
        @pl.when(stale > 0)
        def _():
            tl = token_left(SET_A, seg)
            lhs = {i: _rows(*tl[i]) for i in SET_A}
            for g in range(G):
                c = slice(g * UW, (g + 1) * UW)
                for mat in (Q, K, V):
                    in_tokens(SET_A, mat, g, {i: split(SET_A, i, _dot(lhs[i], w_in(i, mat, slice(None), c)), 0)
                                              for i in SET_A})

        def first_tail(o_mem, last_values):
            last_values()

            @pl.when(l == 0)
            def _():
                wo_copy.wait()
                for cp in ffn_copies:
                    cp.start()
                lax.fori_loop(0, hp, prep_out, 0)

            return project_out(SET_C, False, mem_rows(o_mem))[0]

        mem = attend(SET_C, None, _rows(n_ref[:seg, :], mem0_ref[...].astype(F32)), onext_ref, 0, first_tail)
        best = (jnp.full((8, LANES), -jnp.inf, F32), lax.broadcasted_iota(jnp.int32, (8, LANES), 0))
        _, best = lax.fori_loop(0, n_per, period, (mem, best))

        @pl.when(l == 0)
        def _():
            for cp in ffn_copies:
                cp.wait()

        last, _ = project_out(SET_C, False, lambda kk: tuple(
            onext_ref[p, :, kk * 4 * Dh:(kk + 1) * 4 * Dh] for p in range(2)))
        for u in range(3):
            best = finish(n_seg - 4 + u, a_ref[u * seg:(u + 1) * seg, :], best)
        best_r, best_i = finish(n_seg - 1, last, best)

        top = jnp.max(best_r, axis=0, keepdims=True)
        idx = jnp.min(jnp.where(best_r == top, best_i, S - 1))
        base = pl.multiple_of(jnp.clip(idx // 16 * 16, 0, S - 16), 16)
        rs = pl.ds(base, 16)
        x1 = xm_ref[rs, :].astype(F32)
        n1 = _layernorm(x1)
        nb = n1.astype(BF16)
        gate = _rnd(_dot(nb, wg_ref[...]))
        gate = _rnd(gate * jax.nn.sigmoid(gate))
        up = _rnd(_dot(nb, wu_ref[...]))
        y = _rnd(_dot((gate * up).astype(BF16), wd_ref[...]))
        y = _rnd(y * _rnd(jax.nn.sigmoid(router(n1))))
        chosen = lax.broadcasted_iota(jnp.int32, (16, D), 0) == idx - base
        x2 = _rnd(x1 + _rnd(n1 + jnp.where(chosen, y, 0.0)))
        xr_ref[rs, :] = x2.astype(BF16)
        n_ref[rs, :] = _layernorm(x2)
        return ((idx >= seg) & (idx < seg + P)).astype(jnp.int32)

    lax.fori_loop(0, 2, layer, jnp.int32(1))
    out_copy = pltpu.make_async_copy(xr_ref.at[pl.ds(0, S)], out_hbm, sems.at[0])
    out_copy.start()
    out_copy.wait()


@functools.partial(jax.jit, static_argnames=("A_seg_len",))
def pallas_interleave_layers__memory_aug_recurrent_mem_tr__moe_arch_mod__prompt_kernel(
    A_x, A_mem0, A_Wq, A_Wk, A_Wv, A_Wo, A_seg_len, B_x, B_w_r, B_w_gate, B_w_up, B_w_down,
):
    del B_x
    B, S, D = A_x.shape
    _, H, Dh = A_Wq.shape
    M = A_mem0.shape[1]
    F = B_w_gate.shape[1]
    seg = int(A_seg_len)
    assert B == 1 and Dh == LANES and D == 4 * LANES and H % 8 == 0 and M % 8 == 0
    assert seg % 32 == 0 and S % seg == 0 and (S // seg) % 3 == 1 and S // seg > 7
    n_chunks = 2
    half = H * Dh // 2
    R = 3 * seg // 4
    hbm = pl.BlockSpec(memory_space=pl.ANY)
    vmem = pl.BlockSpec(memory_space=pltpu.VMEM)
    out = pl.pallas_call(
        functools.partial(_kernel, seg=seg, n_heads=H, n_chunks=n_chunks),
        out_shape=jax.ShapeDtypeStruct((S, D), A_x.dtype),
        in_specs=[hbm, vmem, hbm, hbm, hbm, hbm, vmem, hbm, hbm, hbm],
        out_specs=hbm,
        scratch_shapes=[
            pltpu.VMEM((3, D * H, Dh), BF16),
            pltpu.VMEM((H * Dh, D), BF16),
            pltpu.VMEM((7, 3, D // 4, half), U32),
            pltpu.VMEM((7, half // 2, D // 2), U32),
            pltpu.VMEM((D, F), BF16),
            pltpu.VMEM((D, F), BF16),
            pltpu.VMEM((F, D), BF16),
            pltpu.VMEM((S + seg, D), BF16),
            pltpu.VMEM((S + seg, D), BF16),
            pltpu.VMEM((S + seg, D), F32),
            pltpu.VMEM((4, 3, R, half), F32),
            pltpu.VMEM((2, 3, R, half), F32),
            pltpu.VMEM((2, 3, seg, half), F32),
            pltpu.VMEM((2, 3 * seg, half), F32),
            pltpu.VMEM((2, seg, half), F32),
            pltpu.VMEM((3 * seg, D), F32),
            pltpu.SemaphoreType.DMA((5 + 6 * n_chunks,)),
        ],
        compiler_params=pltpu.CompilerParams(vmem_limit_bytes=110 * 1024 * 1024),
        name="rmt_mod",
    )(A_x.reshape(S, D), A_mem0.reshape(M, D), A_Wq.reshape(D * H, Dh), A_Wk.reshape(D * H, Dh),
      A_Wv.reshape(D * H, Dh), A_Wo.reshape(H * Dh, D), B_w_r.reshape(1, D), B_w_gate, B_w_up, B_w_down)
    return out.reshape(B, S, D)
```

```python
import functools

import jax
import jax.numpy as jnp
from jax import lax
import jax.experimental.pallas as pl
import jax.experimental.pallas.tpu as pltpu

F32 = jnp.float32
BF16 = jnp.bfloat16
U32 = jnp.uint32
LANES = 128
DEPTH = 2
UW = 2 * LANES
EPS_BF16 = 1.0013580322265625e-05
K, Q, V, O = 0, 1, 2, 3


def _rnd(x):
    return x.astype(BF16).astype(F32)


def _layernorm(x):
    inv_d = 1.0 / x.shape[-1]
    m = jnp.sum(x, axis=-1, keepdims=True) * inv_d
    c = x - m
    v = jnp.sum(c * c, axis=-1, keepdims=True) * inv_d
    sd = _rnd(jnp.sqrt(_rnd(_rnd(v) + EPS_BF16)))
    return _rnd(_rnd(x - _rnd(m)) / sd)


def _dot(a, b):
    return jnp.dot(a, b, preferred_element_type=F32)


def _rows(*xs):
    return xs[0] if len(xs) == 1 else jnp.concatenate(xs, axis=0)


def _cols(*xs):
    return jnp.concatenate(xs, axis=1)


def _right(b11, b12, b21, b22):
    return {1: b11 + b22, 2: b11, 3: b12 - b22, 4: b21 - b11, 5: b22, 6: b11 + b12, 7: b21 + b22}


def _left(i, a11, a12, a21, a22):
    return {1: lambda: a11 + a22, 2: lambda: a21 + a22, 3: lambda: a11, 4: lambda: a22,
            5: lambda: a11 + a12, 6: lambda: a21 - a11, 7: lambda: a12 - a22}[i]()


SET_A, SET_B, SET_C = (1, 3, 5, 7), (1, 2, 4, 6), (2, 3, 4, 5)
HALVES = {SET_A: {1: "x", 3: "x", 5: "x", 7: "xy"},
          SET_B: {1: "y", 2: "x", 4: "x", 6: "xy"},
          SET_C: {2: "y", 3: "y", 4: "y", 5: "y"}}


def _direct_left(ops, a1, a2):
    both = a1 + a2
    return {1: a1 if ops == SET_A else a2, 2: both, 3: a1, 4: a2, 5: both, 6: a1, 7: a2}


def _direct_out(ops, p):
    c1 = p[1] - p[5] + p[7] if ops == SET_A else p[2] + p[4]
    c2 = p[1] - p[2] + p[6] if ops == SET_B else p[3] + p[5]
    return c1, c2


def _kernel(x_hbm, mem0_hbm, wq_hbm, wk_hbm, wv_hbm, wo_hbm, wr_hbm, wg_hbm, wu_hbm, wd_hbm,
            out_hbm,
            raw_ref, rawo_ref, wk_ref, wq_ref, wv_ref, wo_ref, wg_ref, wu_ref, wd_ref,
            xr_ref, xm_ref, n_ref, ly_ref, px_ref, py_ref, left_ref, o_ref, onext_ref, a_ref,
            patch_ref, mem0_ref, wr1_ref, wr_ref, sems,
            *, seg, n_heads, n_chunks):
    S, D = x_hbm.shape
    M = mem0_ref.shape[0]
    Dh = LANES
    n_seg = S // seg
    L = M + seg
    G = n_heads // 4
    HD = D // 2
    P = 3 * seg
    R = P // 4
    n_per = (n_seg - 1) // 3
    scale = Dh ** -0.5

    hp = n_heads // 2

    w_hbm = {Q: wq_hbm, K: wk_hbm, V: wv_hbm}
    w_ref = {Q: wq_ref, K: wk_ref, V: wv_ref, O: wo_ref}
    op_rows = G * HD // 2

    def ahead_rows(k, g, r):
        return pl.ds(pl.multiple_of(7 * op_rows + (k * G + g) * n_per * R + r, 8), R)

    d_chunk = HD // n_chunks
    o_chunk = hp // n_chunks

    def w_copies(mat, c):
        sem = 6 + 2 * (mat * n_chunks + c)
        if mat > V:
            r = pl.ds(c * o_chunk * UW, o_chunk * UW)
            return [pltpu.make_async_copy(wo_hbm.at[r], rawo_ref.at[r], sems.at[sem])]
        r = pl.ds(c * d_chunk * n_heads, d_chunk * n_heads)
        return [pltpu.make_async_copy(w_hbm[mat].at[half, r], raw_ref.at[mat, half, r], sems.at[sem + half])
                for half in range(2)]

    x_copy = pltpu.make_async_copy(x_hbm, xr_ref.at[pl.ds(0, S)], sems.at[0])
    ffn_copies = [pltpu.make_async_copy(src, dst, sems.at[1 + i])
                  for i, (src, dst) in enumerate(((wg_hbm, wg_ref), (wu_hbm, wu_ref), (wd_hbm, wd_ref)))]
    small_copies = [pltpu.make_async_copy(mem0_hbm, mem0_ref, sems.at[4]),
                    pltpu.make_async_copy(wr_hbm, wr1_ref, sems.at[5])]
    x_copy.start()
    for cp in small_copies:
        cp.start()
    for mat in range(DEPTH):
        for c in range(n_chunks):
            for cp in w_copies(mat, c):
                cp.start()

    a_ref[...] = jnp.zeros_like(a_ref)
    x_copy.wait()
    for cp in small_copies:
        cp.wait()
    wr_ref[...] = jnp.broadcast_to(wr1_ref[...].astype(F32).reshape(1, D), wr_ref.shape)
    n_ref[:seg, :] = _layernorm(xr_ref[:seg, :].astype(F32))

    def ln_body(jj, carry):
        for j in [jj * 3 + u for u in range(3)]:
            rs = pl.ds(pl.multiple_of(seg + j * P, seg), P)
            n = _layernorm(xr_ref[rs, :].astype(F32))
            n_ref[rs, :] = n
            y = (n[2 * R:3 * R, :HD], n[2 * R:3 * R, HD:], n[3 * R:, :HD], n[3 * R:, HD:])
            for t, i in enumerate((6, 7)):
                ly_ref[t, pl.ds(pl.multiple_of(j * R, 8), R), :] = _left(i, *y)
        return carry

    lax.fori_loop(0, n_per // 3, ln_body, 0)

    def pack(x):
        return pltpu.bitcast(x.astype(BF16), U32)

    raw32 = raw_ref.bitcast(U32)

    def prep_in(mat, c, t):
        b, j = divmod(t, hp)
        d0 = c * d_chunk + b * 16
        dst = j // 2 * (HD // 2) + c * (d_chunk // 2) + b * 8
        w1, w2 = (raw32.at[mat, half, pl.ds(pl.multiple_of(d0 * hp, 16 * hp), 16 * hp)][pl.ds(j, 16, stride=hp), :]
                  for half in range(2))
        blocks = [pltpu.bitcast(w, F32) for w in (w1 << 16, w1 & U32(0xFFFF0000), w2 << 16, w2 & U32(0xFFFF0000))]
        for op, w in _right(*blocks).items():
            w_ref[mat][pl.ds(pl.multiple_of((op - 1) * op_rows + dst, 8), 8), pl.ds(j % 2 * Dh, Dh)] = pack(w)

    def prep_out(c, t):
        j, r = divmod(t * 16, Dh)
        even, odd = (rawo_ref[pl.ds(pl.multiple_of((c * o_chunk + j) * UW + p * Dh + r, 16), 16), :].astype(F32)
                     for p in range(2))
        dst = c * (o_chunk * Dh // 2) + t * 8
        for op, w in _right(even[:, :HD], even[:, HD:], odd[:, :HD], odd[:, HD:]).items():
            wo_ref[pl.ds(pl.multiple_of((op - 1) * op_rows + dst, 8), 8), :] = pack(w)

    def w_in(i, mat, g, r=0, rows=HD // 2):
        r = (i - 1) * op_rows + g * (HD // 2) + r
        return pltpu.bitcast(w_ref[mat][pl.ds(r if isinstance(r, int) else pl.multiple_of(r, 8), rows), :], BF16)

    for mat in (K, Q, V, O):
        def stream(c, carry, mat=mat):
            for cp in w_copies(mat, c):
                cp.wait()
            prep, n_prep = ((functools.partial(prep_in, mat), d_chunk // 16 * hp) if mat < O
                            else (prep_out, o_chunk * Dh // 16))
            n_dot = G // n_chunks * 2
            for t in range(n_dot):
                g, k = c * (G // n_chunks) + t // 2, t % 2
                if mat > K:
                    prod = pltpu.bitcast(_dot(ly_ref[k], w_in(6 + k, mat - 1, g)), U32)
                for j in range(n_per):
                    for i in range((t * n_per + j) * n_prep // (n_dot * n_per),
                                   (t * n_per + j + 1) * n_prep // (n_dot * n_per)):
                        prep(c, i)
                    if mat > K:
                        w_ref[mat][ahead_rows(k, g, j * R), :] = prod[j * R:(j + 1) * R]
            if mat + DEPTH <= O:
                for cp in w_copies(mat + DEPTH, c):
                    cp.start()
            return carry

        lax.fori_loop(0, n_chunks, stream, 0)
    for cp in ffn_copies:
        cp.start()

    def token_left(halves, t0):
        def block(r):
            t = n_ref[pl.ds(pl.multiple_of(t0 + r * R, 8), R), :]
            return t[:, :HD], t[:, HD:]

        used = "".join(halves.values())
        blocks = {h: block(r) + block(r + 1) for h, r in (("x", 0), ("y", 2)) if h in used}
        return {i: [_left(i, *blocks[h]) for h in hs] for i, hs in halves.items()}

    def split(hs, prod):
        return {h: prod[t * R:(t + 1) * R] for t, h in enumerate(hs)}

    def in_tokens(ops, mat, g, m, it):
        if ops == SET_A:
            if "x" in m[7]:
                px_ref[0, mat, g] = m[1]["x"] - m[5]["x"] + m[7]["x"]
                px_ref[1, mat, g] = m[3]["x"] + m[5]["x"]
                px_ref[2, mat, g] = m[1]["x"] + m[3]["x"]
            if "y" in m[7]:
                px_ref[3, mat, g] = m[7]["y"]
            return None if it is None else (left_ref[0, mat, g], left_ref[1, mat, g])
        if ops == SET_B:
            even = _rows(px_ref[0, mat, g] + m[4]["x"], m[2]["x"] + m[4]["x"])
            odd = _rows(px_ref[1, mat, g], px_ref[2, mat, g] - m[2]["x"] + m[6]["x"])
            if "y" in m[6]:
                m6, m7 = m[6]["y"], px_ref[3, mat, g]
            else:
                m6, m7 = (pltpu.bitcast(w_ref[mat + 1][ahead_rows(k, g, it * R), :], F32) for k in range(2))
            py_ref[0, mat, g] = m7 + m[1]["y"]
            py_ref[1, mat, g] = m[1]["y"] + m6
            left_ref[0, mat, g, :2 * R - seg] = even[seg:]
            left_ref[1, mat, g, :2 * R - seg] = odd[seg:]
            return even[:seg], odd[:seg]
        even = _rows(left_ref[0, mat, g, :2 * R - seg],
                     py_ref[0, mat, g] + m[4]["y"] - m[5]["y"], m[2]["y"] + m[4]["y"])
        odd = _rows(left_ref[1, mat, g, :2 * R - seg],
                    m[3]["y"] + m[5]["y"], py_ref[1, mat, g] - m[2]["y"] + m[3]["y"])
        left_ref[0, mat, g] = even[seg:]
        left_ref[1, mat, g] = odd[seg:]
        return even[:seg], odd[:seg]

    def attend(ops, halves, t0, it, direct, o_dst, o_row, tail):
        nd = direct.shape[0]
        dl = _direct_left(ops, direct[:, :HD], direct[:, HD:])
        tl = token_left(halves, t0)
        lhs = {i: _rows(*tl[i], dl[i]) for i in ops}
        qi = lax.broadcasted_iota(jnp.int32, (L, L), 0)
        ki = lax.broadcasted_iota(jnp.int32, (L, L), 1)
        visible = (qi >= seg) | (ki >= seg) | (qi >= ki)
        qkv, e, inv, o_mem = {}, {}, {}, {}

        def first_units(i, t):
            w = _cols(*[w_in(i, K, g, t * LANES // 2, LANES // 2) for g in range(2)])
            return _dot(lhs[i][:, t * LANES:(t + 1) * LANES], w)

        early = {i: first_units(i, 0) for i in ops}
        early = {i: first_units(i, 1) + early[i] for i in ops}

        def project(mat, g):
            if mat == K and g < 2:
                prod = {i: early[i][:, g * UW:(g + 1) * UW] for i in ops}
            else:
                prod = {i: _dot(lhs[i], w_in(i, mat, g)) for i in ops}
            pair = _direct_out(ops, {i: prod[i][-nd:] for i in ops})
            own = in_tokens(ops, mat, g, {i: split(halves[i], prod[i]) for i in ops}, it)
            if own is not None:
                pair = [_rows(t, d) for t, d in zip(own, pair)]
            for p, x in enumerate(pair):
                x = x if mat == Q else x.astype(BF16)
                for j in range(2):
                    qkv[mat, g, p, j] = x[:, j * Dh:(j + 1) * Dh]

        heads = [(p, j) for p in range(2) for j in range(2)]

        def scores(g):
            for p, j in heads:
                sc = lax.dot_general(qkv[Q, g, p, j], qkv[K, g, p, j], (((1,), (1,)), ((), ())),
                                     preferred_element_type=F32)
                sc = jnp.where(visible, sc * scale, -1e9)
                w = jnp.exp(sc - jnp.max(sc, axis=-1, keepdims=True))
                e[g, p, j] = w
                inv[g, p, j] = pl.reciprocal(jnp.sum(w, axis=-1, keepdims=True), approx=True)

        def values(g):
            for p, j in heads:
                o = _dot(e[g, p, j], qkv[V, g, p, j]) * inv[g, p, j]
                o_dst[p, o_row:o_row + seg, (2 * g + j) * Dh:(2 * g + j + 1) * Dh] = o[:seg]
                o_mem[p, 2 * g + j] = o[seg:]

        project(K, 0)
        project(K, 1)
        for g in range(G):
            if g > 1:
                project(K, g)
            project(Q, g)
            project(V, g)
            scores(g)
            if g:
                values(g - 1)
        return tail(o_mem, lambda: values(G - 1))

    def project_out(ops, with_tokens, direct, midway=None):
        n_k = hp // 4
        lhs, acc = {}, {}

        def run(n, kk):
            c = slice(kk * 4 * Dh, (kk + 1) * 4 * Dh)
            if kk not in lhs:
                dl = _direct_left(ops, *direct(kk))
                block = lambda r: (o_ref[0, r * R:(r + 1) * R, c], o_ref[1, r * R:(r + 1) * R, c])
                used = "".join(HALVES[ops].values()) if with_tokens else ""
                blocks = {h: block(r) + block(r + 1) for h, r in (("y", 0), ("x", 2)) if h in used}
                lhs[kk] = {i: _rows(dl[i], *[_left(i, *blocks[h]) for h in HALVES[ops][i] if h in used])
                           for i in ops}
            for i in ops:
                w = wo_ref[pl.ds((i - 1) * op_rows + kk * 2 * Dh, 2 * Dh), n * LANES:(n + 1) * LANES]
                t = _dot(lhs[kk][i], pltpu.bitcast(w, BF16))
                acc[i, n] = t + acc[i, n] if kk else t

        for n in range(HD // LANES):
            for kk in range(n_k):
                if midway is not None and n == 0 and kk == n_k - 2:
                    midway()
                run(n, kk)
        prod = {i: _cols(*[acc[i, n] for n in range(HD // LANES)]) for i in ops}
        nd = direct(0)[0].shape[0]
        res = [_direct_out(ops, {i: acc[i, n][:nd] for i in ops}) for n in range(HD // LANES)]
        res = _cols(*[r[p] for p in range(2) for r in res])
        return res, {i: split(HALVES[ops][i], prod[i][nd:]) for i in ops} if with_tokens else None

    def mem_rows(o_mem):
        return lambda kk: tuple(_cols(*[o_mem[p, 4 * kk + t] for t in range(4)]) for p in range(2))

    def router(n):
        return _rnd(jnp.sum(n * _rows(*[wr_ref[...]] * (n.shape[0] // 8)), axis=-1, keepdims=True))

    def finish(s, a, best, more=True):
        src = pl.ds(pl.multiple_of(jnp.maximum(s, 0) * seg, seg), seg)
        rs = pl.ds(pl.multiple_of(jnp.where(s < 0, n_seg, s) * seg, seg), seg)
        x1 = _rnd(xr_ref[src, :].astype(F32) + a)
        n1 = _layernorm(x1)
        x2 = _rnd(x1 + n1)
        xm_ref[rs, :] = x1.astype(BF16)
        xr_ref[rs, :] = x2.astype(BF16)
        if more:
            n_ref[rs, :] = _layernorm(x2)
        r = jnp.where(s < 0, -jnp.inf, jnp.broadcast_to(router(n1), (seg, LANES)))
        best_r, best_i = best
        sub = lax.broadcasted_iota(jnp.int32, (8, LANES), 0)
        for b in range(seg // 8):
            rb = r[b * 8:(b + 1) * 8]
            better = rb > best_r
            best_r = jnp.where(better, rb, best_r)
            best_i = jnp.where(better, sub + (s * seg + b * 8), best_i)
        return best_r, best_i

    def riders(l, ops):
        return {i: hs[0] if l == 0 else hs for i, hs in HALVES[ops].items()}

    n_early = (n_seg - 7) * seg
    early_copy = pltpu.make_async_copy(xr_ref.at[pl.ds(0, n_early)], out_hbm.at[pl.ds(0, n_early)], sems.at[0])
    late_copy = pltpu.make_async_copy(xr_ref.at[pl.ds(n_early, S - n_early)],
                                      out_hbm.at[pl.ds(n_early, S - n_early)], sems.at[1])

    def period(l, it, carry):
        mem, best = carry
        if l == 1:
            pl.when(it == n_per - 1)(early_copy.start)
        t0 = seg + it * P
        t1 = jnp.where(it == n_per - 1, seg, t0 + P)
        o_ref[:, :seg, :] = onext_ref[...]
        m = {}
        for u, (ops_in, t, ops_out, dst, row) in enumerate(((SET_B, t0, SET_C, o_ref, seg),
                                                           (SET_C, t0, SET_B, o_ref, 2 * seg),
                                                           (SET_A, t1, SET_A, onext_ref, 0))):
            def tail(o_mem, last_values, u=u, ops_out=ops_out):
                new_best = finish(3 * (it - 1) + u, a_ref[u * seg:(u + 1) * seg, :], best, l == 0)
                return project_out(ops_out, True, mem_rows(o_mem), last_values), new_best

            (mem, prods), best = attend(ops_in, riders(l, ops_in), t, it, mem, dst, row, tail)
            for i in ops_out:
                for h, x in prods[i].items():
                    m[i, h] = x
        for t, h in enumerate("yx"):
            top = _cols(m[1, h] + m[4, h] - m[5, h] + m[7, h], m[3, h] + m[5, h])
            bottom = _cols(m[2, h] + m[4, h], m[1, h] - m[2, h] + m[3, h] + m[6, h])
            a_ref[2 * t * R:2 * (t + 1) * R, :] = _rnd(_rows(top, bottom))
        return mem, best

    def layer(l, routed):
        @pl.when((routed >= seg) & (routed < seg + P))
        def _():
            def unit(g, carry):
                tl = token_left(riders(0, SET_A), seg)
                for mat in (K, Q, V):
                    in_tokens(SET_A, mat, g, {i: {"x": _dot(tl[i][0], w_in(i, mat, g))} for i in SET_A}, None)
                return carry

            lax.fori_loop(0, G, unit, 0)

        mem = attend(SET_A, {i: hs[1:] for i, hs in HALVES[SET_A].items()}, seg, None,
                     _rows(n_ref[:seg, :], mem0_ref[...].astype(F32)), onext_ref, 0,
                     lambda o_mem, last_values: project_out(SET_C, False, mem_rows(o_mem), last_values)[0])
        best = (jnp.full((8, LANES), -jnp.inf, F32), lax.broadcasted_iota(jnp.int32, (8, LANES), 0))
        carry = lax.fori_loop(0, (1 - l) * n_per, functools.partial(period, 0), (mem, best))
        _, best = lax.fori_loop(0, l * n_per, functools.partial(period, 1), carry)

        @pl.when(l == 0)
        def _():
            for cp in ffn_copies:
                cp.wait()

        last, _ = project_out(SET_C, False, lambda kk: tuple(
            onext_ref[p, :, kk * 4 * Dh:(kk + 1) * 4 * Dh] for p in range(2)))
        for u in range(3):
            best = finish(n_seg - 4 + u, a_ref[u * seg:(u + 1) * seg, :], best)
        best_r, best_i = finish(n_seg - 1, _rnd(last), best)
        pl.when(l == 1)(late_copy.start)

        top = jnp.max(best_r, axis=0, keepdims=True)
        idx = jnp.min(jnp.where(best_r == top, best_i, S - 1))
        base = pl.multiple_of(jnp.clip(idx // 16 * 16, 0, S - 16), 16)
        rs = pl.ds(base, 16)
        x1 = xm_ref[rs, :].astype(F32)
        n1 = _layernorm(x1)
        nb = n1.astype(BF16)
        gate = _rnd(_dot(nb, wg_ref[...]))
        gate = _rnd(gate * jax.nn.sigmoid(gate))
        up = _rnd(_dot(nb, wu_ref[...]))
        y = _rnd(_dot((gate * up).astype(BF16), wd_ref[...]))
        y = _rnd(y * _rnd(jax.nn.sigmoid(router(n1))))
        chosen = lax.broadcasted_iota(jnp.int32, (16, D), 0) == idx - base
        x2 = _rnd(x1 + _rnd(n1 + jnp.where(chosen, y, 0.0)))
        patch_ref[...] = x2.astype(BF16)

        @pl.when(l == 0)
        def _():
            xr_ref[rs, :] = x2.astype(BF16)
            n_ref[rs, :] = _layernorm(x2)

        return idx

    routed = lax.fori_loop(0, 2, layer, jnp.int32(seg))
    early_copy.wait()
    late_copy.wait()
    base = pl.multiple_of(jnp.clip(routed // 16 * 16, 0, S - 16), 16)
    patch_copy = pltpu.make_async_copy(patch_ref, out_hbm.at[pl.ds(base, 16)], sems.at[0])
    patch_copy.start()
    patch_copy.wait()


@functools.partial(jax.jit, static_argnames=("A_seg_len",))
def pallas_interleave_layers__memory_aug_recurrent_mem_tr__moe_arch_mod__prompt_kernel(
    A_x, A_mem0, A_Wq, A_Wk, A_Wv, A_Wo, A_seg_len, B_x, B_w_r, B_w_gate, B_w_up, B_w_down,
):
    del B_x
    B, S, D = A_x.shape
    _, H, Dh = A_Wq.shape
    M = A_mem0.shape[1]
    F = B_w_gate.shape[1]
    seg = int(A_seg_len)
    assert B == 1 and Dh == LANES and D == 4 * LANES and H % 8 == 0 and M % 8 == 0
    assert seg % 32 == 0 and S % seg == 0 and (S // seg) % 9 == 1 and S // seg > 7
    n_chunks = 4
    half = H * Dh // 2
    R = 3 * seg // 4
    hbm = pl.BlockSpec(memory_space=pl.ANY)
    out = pl.pallas_call(
        functools.partial(_kernel, seg=seg, n_heads=H, n_chunks=n_chunks),
        out_shape=jax.ShapeDtypeStruct((S, D), A_x.dtype),
        in_specs=[hbm] * 10,
        out_specs=hbm,
        scratch_shapes=[
            pltpu.VMEM((3, 2, D * H // 2, Dh), BF16),
            pltpu.VMEM((H * Dh, D), BF16),
            pltpu.VMEM((7 * half // 2, UW), U32),
            *[pltpu.VMEM((7 * half // 2 + H // 2 * (S - seg) // 4, UW), U32)] * 3,
            pltpu.VMEM((D, F), BF16),
            pltpu.VMEM((D, F), BF16),
            pltpu.VMEM((F, D), BF16),
            pltpu.VMEM((S + seg, D), BF16),
            pltpu.VMEM((S + seg, D), BF16),
            pltpu.VMEM((S + seg, D), F32),
            pltpu.VMEM((2, (S - seg) // 4, D // 2), F32),
            pltpu.VMEM((4, 3, H // 4, R, UW), F32),
            pltpu.VMEM((2, 3, H // 4, R, UW), F32),
            pltpu.VMEM((2, 3, H // 4, seg, UW), F32),
            pltpu.VMEM((2, 3 * seg, half), F32),
            pltpu.VMEM((2, seg, half), F32),
            pltpu.VMEM((3 * seg, D), F32),
            pltpu.VMEM((16, D), BF16),
            pltpu.VMEM((M, D), BF16),
            pltpu.VMEM((D,), BF16),
            pltpu.VMEM((8, D), F32),
            pltpu.SemaphoreType.DMA((6 + 8 * n_chunks,)),
        ],
        compiler_params=pltpu.CompilerParams(vmem_limit_bytes=110 * 1024 * 1024),
        name="rmt_mod",
    )(A_x.reshape(S, D), A_mem0.reshape(M, D), A_Wq.reshape(2, D * H // 2, Dh), A_Wk.reshape(2, D * H // 2, Dh),
      A_Wv.reshape(2, D * H // 2, Dh), A_Wo.reshape(H * Dh, D), B_w_r, B_w_gate, B_w_up, B_w_down)
    return out.reshape(B, S, D)
```

```python
import functools

import jax
import jax.numpy as jnp
from jax import lax
import jax.experimental.pallas as pl
import jax.experimental.pallas.tpu as pltpu

F32 = jnp.float32
BF16 = jnp.bfloat16
U32 = jnp.uint32
LANES = 128
DEPTH = 2
SCORES_AFTER = (7, 7, 7, 7, 7, 7, 7, 11)
VALUES_AFTER = (8, 8, 8, 8, 8, 8, 8, 8)
OUT_ORDER = ((0, 0), (1, 0), (0, 1), (1, 1), (0, 2), (1, 2), (0, 3), (1, 3))
UW = 2 * LANES
EPS_BF16 = 1.0013580322265625e-05
K, Q, V, O = 0, 1, 2, 3


def _rnd(x):
    return x.astype(BF16).astype(F32)


def _layernorm(x):
    inv_d = 1.0 / x.shape[-1]
    m = jnp.sum(x, axis=-1, keepdims=True) * inv_d
    c = x - m
    v = jnp.sum(c * c, axis=-1, keepdims=True) * inv_d
    sd = _rnd(jnp.sqrt(_rnd(_rnd(v) + EPS_BF16)))
    return _rnd(_rnd(x - _rnd(m)) / sd)


def _dot(a, b):
    return jnp.dot(a, b, preferred_element_type=F32)


def _rows(*xs):
    return xs[0] if len(xs) == 1 else jnp.concatenate(xs, axis=0)


def _feed(*xs):
    x = _rows(*xs)
    return x if x.shape[0] % 16 else x.astype(BF16)


def _cols(*xs):
    return jnp.concatenate(xs, axis=1)


def _right(b11, b12, b21, b22):
    return {1: b11 + b22, 2: b11, 3: b12 - b22, 4: b21 - b11, 5: b22, 6: b11 + b12, 7: b21 + b22}


def _left(i, a11, a12, a21, a22):
    return {1: lambda: a11 + a22, 2: lambda: a21 + a22, 3: lambda: a11, 4: lambda: a22,
            5: lambda: a11 + a12, 6: lambda: a21 - a11, 7: lambda: a12 - a22}[i]()


SET_A, SET_B, SET_C = (1, 3, 5, 7), (1, 2, 4, 6), (2, 3, 4, 5)
HALVES = {SET_A: {1: "x", 3: "x", 5: "x", 7: "xy"},
          SET_B: {1: "y", 2: "x", 4: "x", 6: "xy"},
          SET_C: {2: "y", 3: "y", 4: "y", 5: "y"}}


def _direct_left(ops, a1, a2):
    both = a1 + a2
    return {1: a1 if ops == SET_A else a2, 2: both, 3: a1, 4: a2, 5: both, 6: a1, 7: a2}


def _direct_out(ops, p):
    c1 = p[1] - p[5] + p[7] if ops == SET_A else p[2] + p[4]
    c2 = p[1] - p[2] + p[6] if ops == SET_B else p[3] + p[5]
    return c1, c2


def _kernel(x_hbm, mem0_hbm, wq_hbm, wk_hbm, wv_hbm, wo_hbm, wr_hbm, wg_hbm, wu_hbm, wd_hbm,
            out_hbm,
            raw_ref, rawo_ref, wk_ref, wq_ref, wv_ref, wo_ref, wg_ref, wu_ref, wd_ref,
            xr_ref, xm_ref, n_ref, ly_ref, px_ref, py_ref, left_ref, o_ref, onext_ref, a_ref,
            patch_ref, mem0_ref, wr1_ref, wr_ref, sems,
            *, seg, n_heads, n_chunks):
    S, D = x_hbm.shape
    M = mem0_ref.shape[0]
    Dh = LANES
    n_seg = S // seg
    L = M + seg
    G = n_heads // 4
    HD = D // 2
    P = 3 * seg
    R = P // 4
    n_per = (n_seg - 1) // 3
    scale = Dh ** -0.5

    hp = n_heads // 2

    w_hbm = {Q: wq_hbm, K: wk_hbm, V: wv_hbm}
    w_ref = {Q: wq_ref, K: wk_ref, V: wv_ref, O: wo_ref}
    op_rows = G * HD // 2

    def ahead_rows(k, g, r):
        return pl.ds(pl.multiple_of(7 * op_rows + (k * G + g) * n_per * R + r, 8), R)

    d_chunk = HD // n_chunks
    o_chunk = hp // n_chunks

    def w_copies(mat, c):
        sem = 6 + 2 * (mat * n_chunks + c)
        if mat > V:
            r = pl.ds(c * o_chunk * UW, o_chunk * UW)
            return [pltpu.make_async_copy(wo_hbm.at[r], rawo_ref.at[r], sems.at[sem])]
        r = pl.ds(c * d_chunk * n_heads, d_chunk * n_heads)
        return [pltpu.make_async_copy(w_hbm[mat].at[half, r], raw_ref.at[mat, half, r], sems.at[sem + half])
                for half in range(2)]

    x_copy = pltpu.make_async_copy(x_hbm, xr_ref.at[pl.ds(0, S)], sems.at[0])
    ffn_copies = [pltpu.make_async_copy(src, dst, sems.at[1 + i])
                  for i, (src, dst) in enumerate(((wg_hbm, wg_ref), (wu_hbm, wu_ref), (wd_hbm, wd_ref)))]
    small_copies = [pltpu.make_async_copy(mem0_hbm, mem0_ref, sems.at[4]),
                    pltpu.make_async_copy(wr_hbm, wr1_ref, sems.at[5])]
    x_copy.start()
    for cp in small_copies:
        cp.start()
    for mat in range(DEPTH):
        for c in range(n_chunks):
            for cp in w_copies(mat, c):
                cp.start()

    a_ref[...] = jnp.zeros_like(a_ref)
    x_copy.wait()
    for cp in small_copies:
        cp.wait()
    wr_ref[...] = jnp.broadcast_to(wr1_ref[...].astype(F32).reshape(1, D), wr_ref.shape)
    n_ref[:seg, :] = _layernorm(xr_ref[:seg, :].astype(F32))

    def ln_body(jj, carry):
        for j in [jj * 3 + u for u in range(3)]:
            rs = pl.ds(pl.multiple_of(seg + j * P, seg), P)
            n = _layernorm(xr_ref[rs, :].astype(F32))
            n_ref[rs, :] = n
            y = (n[2 * R:3 * R, :HD], n[2 * R:3 * R, HD:], n[3 * R:, :HD], n[3 * R:, HD:])
            for t, i in enumerate((6, 7)):
                ly_ref[t, pl.ds(pl.multiple_of(j * R, 8), R), :] = _left(i, *y)
        return carry

    lax.fori_loop(0, n_per // 3, ln_body, 0)

    def pack(x):
        return pltpu.bitcast(x.astype(BF16), U32)

    raw32 = raw_ref.bitcast(U32)

    def prep_in(mat, c, t):
        b, j = divmod(t, hp)
        d0 = c * d_chunk + b * 16
        dst = j // 2 * (HD // 2) + c * (d_chunk // 2) + b * 8
        w1, w2 = (raw32.at[mat, half, pl.ds(pl.multiple_of(d0 * hp, 16 * hp), 16 * hp)][pl.ds(j, 16, stride=hp), :]
                  for half in range(2))
        blocks = [pltpu.bitcast(w, F32) for w in (w1 << 16, w1 & U32(0xFFFF0000), w2 << 16, w2 & U32(0xFFFF0000))]
        for op, w in _right(*blocks).items():
            w_ref[mat][pl.ds(pl.multiple_of((op - 1) * op_rows + dst, 8), 8), pl.ds(j % 2 * Dh, Dh)] = pack(w)

    def prep_out(c, t):
        j, r = divmod(t * 16, Dh)
        even, odd = (rawo_ref[pl.ds(pl.multiple_of((c * o_chunk + j) * UW + p * Dh + r, 16), 16), :].astype(F32)
                     for p in range(2))
        dst = c * (o_chunk * Dh // 2) + t * 8
        for op, w in _right(even[:, :HD], even[:, HD:], odd[:, :HD], odd[:, HD:]).items():
            wo_ref[pl.ds(pl.multiple_of((op - 1) * op_rows + dst, 8), 8), :] = pack(w)

    def w_in(i, mat, g, r=0, rows=HD // 2):
        r = (i - 1) * op_rows + g * (HD // 2) + r
        return pltpu.bitcast(w_ref[mat][pl.ds(r if isinstance(r, int) else pl.multiple_of(r, 8), rows), :], BF16)

    for mat in (K, Q, V, O):
        def stream(c, carry, mat=mat):
            for cp in w_copies(mat, c):
                cp.wait()
            prep, n_prep = ((functools.partial(prep_in, mat), d_chunk // 16 * hp) if mat < O
                            else (prep_out, o_chunk * Dh // 16))
            n_dot = G // n_chunks * 2
            for t in range(n_dot):
                g, k = c * (G // n_chunks) + t // 2, t % 2
                if mat > K:
                    prod = pltpu.bitcast(_dot(ly_ref[k], w_in(6 + k, mat - 1, g)), U32)
                for j in range(n_per):
                    for i in range((t * n_per + j) * n_prep // (n_dot * n_per),
                                   (t * n_per + j + 1) * n_prep // (n_dot * n_per)):
                        prep(c, i)
                    if mat > K:
                        w_ref[mat][ahead_rows(k, g, j * R), :] = prod[j * R:(j + 1) * R]
            if mat + DEPTH <= O:
                for cp in w_copies(mat + DEPTH, c):
                    cp.start()
            return carry

        lax.fori_loop(0, n_chunks, stream, 0)
    for cp in ffn_copies:
        cp.start()

    def token_left(halves, t0):
        def block(r):
            t = n_ref[pl.ds(pl.multiple_of(t0 + r * R, 8), R), :]
            return t[:, :HD], t[:, HD:]

        used = "".join(halves.values())
        blocks = {h: block(r) + block(r + 1) for h, r in (("x", 0), ("y", 2)) if h in used}
        return {i: [_left(i, *blocks[h]) for h in hs] for i, hs in halves.items()}

    def split(hs, prod):
        return {h: prod[t * R:(t + 1) * R] for t, h in enumerate(hs)}

    def in_tokens(ops, mat, g, m, it):
        if ops == SET_A:
            if "x" in m[7]:
                px_ref[0, mat, g] = m[1]["x"] - m[5]["x"] + m[7]["x"]
                px_ref[1, mat, g] = m[3]["x"] + m[5]["x"]
                px_ref[2, mat, g] = m[1]["x"] + m[3]["x"]
            if "y" in m[7]:
                px_ref[3, mat, g] = m[7]["y"]
            return None if it is None else (left_ref[0, mat, g], left_ref[1, mat, g])
        if ops == SET_B:
            even = _rows(px_ref[0, mat, g] + m[4]["x"], m[2]["x"] + m[4]["x"])
            odd = _rows(px_ref[1, mat, g], px_ref[2, mat, g] - m[2]["x"] + m[6]["x"])
            if "y" in m[6]:
                m6, m7 = m[6]["y"], px_ref[3, mat, g]
            else:
                m6, m7 = (pltpu.bitcast(w_ref[mat + 1][ahead_rows(k, g, it * R), :], F32) for k in range(2))
            py_ref[0, mat, g] = m7 + m[1]["y"]
            py_ref[1, mat, g] = m[1]["y"] + m6
            left_ref[0, mat, g, :2 * R - seg] = even[seg:]
            left_ref[1, mat, g, :2 * R - seg] = odd[seg:]
            return even[:seg], odd[:seg]
        even = _rows(left_ref[0, mat, g, :2 * R - seg],
                     py_ref[0, mat, g] + m[4]["y"] - m[5]["y"], m[2]["y"] + m[4]["y"])
        odd = _rows(left_ref[1, mat, g, :2 * R - seg],
                    m[3]["y"] + m[5]["y"], py_ref[1, mat, g] - m[2]["y"] + m[3]["y"])
        left_ref[0, mat, g] = even[seg:]
        left_ref[1, mat, g] = odd[seg:]
        return even[:seg], odd[:seg]

    def attend(ops, halves, t0, it, direct, o_dst, o_row, tail):
        nd = direct[0].shape[0]
        dl = [_direct_left(ops, direct[t], direct[2 + t]) for t in range(2)]
        tl = token_left(halves, t0)
        tiles = {i: [_feed(*[x[:, t * LANES:(t + 1) * LANES] for x in tl[i]], dl[t][i]) for t in range(2)]
                 for i in ops}
        lhs = {i: _cols(*tiles[i]) for i in ops}
        qi = lax.broadcasted_iota(jnp.int32, (L, L), 0)
        ki = lax.broadcasted_iota(jnp.int32, (L, L), 1)
        visible = (qi >= seg) | (ki >= seg) | (qi >= ki)
        qkv, e, inv, o_mem = {}, {}, {}, {}

        def first_units(i, t):
            w = _cols(*[w_in(i, K, g, t * LANES // 2, LANES // 2) for g in range(2)])
            return _dot(tiles[i][t], w)

        early = {i: first_units(i, 0) for i in ops}
        early = {i: first_units(i, 1) + early[i] for i in ops}
        clock, due = [0], {}

        def tick():
            clock[0] += 1
            for job in due.pop(clock[0], ()):
                job()

        def later(rounds, job, g):
            due.setdefault(clock[0] + rounds, []).append(functools.partial(job, g))

        def project(mat, g):
            prod = {}
            for i in ops:
                if mat == K and g < 2:
                    prod[i] = early[i][:, g * UW:(g + 1) * UW]
                else:
                    prod[i] = _dot(lhs[i], w_in(i, mat, g))
                    tick()
            pair = _direct_out(ops, {i: prod[i][-nd:] for i in ops})
            own = in_tokens(ops, mat, g, {i: split(halves[i], prod[i]) for i in ops}, it)
            if own is not None:
                pair = [_rows(t, d) for t, d in zip(own, pair)]
            for p, x in enumerate(pair):
                x = x if mat == Q else x.astype(BF16)
                for j in range(2):
                    qkv[mat, g, p, j] = x[:, j * Dh:(j + 1) * Dh]

        heads = [(p, j) for p in range(2) for j in range(2)]

        def scores(g):
            for p, j in heads:
                sc = lax.dot_general(qkv[Q, g, p, j], qkv[K, g, p, j], (((1,), (1,)), ((), ())),
                                     preferred_element_type=F32)
                sc = jnp.where(visible, sc * scale, -1e9)
                w = jnp.exp(sc - jnp.max(sc, axis=-1, keepdims=True))
                e[g, p, j] = w
                inv[g, p, j] = pl.reciprocal(jnp.sum(w, axis=-1, keepdims=True), approx=True)
            later(VALUES_AFTER[g], values, g)

        def values(g):
            for p, j in heads:
                o = _dot(e[g, p, j], qkv[V, g, p, j]) * inv[g, p, j]
                o_dst[p, o_row:o_row + seg, (2 * g + j) * Dh:(2 * g + j + 1) * Dh] = o[:seg]
                o_mem[p, 2 * g + j] = o[seg:]

        project(K, 0)
        project(K, 1)
        for g in range(G):
            project(Q, g)
            later(SCORES_AFTER[g], scores, g)
            project(V, g)
            if g + 2 < G:
                project(K, g + 2)
        return tail(o_mem, tick)

    def project_out(ops, with_tokens, direct, tick=lambda: None):
        n_k = hp // 4
        lhs, acc = {}, {}

        def run(n, kk):
            c = slice(kk * 4 * Dh, (kk + 1) * 4 * Dh)
            if kk not in lhs:
                dl = _direct_left(ops, *direct(kk))
                block = lambda r: (o_ref[0, r * R:(r + 1) * R, c], o_ref[1, r * R:(r + 1) * R, c])
                used = "".join(HALVES[ops].values()) if with_tokens else ""
                blocks = {h: block(r) + block(r + 1) for h, r in (("y", 0), ("x", 2)) if h in used}
                lhs[kk] = {i: _feed(dl[i], *[_left(i, *blocks[h]) for h in HALVES[ops][i] if h in used])
                           for i in ops}
            for i in ops:
                w = wo_ref[pl.ds((i - 1) * op_rows + kk * 2 * Dh, 2 * Dh), n * LANES:(n + 1) * LANES]
                t = _dot(lhs[kk][i], pltpu.bitcast(w, BF16))
                acc[i, n] = t + acc[i, n] if kk else t
                tick()

        for n, kk in OUT_ORDER:
            run(n, kk)
        prod = {i: _cols(*[acc[i, n] for n in range(HD // LANES)]) for i in ops}
        nd = direct(0)[0].shape[0]
        res = [_direct_out(ops, {i: acc[i, n][:nd] for i in ops}) for n in range(HD // LANES)]
        res = tuple(r[p] for p in range(2) for r in res)
        return res, {i: split(HALVES[ops][i], prod[i][nd:]) for i in ops} if with_tokens else None

    def mem_rows(o_mem):
        return lambda kk: tuple(_cols(*[o_mem[p, 4 * kk + t] for t in range(4)]) for p in range(2))

    def router(n):
        return _rnd(jnp.sum(n * _rows(*[wr_ref[...]] * (n.shape[0] // 8)), axis=-1, keepdims=True))

    def finish(s, a, best, more=True):
        src = pl.ds(pl.multiple_of(jnp.maximum(s, 0) * seg, seg), seg)
        rs = pl.ds(pl.multiple_of(jnp.where(s < 0, n_seg, s) * seg, seg), seg)
        x1 = _rnd(xr_ref[src, :].astype(F32) + a)
        n1 = _layernorm(x1)
        x2 = _rnd(x1 + n1)
        xm_ref[rs, :] = x1.astype(BF16)
        xr_ref[rs, :] = x2.astype(BF16)
        n_ref[rs, :] = _layernorm(x2) if more else x2
        r = jnp.where(s < 0, -jnp.inf, jnp.broadcast_to(router(n1), (seg, LANES)))
        best_r, best_i = best
        sub = lax.broadcasted_iota(jnp.int32, (8, LANES), 0)
        for b in range(seg // 8):
            rb = r[b * 8:(b + 1) * 8]
            better = rb > best_r
            best_r = jnp.where(better, rb, best_r)
            best_i = jnp.where(better, sub + (s * seg + b * 8), best_i)
        return best_r, best_i

    def riders(l, ops):
        return {i: hs[0] if l == 0 else hs for i, hs in HALVES[ops].items()}

    n_early = (n_seg - 7) * seg
    early_copy = pltpu.make_async_copy(xr_ref.at[pl.ds(0, n_early)], out_hbm.at[pl.ds(0, n_early)], sems.at[0])
    late_copy = pltpu.make_async_copy(xr_ref.at[pl.ds(n_early, S - n_early)],
                                      out_hbm.at[pl.ds(n_early, S - n_early)], sems.at[1])

    def period(l, it, carry):
        mem, best = carry
        if l == 1:
            pl.when(it == n_per - 1)(early_copy.start)
        t0 = seg + it * P
        t1 = jnp.where(it == n_per - 1, seg, t0 + P)
        o_ref[:, :seg, :] = onext_ref[...]
        m = {}
        for u, (ops_in, t, ops_out, dst, row) in enumerate(((SET_B, t0, SET_C, o_ref, seg),
                                                           (SET_C, t0, SET_B, o_ref, 2 * seg),
                                                           (SET_A, t1, SET_A, onext_ref, 0))):
            def tail(o_mem, tick, u=u, ops_out=ops_out):
                new_best = finish(3 * (it - 1) + u, a_ref[u * seg:(u + 1) * seg, :], best, l == 0)
                return project_out(ops_out, True, mem_rows(o_mem), tick), new_best

            (mem, prods), best = attend(ops_in, riders(l, ops_in), t, it, mem, dst, row, tail)
            for i in ops_out:
                for h, x in prods[i].items():
                    m[i, h] = x
        for t, h in enumerate("yx"):
            top = _cols(m[1, h] + m[4, h] - m[5, h] + m[7, h], m[3, h] + m[5, h])
            bottom = _cols(m[2, h] + m[4, h], m[1, h] - m[2, h] + m[3, h] + m[6, h])
            a_ref[2 * t * R:2 * (t + 1) * R, :] = _rnd(_rows(top, bottom))
        return mem, best

    def layer(l, routed):
        @pl.when((routed >= seg) & (routed < seg + P))
        def _():
            def unit(g, carry):
                tl = token_left(riders(0, SET_A), seg)
                for mat in (K, Q, V):
                    in_tokens(SET_A, mat, g, {i: {"x": _dot(tl[i][0], w_in(i, mat, g))} for i in SET_A}, None)
                return carry

            lax.fori_loop(0, G, unit, 0)

        mem = attend(SET_A, {i: hs[1:] for i, hs in HALVES[SET_A].items()}, seg, None,
                     jnp.split(_rows(n_ref[:seg, :], mem0_ref[...].astype(F32)), D // LANES, axis=1), onext_ref, 0,
                     lambda o_mem, tick: project_out(SET_C, False, mem_rows(o_mem), tick)[0])
        best = (jnp.full((8, LANES), -jnp.inf, F32), lax.broadcasted_iota(jnp.int32, (8, LANES), 0))
        carry = lax.fori_loop(0, (1 - l) * n_per, functools.partial(period, 0), (mem, best))
        _, best = lax.fori_loop(0, l * n_per, functools.partial(period, 1), carry)

        @pl.when(l == 0)
        def _():
            for cp in ffn_copies:
                cp.wait()

        last, _ = project_out(SET_C, False, lambda kk: tuple(
            onext_ref[p, :, kk * 4 * Dh:(kk + 1) * 4 * Dh] for p in range(2)))
        for u in range(3):
            best = finish(n_seg - 4 + u, a_ref[u * seg:(u + 1) * seg, :], best)
        best_r, best_i = finish(n_seg - 1, _rnd(_cols(*last)), best)
        pl.when(l == 1)(late_copy.start)

        top = jnp.max(best_r, axis=0, keepdims=True)
        idx = jnp.min(jnp.where(best_r == top, best_i, S - 1))
        base = pl.multiple_of(jnp.clip(idx // 16 * 16, 0, S - 16), 16)
        rs = pl.ds(base, 16)
        x1 = xm_ref[rs, :].astype(F32)
        n1 = _layernorm(x1)
        nb = n1.astype(BF16)
        gate = _rnd(_dot(nb, wg_ref[...]))
        gate = _rnd(gate * jax.nn.sigmoid(gate))
        up = _rnd(_dot(nb, wu_ref[...]))
        y = _rnd(_dot((gate * up).astype(BF16), wd_ref[...]))
        y = _rnd(y * _rnd(jax.nn.sigmoid(router(n1))))
        chosen = lax.broadcasted_iota(jnp.int32, (16, D), 0) == idx - base
        x2 = _rnd(x1 + _rnd(n1 + jnp.where(chosen, y, 0.0)))
        patch_ref[...] = x2.astype(BF16)

        @pl.when(l == 0)
        def _():
            xr_ref[rs, :] = x2.astype(BF16)
            n_ref[rs, :] = _layernorm(x2)

        return idx

    routed = lax.fori_loop(0, 2, layer, jnp.int32(seg))
    early_copy.wait()
    late_copy.wait()
    base = pl.multiple_of(jnp.clip(routed // 16 * 16, 0, S - 16), 16)
    patch_copy = pltpu.make_async_copy(patch_ref, out_hbm.at[pl.ds(base, 16)], sems.at[0])
    patch_copy.start()
    patch_copy.wait()


@functools.partial(jax.jit, static_argnames=("A_seg_len",))
def pallas_interleave_layers__memory_aug_recurrent_mem_tr__moe_arch_mod__prompt_kernel(
    A_x, A_mem0, A_Wq, A_Wk, A_Wv, A_Wo, A_seg_len, B_x, B_w_r, B_w_gate, B_w_up, B_w_down,
):
    del B_x
    B, S, D = A_x.shape
    _, H, Dh = A_Wq.shape
    M = A_mem0.shape[1]
    F = B_w_gate.shape[1]
    seg = int(A_seg_len)
    assert B == 1 and Dh == LANES and D == 4 * LANES and H % 8 == 0 and M % 8 == 0
    assert seg % 32 == 0 and S % seg == 0 and (S // seg) % 9 == 1 and S // seg > 7
    n_chunks = 4
    half = H * Dh // 2
    R = 3 * seg // 4
    hbm = pl.BlockSpec(memory_space=pl.ANY)
    out = pl.pallas_call(
        functools.partial(_kernel, seg=seg, n_heads=H, n_chunks=n_chunks),
        out_shape=jax.ShapeDtypeStruct((S, D), A_x.dtype),
        in_specs=[hbm] * 10,
        out_specs=hbm,
        scratch_shapes=[
            pltpu.VMEM((3, 2, D * H // 2, Dh), BF16),
            pltpu.VMEM((H * Dh, D), BF16),
            pltpu.VMEM((7 * half // 2, UW), U32),
            *[pltpu.VMEM((7 * half // 2 + H // 2 * (S - seg) // 4, UW), U32)] * 3,
            pltpu.VMEM((D, F), BF16),
            pltpu.VMEM((D, F), BF16),
            pltpu.VMEM((F, D), BF16),
            pltpu.VMEM((S + seg, D), BF16),
            pltpu.VMEM((S + seg, D), BF16),
            pltpu.VMEM((S + seg, D), F32),
            pltpu.VMEM((2, (S - seg) // 4, D // 2), F32),
            pltpu.VMEM((4, 3, H // 4, R, UW), F32),
            pltpu.VMEM((2, 3, H // 4, R, UW), F32),
            pltpu.VMEM((2, 3, H // 4, seg, UW), F32),
            pltpu.VMEM((2, 3 * seg, half), F32),
            pltpu.VMEM((2, seg, half), F32),
            pltpu.VMEM((3 * seg, D), F32),
            pltpu.VMEM((16, D), BF16),
            pltpu.VMEM((M, D), BF16),
            pltpu.VMEM((D,), BF16),
            pltpu.VMEM((8, D), F32),
            pltpu.SemaphoreType.DMA((6 + 8 * n_chunks,)),
        ],
        compiler_params=pltpu.CompilerParams(vmem_limit_bytes=110 * 1024 * 1024),
        name="rmt_mod",
    )(A_x.reshape(S, D), A_mem0.reshape(M, D), A_Wq.reshape(2, D * H // 2, Dh), A_Wk.reshape(2, D * H // 2, Dh),
      A_Wv.reshape(2, D * H // 2, Dh), A_Wo.reshape(H * Dh, D), B_w_r, B_w_gate, B_w_up, B_w_down)
    return out.reshape(B, S, D)
```

```python
import functools

import jax
import jax.numpy as jnp
from jax import lax
import jax.experimental.pallas as pl
import jax.experimental.pallas.tpu as pltpu

F32 = jnp.float32
BF16 = jnp.bfloat16
U32 = jnp.uint32
LANES = 128
DEPTH = 2
SCORES_AFTER = (7, 7, 7, 7, 7, 7, 7, 11)
VALUES_AFTER = (8, 8, 8, 8, 8, 8, 8, 8)
OUT_ORDER = ((0, 0), (1, 0), (0, 1), (1, 1), (0, 2), (1, 2), (0, 3), (1, 3))
UW = 2 * LANES
EPS_BF16 = 1.0013580322265625e-05
K, Q, V, O = 0, 1, 2, 3


def _rnd(x):
    return x.astype(BF16).astype(F32)


def _layernorm(x):
    inv_d = 1.0 / x.shape[-1]
    m = jnp.sum(x, axis=-1, keepdims=True) * inv_d
    c = x - m
    v = jnp.sum(c * c, axis=-1, keepdims=True) * inv_d
    sd = _rnd(jnp.sqrt(_rnd(_rnd(v) + EPS_BF16)))
    return _rnd(_rnd(x - _rnd(m)) / sd)


def _dot(a, b):
    return jnp.dot(a, b, preferred_element_type=F32)


def _rows(*xs):
    return xs[0] if len(xs) == 1 else jnp.concatenate(xs, axis=0)


def _feed(*xs):
    x = _rows(*xs)
    return x if x.shape[0] % 16 else x.astype(BF16)


def _cols(*xs):
    return jnp.concatenate(xs, axis=1)


def _right(b11, b12, b21, b22):
    return {1: b11 + b22, 2: b11, 3: b12 - b22, 4: b21 - b11, 5: b22, 6: b11 + b12, 7: b21 + b22}


def _left(i, a11, a12, a21, a22):
    return {1: lambda: a11 + a22, 2: lambda: a21 + a22, 3: lambda: a11, 4: lambda: a22,
            5: lambda: a11 + a12, 6: lambda: a21 - a11, 7: lambda: a12 - a22}[i]()


SET_A, SET_B, SET_C = (1, 3, 5, 7), (1, 2, 4, 6), (2, 3, 4, 5)
HALVES = {SET_A: {1: "x", 3: "x", 5: "x", 7: "xy"},
          SET_B: {1: "y", 2: "x", 4: "x", 6: "xy"},
          SET_C: {2: "y", 3: "y", 4: "y", 5: "y"}}


def _direct_left(ops, a1, a2):
    both = a1 + a2
    return {1: a1 if ops == SET_A else a2, 2: both, 3: a1, 4: a2, 5: both, 6: a1, 7: a2}


def _direct_out(ops, p):
    c1 = p[1] - p[5] + p[7] if ops == SET_A else p[2] + p[4]
    c2 = p[1] - p[2] + p[6] if ops == SET_B else p[3] + p[5]
    return c1, c2


def _kernel(x_hbm, mem0_hbm, wq_hbm, wk_hbm, wv_hbm, wo_hbm, wr_hbm, wg_hbm, wu_hbm, wd_hbm,
            out_hbm,
            raw_ref, rawo_ref, wk_ref, wq_ref, wv_ref, wo_ref, wg_ref, wu_ref, wd_ref,
            xr_ref, xm_ref, n_ref, ly_ref, px_ref, py_ref, left_ref, o_ref, onext_ref, a_ref,
            patch_ref, mem0_ref, wr1_ref, wr_ref, sems,
            *, seg, n_heads):
    S, D = x_hbm.shape
    M = mem0_ref.shape[0]
    Dh = LANES
    n_seg = S // seg
    L = M + seg
    G = n_heads // 4
    HD = D // 2
    P = 3 * seg
    R = P // 4
    n_per = (n_seg - 1) // 3
    scale = Dh ** -0.5

    hp = n_heads // 2

    w_hbm = {Q: wq_hbm, K: wk_hbm, V: wv_hbm}
    w_ref = {Q: wq_ref, K: wk_ref, V: wv_ref, O: wo_ref}
    op_rows = G * HD // 2

    def ahead_rows(k, g, r):
        return pl.ds(pl.multiple_of(7 * op_rows + (k * G + g) * n_per * R + r, 8), R)

    n_oct = n_heads // 8

    def w_copy(mat, c):
        sem = sems.at[6 + 4 * c + mat]
        if mat == O:
            return pltpu.make_async_copy(wo_hbm.at[pl.ds(c * 8 * Dh, 8 * Dh)], rawo_ref.at[c], sem)
        col = c * Dh if isinstance(c, int) else pl.multiple_of(c * Dh, Dh)
        return pltpu.make_async_copy(w_hbm[mat].at[:, pl.ds(col, Dh)], raw_ref.at[mat, c], sem)

    x_copy = pltpu.make_async_copy(x_hbm, xr_ref.at[pl.ds(0, S)], sems.at[0])
    ffn_copies = [pltpu.make_async_copy(src, dst, sems.at[1 + i])
                  for i, (src, dst) in enumerate(((wg_hbm, wg_ref), (wu_hbm, wu_ref), (wd_hbm, wd_ref)))]
    small_copies = [pltpu.make_async_copy(mem0_hbm, mem0_ref, sems.at[4]),
                    pltpu.make_async_copy(wr_hbm, wr1_ref, sems.at[5])]
    x_copy.start()
    for cp in small_copies:
        cp.start()
    for c in range(DEPTH):
        for mat in (K, Q, V, O):
            w_copy(mat, c).start()

    a_ref[...] = jnp.zeros_like(a_ref)
    x_copy.wait()
    for cp in small_copies:
        cp.wait()
    wr_ref[...] = jnp.broadcast_to(wr1_ref[...].astype(F32).reshape(1, D), wr_ref.shape)
    n_ref[:seg, :] = _layernorm(xr_ref[:seg, :].astype(F32))

    def ln_body(jj, carry):
        for j in [jj * 3 + u for u in range(3)]:
            rs = pl.ds(pl.multiple_of(seg + j * P, seg), P)
            n = _layernorm(xr_ref[rs, :].astype(F32))
            n_ref[rs, :] = n
            y = (n[2 * R:3 * R, :HD], n[2 * R:3 * R, HD:], n[3 * R:, :HD], n[3 * R:, HD:])
            for t, i in enumerate((6, 7)):
                ly_ref[t, pl.ds(pl.multiple_of(j * R, 8), R), :] = _left(i, *y)
        return carry

    lax.fori_loop(0, n_per // 3, ln_body, 0)

    def pack(x):
        return pltpu.bitcast(x.astype(BF16), U32)

    raw32 = raw_ref.bitcast(U32)

    def prep_in(mat, c, t):
        b, j = divmod(t, 4)
        dst = (2 * c + j // 2) * (HD // 2) + b * 8
        w1, w2 = (raw32.at[mat, c][pl.ds((half * HD + b * 16) * 4 + j, 16, stride=4), :] for half in range(2))
        blocks = [pltpu.bitcast(w, F32) for w in (w1 << 16, w1 & U32(0xFFFF0000), w2 << 16, w2 & U32(0xFFFF0000))]
        for op, w in _right(*blocks).items():
            w_ref[mat][pl.ds(pl.multiple_of((op - 1) * op_rows + dst, 8), 8), pl.ds(j % 2 * Dh, Dh)] = pack(w)

    def prep_out(c, t):
        j, r = divmod(t * 16, Dh)
        even, odd = (rawo_ref[c, pl.ds(j * UW + p * Dh + r, 16), :].astype(F32) for p in range(2))
        dst = c * 2 * Dh + t * 8
        for op, w in _right(even[:, :HD], even[:, HD:], odd[:, :HD], odd[:, HD:]).items():
            wo_ref[pl.ds(pl.multiple_of((op - 1) * op_rows + dst, 8), 8), :] = pack(w)

    def w_in(i, mat, g, r=0, rows=HD // 2):
        r = (i - 1) * op_rows + g * (HD // 2) + r
        return pltpu.bitcast(w_ref[mat][pl.ds(r if isinstance(r, int) else pl.multiple_of(r, 8), rows), :], BF16)

    def token_left(halves, t0):
        def block(r):
            t = n_ref[pl.ds(pl.multiple_of(t0 + r * R, 8), R), :]
            return t[:, :HD], t[:, HD:]

        used = "".join(halves.values())
        blocks = {h: block(r) + block(r + 1) for h, r in (("x", 0), ("y", 2)) if h in used}
        return {i: [_left(i, *blocks[h]) for h in hs] for i, hs in halves.items()}

    def split(hs, prod):
        return {h: prod[t * R:(t + 1) * R] for t, h in enumerate(hs)}

    def in_tokens(ops, mat, g, m, it):
        if ops == SET_A:
            if "x" in m[7]:
                px_ref[0, mat, g] = m[1]["x"] - m[5]["x"] + m[7]["x"]
                px_ref[1, mat, g] = m[3]["x"] + m[5]["x"]
                px_ref[2, mat, g] = m[1]["x"] + m[3]["x"]
            if "y" in m[7]:
                px_ref[3, mat, g] = m[7]["y"]
            return None if it is None else (left_ref[0, mat, g], left_ref[1, mat, g])
        if ops == SET_B:
            even = _rows(px_ref[0, mat, g] + m[4]["x"], m[2]["x"] + m[4]["x"])
            odd = _rows(px_ref[1, mat, g], px_ref[2, mat, g] - m[2]["x"] + m[6]["x"])
            if "y" in m[6]:
                m6, m7 = m[6]["y"], px_ref[3, mat, g]
            else:
                m6, m7 = (pltpu.bitcast(w_ref[mat + 1][ahead_rows(k, g, it * R), :], F32) for k in range(2))
            py_ref[0, mat, g] = m7 + m[1]["y"]
            py_ref[1, mat, g] = m[1]["y"] + m6
            left_ref[0, mat, g, :2 * R - seg] = even[seg:]
            left_ref[1, mat, g, :2 * R - seg] = odd[seg:]
            return even[:seg], odd[:seg]
        even = _rows(left_ref[0, mat, g, :2 * R - seg],
                     py_ref[0, mat, g] + m[4]["y"] - m[5]["y"], m[2]["y"] + m[4]["y"])
        odd = _rows(left_ref[1, mat, g, :2 * R - seg],
                    m[3]["y"] + m[5]["y"], py_ref[1, mat, g] - m[2]["y"] + m[3]["y"])
        left_ref[0, mat, g] = even[seg:]
        left_ref[1, mat, g] = odd[seg:]
        return even[:seg], odd[:seg]

    def first_products(g):
        tl = token_left({i: "x" for i in SET_A}, seg)
        for mat in (K, Q, V):
            in_tokens(SET_A, mat, g, {i: {"x": _dot(tl[i][0], w_in(i, mat, g))} for i in SET_A}, None)

    def stream(mat, c):
        w_copy(mat, c).wait()
        prep, n_prep = (prep_out, Dh // 4) if mat == O else (functools.partial(prep_in, mat), HD // 4)
        if mat == O:
            first_products(2 * c)
            first_products(2 * c + 1)
        for t in range(4):
            g, k = 2 * c + t // 2, t % 2
            if mat > K:
                prod = pltpu.bitcast(_dot(ly_ref[k], w_in(6 + k, mat - 1, g)), U32)
            for j in range(n_per):
                for i in range((t * n_per + j) * n_prep // (4 * n_per), (t * n_per + j + 1) * n_prep // (4 * n_per)):
                    prep(c, i)
                if mat > K:
                    w_ref[mat][ahead_rows(k, g, j * R), :] = prod[j * R:(j + 1) * R]

        @pl.when(c + DEPTH < n_oct)
        def _():
            w_copy(mat, jnp.minimum(c + DEPTH, n_oct - 1)).start()

    def stream_body(i, carry):
        for mat in (K, Q, V, O):
            pl.when(i % 4 == mat)(functools.partial(stream, mat, i // 4))
        return carry

    lax.fori_loop(0, 4 * n_oct, stream_body, 0)
    for cp in ffn_copies:
        cp.start()

    def attend(ops, halves, t0, it, direct, o_dst, o_row, tail):
        nd = direct[0].shape[0]
        dl = [_direct_left(ops, direct[t], direct[2 + t]) for t in range(2)]
        tl = token_left(halves, t0)
        tiles = {i: [_feed(*[x[:, t * LANES:(t + 1) * LANES] for x in tl[i]], dl[t][i]) for t in range(2)]
                 for i in ops}
        lhs = {i: _cols(*tiles[i]) for i in ops}
        qi = lax.broadcasted_iota(jnp.int32, (L, L), 0)
        ki = lax.broadcasted_iota(jnp.int32, (L, L), 1)
        visible = (qi >= seg) | (ki >= seg) | (qi >= ki)
        qkv, e, inv, o_mem = {}, {}, {}, {}

        def first_units(i, t):
            w = _cols(*[w_in(i, K, g, t * LANES // 2, LANES // 2) for g in range(2)])
            return _dot(tiles[i][t], w)

        early = {i: first_units(i, 0) for i in ops}
        early = {i: first_units(i, 1) + early[i] for i in ops}
        clock, due = [0], {}

        def tick():
            clock[0] += 1
            for job in due.pop(clock[0], ()):
                job()

        def later(rounds, job, g):
            due.setdefault(clock[0] + rounds, []).append(functools.partial(job, g))

        def project(mat, g):
            prod = {}
            for i in ops:
                if mat == K and g < 2:
                    prod[i] = early[i][:, g * UW:(g + 1) * UW]
                else:
                    prod[i] = _dot(lhs[i], w_in(i, mat, g))
                    tick()
            pair = _direct_out(ops, {i: prod[i][-nd:] for i in ops})
            own = in_tokens(ops, mat, g, {i: split(halves[i], prod[i]) for i in ops}, it)
            if own is not None:
                pair = [_rows(t, d) for t, d in zip(own, pair)]
            for p, x in enumerate(pair):
                x = x if mat == Q else x.astype(BF16)
                for j in range(2):
                    qkv[mat, g, p, j] = x[:, j * Dh:(j + 1) * Dh]

        heads = [(p, j) for p in range(2) for j in range(2)]

        def scores(g):
            for p, j in heads:
                sc = lax.dot_general(qkv[Q, g, p, j], qkv[K, g, p, j], (((1,), (1,)), ((), ())),
                                     preferred_element_type=F32)
                sc = jnp.where(visible, sc * scale, -1e9)
                w = jnp.exp(sc - jnp.max(sc, axis=-1, keepdims=True))
                e[g, p, j] = w
                inv[g, p, j] = pl.reciprocal(jnp.sum(w, axis=-1, keepdims=True), approx=True)
            later(VALUES_AFTER[g], values, g)

        def values(g):
            for p, j in heads:
                o = _dot(e[g, p, j], qkv[V, g, p, j]) * inv[g, p, j]
                o_dst[p, o_row:o_row + seg, (2 * g + j) * Dh:(2 * g + j + 1) * Dh] = o[:seg]
                o_mem[p, 2 * g + j] = o[seg:]

        project(K, 0)
        project(K, 1)
        for g in range(G):
            project(Q, g)
            later(SCORES_AFTER[g], scores, g)
            project(V, g)
            if g + 2 < G:
                project(K, g + 2)
        return tail(o_mem, tick)

    def project_out(ops, with_tokens, direct, tick=lambda: None):
        n_k = hp // 4
        lhs, acc = {}, {}

        def run(n, kk):
            c = slice(kk * 4 * Dh, (kk + 1) * 4 * Dh)
            if kk not in lhs:
                dl = _direct_left(ops, *direct(kk))
                block = lambda r: (o_ref[0, r * R:(r + 1) * R, c], o_ref[1, r * R:(r + 1) * R, c])
                used = "".join(HALVES[ops].values()) if with_tokens else ""
                blocks = {h: block(r) + block(r + 1) for h, r in (("y", 0), ("x", 2)) if h in used}
                lhs[kk] = {i: _rows(dl[i], *[_left(i, *blocks[h]) for h in HALVES[ops][i] if h in used])
                           for i in ops}
            for i in ops:
                w = wo_ref[pl.ds((i - 1) * op_rows + kk * 2 * Dh, 2 * Dh), n * LANES:(n + 1) * LANES]
                t = _dot(lhs[kk][i], pltpu.bitcast(w, BF16))
                acc[i, n] = t + acc[i, n] if kk else t
                tick()

        for n, kk in OUT_ORDER:
            run(n, kk)
        prod = {i: _cols(*[acc[i, n] for n in range(HD // LANES)]) for i in ops}
        nd = direct(0)[0].shape[0]
        res = [_direct_out(ops, {i: acc[i, n][:nd] for i in ops}) for n in range(HD // LANES)]
        res = tuple(r[p] for p in range(2) for r in res)
        return res, {i: split(HALVES[ops][i], prod[i][nd:]) for i in ops} if with_tokens else None

    def mem_rows(o_mem):
        return lambda kk: tuple(_cols(*[o_mem[p, 4 * kk + t] for t in range(4)]) for p in range(2))

    def router(n):
        return _rnd(jnp.sum(n * _rows(*[wr_ref[...]] * (n.shape[0] // 8)), axis=-1, keepdims=True))

    def finish(s, a, best, more=True):
        src = pl.ds(pl.multiple_of(jnp.maximum(s, 0) * seg, seg), seg)
        rs = pl.ds(pl.multiple_of(jnp.where(s < 0, n_seg, s) * seg, seg), seg)
        x1 = _rnd(xr_ref[src, :].astype(F32) + a)
        n1 = _layernorm(x1)
        x2 = _rnd(x1 + n1)
        xm_ref[rs, :] = x1.astype(BF16)
        xr_ref[rs, :] = x2.astype(BF16)
        n_ref[rs, :] = _layernorm(x2) if more else x2
        r = jnp.where(s < 0, -jnp.inf, jnp.broadcast_to(router(n1), (seg, LANES)))
        best_r, best_i = best
        sub = lax.broadcasted_iota(jnp.int32, (8, LANES), 0)
        for b in range(seg // 8):
            rb = r[b * 8:(b + 1) * 8]
            better = rb > best_r
            best_r = jnp.where(better, rb, best_r)
            best_i = jnp.where(better, sub + (s * seg + b * 8), best_i)
        return best_r, best_i

    def riders(l, ops):
        return {i: hs[0] if l == 0 else hs for i, hs in HALVES[ops].items()}

    n_early = (n_seg - 7) * seg
    early_copy = pltpu.make_async_copy(xr_ref.at[pl.ds(0, n_early)], out_hbm.at[pl.ds(0, n_early)], sems.at[0])
    late_copy = pltpu.make_async_copy(xr_ref.at[pl.ds(n_early, S - n_early)],
                                      out_hbm.at[pl.ds(n_early, S - n_early)], sems.at[1])

    def period(l, it, carry):
        mem, best = carry
        if l == 1:
            pl.when(it == n_per - 1)(early_copy.start)
        t0 = seg + it * P
        t1 = jnp.where(it == n_per - 1, seg, t0 + P)
        o_ref[:, :seg, :] = onext_ref[...]
        m = {}
        for u, (ops_in, t, ops_out, dst, row) in enumerate(((SET_B, t0, SET_C, o_ref, seg),
                                                           (SET_C, t0, SET_B, o_ref, 2 * seg),
                                                           (SET_A, t1, SET_A, onext_ref, 0))):
            def tail(o_mem, tick, u=u, ops_out=ops_out):
                new_best = finish(3 * (it - 1) + u, a_ref[u * seg:(u + 1) * seg, :], best, l == 0)
                return project_out(ops_out, True, mem_rows(o_mem), tick), new_best

            (mem, prods), best = attend(ops_in, riders(l, ops_in), t, it, mem, dst, row, tail)
            for i in ops_out:
                for h, x in prods[i].items():
                    m[i, h] = x
        for t, h in enumerate("yx"):
            top = _cols(m[1, h] + m[4, h] - m[5, h] + m[7, h], m[3, h] + m[5, h])
            bottom = _cols(m[2, h] + m[4, h], m[1, h] - m[2, h] + m[3, h] + m[6, h])
            a_ref[2 * t * R:2 * (t + 1) * R, :] = _rnd(_rows(top, bottom))
        return mem, best

    def layer(l, routed):
        @pl.when((routed >= seg) & (routed < seg + P))
        def _():
            pl.loop(0, G)(first_products)

        mem = attend(SET_A, {i: hs[1:] for i, hs in HALVES[SET_A].items()}, seg, None,
                     jnp.split(_rows(n_ref[:seg, :], mem0_ref[...].astype(F32)), D // LANES, axis=1), onext_ref, 0,
                     lambda o_mem, tick: project_out(SET_C, False, mem_rows(o_mem), tick)[0])
        best = (jnp.full((8, LANES), -jnp.inf, F32), lax.broadcasted_iota(jnp.int32, (8, LANES), 0))
        carry = lax.fori_loop(0, (1 - l) * n_per, functools.partial(period, 0), (mem, best))
        _, best = lax.fori_loop(0, l * n_per, functools.partial(period, 1), carry)

        @pl.when(l == 0)
        def _():
            for cp in ffn_copies:
                cp.wait()

        last, _ = project_out(SET_C, False, lambda kk: tuple(
            onext_ref[p, :, kk * 4 * Dh:(kk + 1) * 4 * Dh] for p in range(2)))
        for u in range(3):
            best = finish(n_seg - 4 + u, a_ref[u * seg:(u + 1) * seg, :], best)
        best_r, best_i = finish(n_seg - 1, _rnd(_cols(*last)), best)
        pl.when(l == 1)(late_copy.start)

        top = jnp.max(best_r, axis=0, keepdims=True)
        idx = jnp.min(jnp.where(best_r == top, best_i, S - 1))
        base = pl.multiple_of(jnp.clip(idx // 16 * 16, 0, S - 16), 16)
        rs = pl.ds(base, 16)
        x1 = xm_ref[rs, :].astype(F32)
        n1 = _layernorm(x1)
        nb = n1.astype(BF16)
        gate = _rnd(_dot(nb, wg_ref[...]))
        gate = _rnd(gate * jax.nn.sigmoid(gate))
        up = _rnd(_dot(nb, wu_ref[...]))
        y = _rnd(_dot((gate * up).astype(BF16), wd_ref[...]))
        y = _rnd(y * _rnd(jax.nn.sigmoid(router(n1))))
        chosen = lax.broadcasted_iota(jnp.int32, (16, D), 0) == idx - base
        x2 = _rnd(x1 + _rnd(n1 + jnp.where(chosen, y, 0.0)))
        patch_ref[...] = x2.astype(BF16)

        @pl.when(l == 0)
        def _():
            xr_ref[rs, :] = x2.astype(BF16)
            n_ref[rs, :] = _layernorm(x2)

        return idx

    routed = lax.fori_loop(0, 2, layer, jnp.int32(0))
    early_copy.wait()
    late_copy.wait()
    base = pl.multiple_of(jnp.clip(routed // 16 * 16, 0, S - 16), 16)
    patch_copy = pltpu.make_async_copy(patch_ref, out_hbm.at[pl.ds(base, 16)], sems.at[0])
    patch_copy.start()
    patch_copy.wait()


@functools.partial(jax.jit, static_argnames=("A_seg_len",))
def pallas_interleave_layers__memory_aug_recurrent_mem_tr__moe_arch_mod__prompt_kernel(
    A_x, A_mem0, A_Wq, A_Wk, A_Wv, A_Wo, A_seg_len, B_x, B_w_r, B_w_gate, B_w_up, B_w_down,
):
    del B_x
    B, S, D = A_x.shape
    _, H, Dh = A_Wq.shape
    M = A_mem0.shape[1]
    F = B_w_gate.shape[1]
    seg = int(A_seg_len)
    assert B == 1 and Dh == LANES and D == 4 * LANES and H % 8 == 0 and M % 8 == 0
    assert seg % 32 == 0 and S % seg == 0 and (S // seg) % 9 == 1 and S // seg > 7
    half = H * Dh // 2
    R = 3 * seg // 4
    hbm = pl.BlockSpec(memory_space=pl.ANY)

    def octets(w):
        return w.reshape(D, H // 8, 8, Dh).transpose(0, 2, 1, 3).reshape(8 * D, H // 8 * Dh)

    out = pl.pallas_call(
        functools.partial(_kernel, seg=seg, n_heads=H),
        out_shape=jax.ShapeDtypeStruct((S, D), A_x.dtype),
        in_specs=[hbm] * 10,
        out_specs=hbm,
        scratch_shapes=[
            pltpu.VMEM((3, H // 8, 8 * D, Dh), BF16),
            pltpu.VMEM((H // 8, 8 * Dh, D), BF16),
            pltpu.VMEM((7 * half // 2, UW), U32),
            *[pltpu.VMEM((7 * half // 2 + H // 2 * (S - seg) // 4, UW), U32)] * 3,
            pltpu.VMEM((D, F), BF16),
            pltpu.VMEM((D, F), BF16),
            pltpu.VMEM((F, D), BF16),
            pltpu.VMEM((S + seg, D), BF16),
            pltpu.VMEM((S + seg, D), BF16),
            pltpu.VMEM((S + seg, D), F32),
            pltpu.VMEM((2, (S - seg) // 4, D // 2), F32),
            pltpu.VMEM((4, 3, H // 4, R, UW), F32),
            pltpu.VMEM((2, 3, H // 4, R, UW), F32),
            pltpu.VMEM((2, 3, H // 4, seg, UW), F32),
            pltpu.VMEM((2, 3 * seg, half), F32),
            pltpu.VMEM((2, seg, half), F32),
            pltpu.VMEM((3 * seg, D), F32),
            pltpu.VMEM((16, D), BF16),
            pltpu.VMEM((M, D), BF16),
            pltpu.VMEM((D,), BF16),
            pltpu.VMEM((8, D), F32),
            pltpu.SemaphoreType.DMA((6 + H // 2,)),
        ],
        compiler_params=pltpu.CompilerParams(vmem_limit_bytes=110 * 1024 * 1024),
        name="rmt_mod",
    )(A_x.reshape(S, D), A_mem0.reshape(M, D), octets(A_Wq), octets(A_Wk),
      octets(A_Wv), A_Wo.reshape(H * Dh, D), B_w_r, B_w_gate, B_w_up, B_w_down)
    return out.reshape(B, S, D)
```

```python
import functools

import jax
import jax.numpy as jnp
from jax import lax
import jax.experimental.pallas as pl
import jax.experimental.pallas.tpu as pltpu

F32 = jnp.float32
BF16 = jnp.bfloat16
U32 = jnp.uint32
LANES = 128
DEPTH = 2
FINISH_STEP = ((0, 1, 2), (0, 0, 1, 1, 2, 2))
REST_STEP = 2
SCORES_AFTER = (7, 7, 7, 7, 7, 7, 7, 11)
VALUES_AFTER = (8, 8, 8, 8, 8, 8, 8, 8)
OUT_ORDER = ((0, 0), (1, 0), (0, 1), (1, 1), (0, 2), (1, 2), (0, 3), (1, 3))
UW = 2 * LANES
EPS_BF16 = 1.0013580322265625e-05
K, Q, V, O = 0, 1, 2, 3


def _rnd(x):
    return x.astype(BF16).astype(F32)


def _layernorm(x, stepwise=False):
    inv_d = 1.0 / x.shape[-1]
    m = jnp.sum(x, axis=-1, keepdims=True) * inv_d
    c = x - m
    v = jnp.sum(c * c, axis=-1, keepdims=True) * inv_d
    if not stepwise:
        return c * lax.rsqrt(v + 1e-5)
    sd = _rnd(jnp.sqrt(_rnd(_rnd(v) + EPS_BF16)))
    return _rnd(_rnd(x - _rnd(m)) / sd)


def _dot(a, b):
    return jnp.dot(a, b, preferred_element_type=F32)


def _rows(*xs):
    return xs[0] if len(xs) == 1 else jnp.concatenate(xs, axis=0)


def _feed(*xs):
    x = _rows(*xs)
    return x if x.shape[0] % 16 else x.astype(BF16)


def _cols(*xs):
    return jnp.concatenate(xs, axis=1)


def _right(b11, b12, b21, b22):
    return {1: b11 + b22, 2: b11, 3: b12 - b22, 4: b21 - b11, 5: b22, 6: b11 + b12, 7: b21 + b22}


def _left(i, a11, a12, a21, a22):
    return {1: lambda: a11 + a22, 2: lambda: a21 + a22, 3: lambda: a11, 4: lambda: a22,
            5: lambda: a11 + a12, 6: lambda: a21 - a11, 7: lambda: a12 - a22}[i]()


SET_A, SET_B, SET_C = (1, 3, 5, 7), (1, 2, 4, 6), (2, 3, 4, 5)
HALVES = {SET_A: {1: "x", 3: "x", 5: "x", 7: "xy"},
          SET_B: {1: "y", 2: "x", 4: "x", 6: "xy"},
          SET_C: {2: "y", 3: "y", 4: "y", 5: "y"}}


def _direct_left(ops, a1, a2):
    both = a1 + a2
    return {1: a1 if ops == SET_A else a2, 2: both, 3: a1, 4: a2, 5: both, 6: a1, 7: a2}


def _direct_out(ops, p):
    c1 = p[1] - p[5] + p[7] if ops == SET_A else p[2] + p[4]
    c2 = p[1] - p[2] + p[6] if ops == SET_B else p[3] + p[5]
    return c1, c2


def _kernel(x_hbm, mem0_hbm, wq_hbm, wk_hbm, wv_hbm, wo_hbm, wr_hbm, wg_hbm, wu_hbm, wd_hbm,
            out_hbm,
            raw_ref, rawo_ref, wk_ref, wq_ref, wv_ref, wo_ref, wg_ref, wu_ref, wd_ref,
            xr_ref, xm_ref, n_ref, ly_ref, px_ref, py_ref, left_ref, o_ref, onext_ref, a_ref,
            patch_ref, mem0_ref, wr1_ref, wr_ref, sems,
            *, seg, n_heads):
    S, D = x_hbm.shape
    M = mem0_ref.shape[0]
    Dh = LANES
    n_seg = S // seg
    L = M + seg
    G = n_heads // 4
    HD = D // 2
    P = 3 * seg
    R = P // 4
    n_per = (n_seg - 1) // 3
    scale = Dh ** -0.5

    hp = n_heads // 2

    w_hbm = {Q: wq_hbm, K: wk_hbm, V: wv_hbm}
    w_ref = {Q: wq_ref, K: wk_ref, V: wv_ref, O: wo_ref}
    op_rows = G * HD // 2

    def ahead_rows(k, g, r):
        return pl.ds(pl.multiple_of(7 * op_rows + (k * G + g) * n_per * R + r, 8), R)

    n_oct = n_heads // 8

    def w_copy(mat, c):
        sem = sems.at[9 + 4 * c + mat]
        if mat == O:
            return pltpu.make_async_copy(wo_hbm.at[pl.ds(c * 8 * Dh, 8 * Dh)], rawo_ref.at[c], sem)
        col = c * Dh if isinstance(c, int) else pl.multiple_of(c * Dh, Dh)
        return pltpu.make_async_copy(w_hbm[mat].at[:, pl.ds(col, Dh)], raw_ref.at[mat, c, pl.ds(0, 8 * D)], sem)

    def x_copy(row, rows, sem):
        rs = pl.ds(row if isinstance(row, int) else pl.multiple_of(row, 16), rows)
        return pltpu.make_async_copy(x_hbm.at[rs], xr_ref.at[rs], sems.at[sem])

    n_ln = n_per // 3
    y_copy = lambda j, group: x_copy(seg + j * P + 2 * R, 2 * R, 6 + group)
    rest_copies = [x_copy(seg + j * P, 2 * R, 0) for j in range(2, n_per)]
    ffn_copies = [pltpu.make_async_copy(src, dst, sems.at[1 + i])
                  for i, (src, dst) in enumerate(((wg_hbm, wg_ref), (wu_hbm, wu_ref), (wd_hbm, wd_ref)))]
    first_copies = [x_copy(0, seg + 2 * R, 0), x_copy(seg + P, 2 * R, 1),
                    pltpu.make_async_copy(mem0_hbm, mem0_ref, sems.at[4]),
                    pltpu.make_async_copy(wr_hbm, wr1_ref, sems.at[5])]
    for cp in first_copies:
        cp.start()
    for j in range(n_per):
        y_copy(j, j // n_ln).start()
    for c in range(DEPTH):
        for mat in (K, Q, V, O):
            w_copy(mat, c).start()

    a_ref[...] = jnp.zeros_like(a_ref)
    for cp in first_copies:
        cp.wait()
    wr_ref[...] = jnp.broadcast_to(wr1_ref[...].astype(F32).reshape(1, D), wr_ref.shape)
    for rs in (pl.ds(0, seg + 2 * R), pl.ds(seg + P, 2 * R)):
        n_ref[rs, :] = _layernorm(xr_ref[rs, :].astype(F32))

    def ln_body(group, carry):
        for u in range(n_ln):
            y_copy(group * n_ln + u, group).wait()
        for j in [group * n_ln + u for u in range(n_ln)]:
            rs = pl.ds(pl.multiple_of(seg + j * P + 2 * R, 16), 2 * R)
            n = _layernorm(xr_ref[rs, :].astype(F32))
            n_ref[rs, :] = n
            for t, i in enumerate((6, 7)):
                ly_ref[t, pl.ds(pl.multiple_of(j * R, 8), R), :] = _left(
                    i, n[:R, :HD], n[:R, HD:], n[R:, :HD], n[R:, HD:])
        return carry

    lax.fori_loop(0, 3, ln_body, 0)

    def pack(x):
        return pltpu.bitcast(x.astype(BF16), U32)

    raw32 = raw_ref.bitcast(U32)

    def prep_in(mat, c, t):
        b, j = divmod(t, 4)
        dst = (2 * c + j // 2) * (HD // 2) + b * 8
        w1, w2 = (raw32.at[mat, c][pl.ds((half * HD + b * 16) * 4 + j, 16, stride=4), :] for half in range(2))
        blocks = [pltpu.bitcast(w, F32) for w in (w1 << 16, w1 & U32(0xFFFF0000), w2 << 16, w2 & U32(0xFFFF0000))]
        for op, w in _right(*blocks).items():
            w_ref[mat][pl.ds(pl.multiple_of((op - 1) * op_rows + dst, 8), 8), pl.ds(j % 2 * Dh, Dh)] = pack(w)

    def prep_out(c, t):
        j, r = divmod(t * 16, Dh)
        even, odd = (rawo_ref[c, pl.ds(j * UW + p * Dh + r, 16), :].astype(F32) for p in range(2))
        dst = c * 2 * Dh + t * 8
        for op, w in _right(even[:, :HD], even[:, HD:], odd[:, :HD], odd[:, HD:]).items():
            wo_ref[pl.ds(pl.multiple_of((op - 1) * op_rows + dst, 8), 8), :] = pack(w)

    def w_in(i, mat, g, r=0, rows=HD // 2):
        r = (i - 1) * op_rows + g * (HD // 2) + r
        return pltpu.bitcast(w_ref[mat][pl.ds(r if isinstance(r, int) else pl.multiple_of(r, 8), rows), :], BF16)

    def token_left(halves, t0):
        def block(r):
            t = n_ref[pl.ds(pl.multiple_of(t0 + r * R, 8), R), :]
            return t[:, :HD], t[:, HD:]

        used = "".join(halves.values())
        blocks = {h: block(r) + block(r + 1) for h, r in (("x", 0), ("y", 2)) if h in used}
        return {i: [_left(i, *blocks[h]) for h in hs] for i, hs in halves.items()}

    def split(hs, prod):
        return {h: prod[t * R:(t + 1) * R] for t, h in enumerate(hs)}

    def in_tokens(ops, mat, g, m, it):
        if ops == SET_A:
            if "x" in m[7]:
                px_ref[0, mat, g] = m[1]["x"] - m[5]["x"] + m[7]["x"]
                px_ref[1, mat, g] = m[3]["x"] + m[5]["x"]
                px_ref[2, mat, g] = m[1]["x"] + m[3]["x"]
            if "y" in m[7]:
                px_ref[3, mat, g] = m[7]["y"]
            return None if it is None else (left_ref[0, mat, g], left_ref[1, mat, g])
        if ops == SET_B:
            even = _rows(px_ref[0, mat, g] + m[4]["x"], m[2]["x"] + m[4]["x"])
            odd = _rows(px_ref[1, mat, g], px_ref[2, mat, g] - m[2]["x"] + m[6]["x"])
            if "y" in m[6]:
                m6, m7 = m[6]["y"], px_ref[3, mat, g]
            else:
                m6, m7 = (pltpu.bitcast(w_ref[mat + 1][ahead_rows(k, g, it * R), :], F32) for k in range(2))
            py_ref[0, mat, g] = m7 + m[1]["y"]
            py_ref[1, mat, g] = m[1]["y"] + m6
            left_ref[0, mat, g, :2 * R - seg] = even[seg:]
            left_ref[1, mat, g, :2 * R - seg] = odd[seg:]
            return even[:seg], odd[:seg]
        even = _rows(left_ref[0, mat, g, :2 * R - seg],
                     py_ref[0, mat, g] + m[4]["y"] - m[5]["y"], m[2]["y"] + m[4]["y"])
        odd = _rows(left_ref[1, mat, g, :2 * R - seg],
                    m[3]["y"] + m[5]["y"], py_ref[1, mat, g] - m[2]["y"] + m[3]["y"])
        left_ref[0, mat, g] = even[seg:]
        left_ref[1, mat, g] = odd[seg:]
        return even[:seg], odd[:seg]

    def first_products(g):
        tl = token_left({i: "x" for i in SET_A}, seg)
        for mat in (K, Q, V):
            in_tokens(SET_A, mat, g, {i: {"x": _dot(tl[i][0], w_in(i, mat, g))} for i in SET_A}, None)

    def stream(mat, c):
        w_copy(mat, c).wait()
        prep, n_prep = (prep_out, Dh // 4) if mat == O else (functools.partial(prep_in, mat), HD // 4)
        if mat == O:
            first_products(2 * c)
            first_products(2 * c + 1)
        for t in range(4):
            g, k = 2 * c + t // 2, t % 2
            if mat > K:
                prod = pltpu.bitcast(_dot(ly_ref[k], w_in(6 + k, mat - 1, g)), U32)
            for j in range(n_per):
                for i in range((t * n_per + j) * n_prep // (4 * n_per), (t * n_per + j + 1) * n_prep // (4 * n_per)):
                    prep(c, i)
                if mat > K:
                    w_ref[mat][ahead_rows(k, g, j * R), :] = prod[j * R:(j + 1) * R]

        @pl.when(c + DEPTH < n_oct)
        def _():
            w_copy(mat, jnp.minimum(c + DEPTH, n_oct - 1)).start()

    def stream_body(i, carry):
        for mat in (K, Q, V, O):
            pl.when(i % 4 == mat)(functools.partial(stream, mat, i // 4))
        return carry

    lax.fori_loop(0, 4 * n_oct, stream_body, 0)
    for cp in rest_copies + ffn_copies:
        cp.start()

    def attend(ops, halves, t0, it, direct, o_dst, o_row, tail, jobs=()):
        nd = direct[0].shape[0]
        dl = [_direct_left(ops, direct[t], direct[2 + t]) for t in range(2)]
        tl = token_left(halves, t0)
        tiles = {i: [_feed(*[x[:, t * LANES:(t + 1) * LANES] for x in tl[i]], dl[t][i]) for t in range(2)]
                 for i in ops}
        lhs = {i: _cols(*tiles[i]) for i in ops}
        qi = lax.broadcasted_iota(jnp.int32, (L, L), 0)
        ki = lax.broadcasted_iota(jnp.int32, (L, L), 1)
        visible = (qi >= seg) | (ki >= seg) | (qi >= ki)
        qkv, e, inv, o_mem = {}, {}, {}, {}

        def first_units(i, t):
            w = _cols(*[w_in(i, K, g, t * LANES // 2, LANES // 2) for g in range(2)])
            return _dot(tiles[i][t], w)

        early = {i: first_units(i, 0) for i in ops}
        early = {i: first_units(i, 1) + early[i] for i in ops}
        clock, due = [0], {}

        def tick():
            clock[0] += 1
            for job in due.pop(clock[0], ()):
                job()

        def later(rounds, job, g):
            due.setdefault(clock[0] + rounds, []).append(functools.partial(job, g))

        for rounds, job, arg in jobs:
            later(rounds, job, arg)

        def project(mat, g):
            prod = {}
            for i in ops:
                if mat == K and g < 2:
                    prod[i] = early[i][:, g * UW:(g + 1) * UW]
                else:
                    prod[i] = _dot(lhs[i], w_in(i, mat, g))
                    tick()
            pair = _direct_out(ops, {i: prod[i][-nd:] for i in ops})
            own = in_tokens(ops, mat, g, {i: split(halves[i], prod[i]) for i in ops}, it)
            if own is not None:
                pair = [_rows(t, d) for t, d in zip(own, pair)]
            for p, x in enumerate(pair):
                x = x if mat == Q else x.astype(BF16)
                for j in range(2):
                    qkv[mat, g, p, j] = x[:, j * Dh:(j + 1) * Dh]

        heads = [(p, j) for p in range(2) for j in range(2)]

        def scores(g):
            for p, j in heads:
                sc = lax.dot_general(qkv[Q, g, p, j], qkv[K, g, p, j], (((1,), (1,)), ((), ())),
                                     preferred_element_type=F32)
                sc = jnp.where(visible, sc * scale, -1e9)
                w = jnp.exp(sc - jnp.max(sc, axis=-1, keepdims=True))
                e[g, p, j] = w
                inv[g, p, j] = pl.reciprocal(jnp.sum(w, axis=-1, keepdims=True), approx=True)
            later(VALUES_AFTER[g], values, g)

        def values(g):
            for p, j in heads:
                o = _dot(e[g, p, j], qkv[V, g, p, j]) * inv[g, p, j]
                o_dst[p, o_row:o_row + seg, (2 * g + j) * Dh:(2 * g + j + 1) * Dh] = o[:seg]
                o_mem[p, 2 * g + j] = o[seg:]

        project(K, 0)
        project(K, 1)
        for g in range(G):
            project(Q, g)
            later(SCORES_AFTER[g], scores, g)
            project(V, g)
            if g + 2 < G:
                project(K, g + 2)
        return tail(o_mem, tick)

    def project_out(ops, with_tokens, direct, tick=lambda: None):
        n_k = hp // 4
        lhs, acc = {}, {}

        def run(n, kk):
            c = slice(kk * 4 * Dh, (kk + 1) * 4 * Dh)
            if kk not in lhs:
                dl = _direct_left(ops, *direct(kk))
                block = lambda r: (o_ref[0, r * R:(r + 1) * R, c], o_ref[1, r * R:(r + 1) * R, c])
                used = "".join(HALVES[ops].values()) if with_tokens else ""
                blocks = {h: block(r) + block(r + 1) for h, r in (("y", 0), ("x", 2)) if h in used}
                lhs[kk] = {i: _rows(dl[i], *[_left(i, *blocks[h]) for h in HALVES[ops][i] if h in used])
                           for i in ops}
            for i in ops:
                w = wo_ref[pl.ds((i - 1) * op_rows + kk * 2 * Dh, 2 * Dh), n * LANES:(n + 1) * LANES]
                t = _dot(lhs[kk][i], pltpu.bitcast(w, BF16))
                acc[i, n] = t + acc[i, n] if kk else t
                tick()

        for n, kk in OUT_ORDER:
            run(n, kk)
        prod = {i: _cols(*[acc[i, n] for n in range(HD // LANES)]) for i in ops}
        nd = direct(0)[0].shape[0]
        res = [_direct_out(ops, {i: acc[i, n][:nd] for i in ops}) for n in range(HD // LANES)]
        res = tuple(r[p] for p in range(2) for r in res)
        return res, {i: split(HALVES[ops][i], prod[i][nd:]) for i in ops} if with_tokens else None

    def mem_rows(o_mem):
        return lambda kk: tuple(_cols(*[o_mem[p, 4 * kk + t] for t in range(4)]) for p in range(2))

    def router(n):
        return _rnd(jnp.sum(n * _rows(*[wr_ref[...]] * (n.shape[0] // 8)), axis=-1, keepdims=True))

    def finish(row, a, best, more=True):
        rows = a.shape[0]
        src = pl.ds(pl.multiple_of(jnp.maximum(row, 0), 16), rows)
        rs = pl.ds(pl.multiple_of(jnp.where(row < 0, S, row), 16), rows)
        x1 = _rnd(xr_ref[src, :].astype(F32) + a)
        n1 = _layernorm(x1, True)
        x2 = _rnd(x1 + n1)
        xm_ref[rs, :] = x1.astype(BF16)
        xr_ref[rs, :] = x2.astype(BF16)
        n_ref[rs, :] = _layernorm(x2) if more else x2
        r = jnp.where(row < 0, -jnp.inf, jnp.broadcast_to(router(n1), (rows, LANES)))
        best_r, best_i = best
        sub = lax.broadcasted_iota(jnp.int32, (8, LANES), 0)
        for b in range(0, rows, 8):
            better = r[b:b + 8] > best_r
            best_r = jnp.where(better, r[b:b + 8], best_r)
            best_i = jnp.where(better, sub + (row + b), best_i)
        return best_r, best_i

    def riders(l, ops):
        return {i: hs[0] if l == 0 else hs for i, hs in HALVES[ops].items()}

    n_early = (n_seg - 7) * seg
    early_copy = pltpu.make_async_copy(xr_ref.at[pl.ds(0, n_early)], out_hbm.at[pl.ds(0, n_early)], sems.at[0])
    late_copy = pltpu.make_async_copy(xr_ref.at[pl.ds(n_early, S - n_early)],
                                      out_hbm.at[pl.ds(n_early, S - n_early)], sems.at[1])

    def period(l, it, carry):
        mem, best = carry
        if l == 1:
            pl.when(it == n_per - 1)(early_copy.start)
        t0 = seg + it * P
        t1 = jnp.where(it == n_per - 1, seg, t0 + P)
        o_ref[:, :seg, :] = onext_ref[...]
        m, best = {}, [best]

        def finish_rows(r):
            best[0] = finish((it - 1) * P + r, a_ref[r:r + P // len(FINISH_STEP[l]), :], best[0], l == 0)

        def normalize_rows(_):
            rs = pl.ds(pl.multiple_of(jnp.where(it < n_per - 2, t0 + 2 * P, seg), seg), 2 * R)
            n_ref[rs, :] = _layernorm(xr_ref[rs, :].astype(F32))

        for u, (ops_in, t, ops_out, dst, row) in enumerate(((SET_B, t0, SET_C, o_ref, seg),
                                                           (SET_C, t0, SET_B, o_ref, 2 * seg),
                                                           (SET_A, t1, SET_A, onext_ref, 0))):
            jobs = [(1, normalize_rows, 0)] if l == 0 and u == REST_STEP else []
            jobs += [(88, finish_rows, b * P // len(FINISH_STEP[l])) for b, v in enumerate(FINISH_STEP[l]) if v == u]
            mem, prods = attend(
                ops_in, riders(l, ops_in), t, it, mem, dst, row,
                lambda o_mem, tick: project_out(ops_out, True, mem_rows(o_mem), tick), jobs)
            for i in ops_out:
                for h, x in prods[i].items():
                    m[i, h] = x
        for t, h in enumerate("yx"):
            top = _cols(m[1, h] + m[4, h] - m[5, h] + m[7, h], m[3, h] + m[5, h])
            bottom = _cols(m[2, h] + m[4, h], m[1, h] - m[2, h] + m[3, h] + m[6, h])
            a_ref[2 * t * R:2 * (t + 1) * R, :] = _rnd(_rows(top, bottom))
        return mem, best[0]

    def layer(l, routed):
        @pl.when((routed >= seg) & (routed < seg + 2 * R))
        def _():
            pl.loop(0, G)(first_products)

        mem = attend(SET_A, {i: hs[1:] for i, hs in HALVES[SET_A].items()}, seg, None,
                     jnp.split(_rows(n_ref[:seg, :], mem0_ref[...].astype(F32)), D // LANES, axis=1), onext_ref, 0,
                     lambda o_mem, tick: project_out(SET_C, False, mem_rows(o_mem), tick)[0])

        @pl.when(l == 0)
        def _():
            for cp in rest_copies:
                cp.wait()

        best = (jnp.full((8, LANES), -jnp.inf, F32), lax.broadcasted_iota(jnp.int32, (8, LANES), 0))
        carry = lax.fori_loop(0, (1 - l) * n_per, functools.partial(period, 0), (mem, best))
        _, best = lax.fori_loop(0, l * n_per, functools.partial(period, 1), carry)

        @pl.when(l == 0)
        def _():
            for cp in ffn_copies:
                cp.wait()

        last, _ = project_out(SET_C, False, lambda kk: tuple(
            onext_ref[p, :, kk * 4 * Dh:(kk + 1) * 4 * Dh] for p in range(2)))
        best = finish(S - seg - P, a_ref[...], best)
        best_r, best_i = finish(S - seg, _rnd(_cols(*last)), best)
        pl.when(l == 1)(late_copy.start)

        top = jnp.max(best_r, axis=0, keepdims=True)
        idx = jnp.min(jnp.where(best_r == top, best_i, S - 1))
        base = pl.multiple_of(jnp.clip(idx // 16 * 16, 0, S - 16), 16)
        rs = pl.ds(base, 16)
        x1 = xm_ref[rs, :].astype(F32)
        n1 = _layernorm(x1, True)
        nb = n1.astype(BF16)
        gate = _rnd(_dot(nb, wg_ref[...]))
        gate = _rnd(gate * jax.nn.sigmoid(gate))
        up = _rnd(_dot(nb, wu_ref[...]))
        y = _rnd(_dot((gate * up).astype(BF16), wd_ref[...]))
        y = _rnd(y * _rnd(jax.nn.sigmoid(router(n1))))
        chosen = lax.broadcasted_iota(jnp.int32, (16, D), 0) == idx - base
        x2 = _rnd(x1 + _rnd(n1 + jnp.where(chosen, y, 0.0)))
        patch_ref[...] = x2.astype(BF16)

        @pl.when(l == 0)
        def _():
            xr_ref[rs, :] = x2.astype(BF16)
            n_ref[rs, :] = _layernorm(x2)

        return idx

    routed = lax.fori_loop(0, 2, layer, jnp.int32(0))
    early_copy.wait()
    late_copy.wait()
    base = pl.multiple_of(jnp.clip(routed // 16 * 16, 0, S - 16), 16)
    patch_copy = pltpu.make_async_copy(patch_ref, out_hbm.at[pl.ds(base, 16)], sems.at[0])
    patch_copy.start()
    patch_copy.wait()


@functools.partial(jax.jit, static_argnames=("A_seg_len",))
def pallas_interleave_layers__memory_aug_recurrent_mem_tr__moe_arch_mod__prompt_kernel(
    A_x, A_mem0, A_Wq, A_Wk, A_Wv, A_Wo, A_seg_len, B_x, B_w_r, B_w_gate, B_w_up, B_w_down,
):
    del B_x
    B, S, D = A_x.shape
    _, H, Dh = A_Wq.shape
    M = A_mem0.shape[1]
    F = B_w_gate.shape[1]
    seg = int(A_seg_len)
    assert B == 1 and Dh == LANES and D == 4 * LANES and H % 8 == 0 and M % 8 == 0
    assert seg % 32 == 0 and S % seg == 0 and (S // seg) % 9 == 1 and S // seg > 7
    half = H * Dh // 2
    R = 3 * seg // 4
    hbm = pl.BlockSpec(memory_space=pl.ANY)

    def octets(w):
        return w.reshape(D, H // 8, 8, Dh).transpose(0, 2, 1, 3).reshape(8 * D, H // 8 * Dh)

    out = pl.pallas_call(
        functools.partial(_kernel, seg=seg, n_heads=H),
        out_shape=jax.ShapeDtypeStruct((S, D), A_x.dtype),
        in_specs=[hbm] * 10,
        out_specs=hbm,
        scratch_shapes=[
            pltpu.VMEM((3, H // 8, 8 * D + 16, Dh), BF16),
            pltpu.VMEM((H // 8, 8 * Dh, D), BF16),
            pltpu.VMEM((7 * half // 2, UW), U32),
            *[pltpu.VMEM((7 * half // 2 + H // 2 * (S - seg) // 4, UW), U32)] * 3,
            pltpu.VMEM((D, F), BF16),
            pltpu.VMEM((D, F), BF16),
            pltpu.VMEM((F, D), BF16),
            pltpu.VMEM((S + 3 * seg, D), BF16),
            pltpu.VMEM((S + 3 * seg, D), BF16),
            pltpu.VMEM((S + 3 * seg, D), F32),
            pltpu.VMEM((2, (S - seg) // 4, D // 2), F32),
            pltpu.VMEM((4, 3, H // 4, R, UW), F32),
            pltpu.VMEM((2, 3, H // 4, R, UW), F32),
            pltpu.VMEM((2, 3, H // 4, seg, UW), F32),
            pltpu.VMEM((2, 3 * seg, half), F32),
            pltpu.VMEM((2, seg, half), F32),
            pltpu.VMEM((3 * seg, D), F32),
            pltpu.VMEM((16, D), BF16),
            pltpu.VMEM((M, D), BF16),
            pltpu.VMEM((D,), BF16),
            pltpu.VMEM((8, D), F32),
            pltpu.SemaphoreType.DMA((9 + H // 2,)),
        ],
        compiler_params=pltpu.CompilerParams(vmem_limit_bytes=110 * 1024 * 1024),
        name="rmt_mod",
    )(A_x.reshape(S, D), A_mem0.reshape(M, D), octets(A_Wq), octets(A_Wk),
      octets(A_Wv), A_Wo.reshape(H * Dh, D), B_w_r, B_w_gate, B_w_up, B_w_down)
    return out.reshape(B, S, D)
```

```python
import functools

import jax
import jax.numpy as jnp
from jax import lax
import jax.experimental.pallas as pl
import jax.experimental.pallas.tpu as pltpu

F32 = jnp.float32
BF16 = jnp.bfloat16
U32 = jnp.uint32
LANES = 128
FINISH_STEP = ((0, 1, 2), (0, 0, 1, 1, 2, 2))
REST_STEP = 2
SCORES_AFTER = (7, 7, 7, 7, 7, 7, 7, 11)
VALUES_AFTER = (8, 8, 8, 8, 8, 8, 8, 8)
OUT_ORDER = ((0, 0), (1, 0), (0, 1), (1, 1), (0, 2), (1, 2), (0, 3), (1, 3))
UW = 2 * LANES
EPS_BF16 = 1.0013580322265625e-05
K, Q, V, O = 0, 1, 2, 3


def _rnd(x):
    return x.astype(BF16).astype(F32)


def _layernorm(x, stepwise=False):
    inv_d = 1.0 / x.shape[-1]
    m = jnp.sum(x, axis=-1, keepdims=True) * inv_d
    c = x - m
    v = jnp.sum(c * c, axis=-1, keepdims=True) * inv_d
    if not stepwise:
        return c * lax.rsqrt(v + 1e-5)
    sd = _rnd(jnp.sqrt(_rnd(_rnd(v) + EPS_BF16)))
    return _rnd(_rnd(x - _rnd(m)) / sd)


def _aligned(i, n):
    return i if isinstance(i, int) else pl.multiple_of(i, n)


def _dot(a, b):
    return jnp.dot(a, b, preferred_element_type=F32)


def _rows(*xs):
    return xs[0] if len(xs) == 1 else jnp.concatenate(xs, axis=0)


def _feed(*xs):
    x = _rows(*xs)
    return x if x.shape[0] % 16 else x.astype(BF16)


def _cols(*xs):
    return jnp.concatenate(xs, axis=1)


def _right(b11, b12, b21, b22):
    return {1: b11 + b22, 2: b11, 3: b12 - b22, 4: b21 - b11, 5: b22, 6: b11 + b12, 7: b21 + b22}


def _left(i, a11, a12, a21, a22):
    return {1: lambda: a11 + a22, 2: lambda: a21 + a22, 3: lambda: a11, 4: lambda: a22,
            5: lambda: a11 + a12, 6: lambda: a21 - a11, 7: lambda: a12 - a22}[i]()


SET_A, SET_B, SET_C = (1, 3, 5, 7), (1, 2, 4, 6), (2, 3, 4, 5)
HALVES = {SET_A: {1: "x", 3: "x", 5: "x", 7: "xy"},
          SET_B: {1: "y", 2: "x", 4: "x", 6: "xy"},
          SET_C: {2: "y", 3: "y", 4: "y", 5: "y"}}


def _direct_left(ops, a1, a2):
    both = a1 + a2
    return {1: a1 if ops == SET_A else a2, 2: both, 3: a1, 4: a2, 5: both, 6: a1, 7: a2}


def _direct_out(ops, p):
    c1 = p[1] - p[5] + p[7] if ops == SET_A else p[2] + p[4]
    c2 = p[1] - p[2] + p[6] if ops == SET_B else p[3] + p[5]
    return c1, c2


def _kernel(x_hbm, mem0_hbm, wq_hbm, wk_hbm, wv_hbm, wo_hbm, wr_hbm, wg_hbm, wu_hbm, wd_hbm,
            out_hbm,
            raw_ref, rawo_ref, wk_ref, wq_ref, wv_ref, wo_ref, wg_ref, wu_ref, wd_ref,
            xr_ref, xm_ref, n_ref, ly_ref, px_ref, py_ref, left_ref, o_ref, onext_ref, a_ref,
            patch_ref, mem0_ref, wr1_ref, wr_ref, sems,
            *, seg, n_heads):
    S, D = x_hbm.shape
    M = mem0_ref.shape[0]
    Dh = LANES
    n_seg = S // seg
    L = M + seg
    G = n_heads // 4
    HD = D // 2
    P = 3 * seg
    R = P // 4
    n_per = (n_seg - 1) // 3
    scale = Dh ** -0.5

    hp = n_heads // 2

    w_hbm = {Q: wq_hbm, K: wk_hbm, V: wv_hbm}
    w_ref = {Q: wq_ref, K: wk_ref, V: wv_ref, O: wo_ref}
    op_rows = G * HD // 2

    def ahead(mat, k, g, r):
        ref, slot = (w_ref[mat + 1], k) if mat < V else ((wk_ref, wo_ref)[k], 0)
        return ref, pl.ds(pl.multiple_of(7 * op_rows + (slot * G + g) * n_per * R + r, 8), R)

    n_oct = n_heads // 8

    def w_copy(mat, c):
        sem = sems.at[9 + 4 * c + mat]
        if mat == O:
            return pltpu.make_async_copy(wo_hbm.at[pl.ds(c * 8 * Dh, 8 * Dh)], rawo_ref.at[c], sem)
        col = c * Dh if isinstance(c, int) else pl.multiple_of(c * Dh, Dh)
        return pltpu.make_async_copy(w_hbm[mat].at[:, pl.ds(col, Dh)], raw_ref.at[mat, c, pl.ds(0, 8 * D)], sem)

    def x_copy(row, rows, sem):
        rs = pl.ds(row if isinstance(row, int) else pl.multiple_of(row, 16), rows)
        return pltpu.make_async_copy(x_hbm.at[rs], xr_ref.at[rs], sems.at[sem])

    n_ln = n_per // 3
    y_copy = lambda j, group: x_copy(seg + j * P + 2 * R, 2 * R, 6 + group)
    rest_copies = [x_copy(seg + j * P, 2 * R, 0) for j in range(2, n_per)]
    ffn_copies = [pltpu.make_async_copy(src, dst, sems.at[1 + i])
                  for i, (src, dst) in enumerate(((wg_hbm, wg_ref), (wu_hbm, wu_ref), (wd_hbm, wd_ref)))]
    first_copies = [x_copy(0, seg + 2 * R, 0), x_copy(seg + P, 2 * R, 1),
                    pltpu.make_async_copy(mem0_hbm, mem0_ref, sems.at[4]),
                    pltpu.make_async_copy(wr_hbm, wr1_ref, sems.at[5])]
    for cp in first_copies:
        cp.start()
    for j in range(n_per):
        y_copy(j, j // n_ln).start()
    def arriving(mat, c):
        return [(mat, c)] if mat < O else [(K, c + 1), (O, c - 1)]

    w_copy(K, 0).start()
    for c in range(2):
        for mat in (Q, V, O):
            for chunk in arriving(mat, c):
                if chunk[1] >= 0:
                    w_copy(*chunk).start()

    a_ref[...] = jnp.zeros_like(a_ref)
    rawo_ref[n_oct] = jnp.zeros(rawo_ref.shape[1:], BF16)
    for cp in first_copies:
        cp.wait()
    wr_ref[...] = jnp.broadcast_to(wr1_ref[...].astype(F32).reshape(1, D), wr_ref.shape)
    for rs in (pl.ds(0, seg + 2 * R), pl.ds(seg + P, 2 * R)):
        n_ref[rs, :] = _layernorm(xr_ref[rs, :].astype(F32))

    def ln_body(group, carry):
        for u in range(n_ln):
            y_copy(group * n_ln + u, group).wait()
        for j in [group * n_ln + u for u in range(n_ln)]:
            rs = pl.ds(pl.multiple_of(seg + j * P + 2 * R, 16), 2 * R)
            n = _layernorm(xr_ref[rs, :].astype(F32))
            n_ref[rs, :] = n
            for t, i in enumerate((6, 7)):
                ly_ref[t, pl.ds(pl.multiple_of(j * R, 8), R), :] = _left(
                    i, n[:R, :HD], n[:R, HD:], n[R:, :HD], n[R:, HD:])
        return carry

    lax.fori_loop(0, 3, ln_body, 0)

    def pack(x):
        return pltpu.bitcast(x.astype(BF16), U32)

    raw32 = raw_ref.bitcast(U32)

    def prep_in(mat, c, t):
        b, j = divmod(t, 4)
        dst = (2 * c + j // 2) * (HD // 2) + b * 8
        w1, w2 = (raw32.at[mat, c][pl.ds((half * HD + b * 16) * 4 + j, 16, stride=4), :] for half in range(2))
        blocks = [pltpu.bitcast(w, F32) for w in (w1 << 16, w1 & U32(0xFFFF0000), w2 << 16, w2 & U32(0xFFFF0000))]
        for op, w in _right(*blocks).items():
            w_ref[mat][pl.ds(_aligned((op - 1) * op_rows + dst, 8), 8), pl.ds(j % 2 * Dh, Dh)] = pack(w)

    def prep_out(src, c, t):
        j, r = divmod(t * 16, Dh)
        even, odd = (rawo_ref[src, pl.ds(j * UW + p * Dh + r, 16), :].astype(F32) for p in range(2))
        dst = c * 2 * Dh + t * 8
        for op, w in _right(even[:, :HD], even[:, HD:], odd[:, :HD], odd[:, HD:]).items():
            wo_ref[pl.ds(_aligned((op - 1) * op_rows + dst, 8), 8), :] = pack(w)

    def w_in(i, mat, g, r=0, rows=HD // 2):
        r = (i - 1) * op_rows + g * (HD // 2) + r
        return pltpu.bitcast(w_ref[mat][pl.ds(r if isinstance(r, int) else pl.multiple_of(r, 8), rows), :], BF16)

    def token_left(halves, t0):
        def block(r):
            t = n_ref[pl.ds(pl.multiple_of(t0 + r * R, 8), R), :]
            return t[:, :HD], t[:, HD:]

        used = "".join(halves.values())
        blocks = {h: block(r) + block(r + 1) for h, r in (("x", 0), ("y", 2)) if h in used}
        return {i: [_left(i, *blocks[h]) for h in hs] for i, hs in halves.items()}

    def split(hs, prod):
        return {h: prod[t * R:(t + 1) * R] for t, h in enumerate(hs)}

    def in_tokens(ops, mat, g, m, it):
        if ops == SET_A:
            if "x" in m[7]:
                px_ref[0, mat, g] = m[1]["x"] - m[5]["x"] + m[7]["x"]
                px_ref[1, mat, g] = m[3]["x"] + m[5]["x"]
                px_ref[2, mat, g] = m[1]["x"] + m[3]["x"]
            if "y" in m[7]:
                px_ref[3, mat, g] = m[7]["y"]
            return None if it is None else (left_ref[0, mat, g], left_ref[1, mat, g])
        if ops == SET_B:
            even = _rows(px_ref[0, mat, g] + m[4]["x"], m[2]["x"] + m[4]["x"])
            odd = _rows(px_ref[1, mat, g], px_ref[2, mat, g] - m[2]["x"] + m[6]["x"])
            if "y" in m[6]:
                m6, m7 = m[6]["y"], px_ref[3, mat, g]
            else:
                m6, m7 = (pltpu.bitcast(ref[rs, :], F32) for ref, rs in (ahead(mat, k, g, it * R) for k in range(2)))
            py_ref[0, mat, g] = m7 + m[1]["y"]
            py_ref[1, mat, g] = m[1]["y"] + m6
            left_ref[0, mat, g, :2 * R - seg] = even[seg:]
            left_ref[1, mat, g, :2 * R - seg] = odd[seg:]
            return even[:seg], odd[:seg]
        even = _rows(left_ref[0, mat, g, :2 * R - seg],
                     py_ref[0, mat, g] + m[4]["y"] - m[5]["y"], m[2]["y"] + m[4]["y"])
        odd = _rows(left_ref[1, mat, g, :2 * R - seg],
                    m[3]["y"] + m[5]["y"], py_ref[1, mat, g] - m[2]["y"] + m[3]["y"])
        left_ref[0, mat, g] = even[seg:]
        left_ref[1, mat, g] = odd[seg:]
        return even[:seg], odd[:seg]

    def first_products(g):
        tl = token_left({i: "x" for i in SET_A}, seg)
        for mat in (K, Q, V):
            in_tokens(SET_A, mat, g, {i: {"x": _dot(tl[i][0], w_in(i, mat, g))} for i in SET_A}, None)

    in_jobs = lambda mat, c: [functools.partial(prep_in, mat, c, t) for t in range(HD // 4)]
    out_jobs = lambda src, c: [functools.partial(prep_out, src, c, t) for t in range(Dh // 4)]

    def for_chunks(mat, c, action):
        for m, i in arriving(mat, c):
            pl.when((i >= 0) & (i < n_oct))(lambda: action(w_copy(m, jnp.clip(i, 0, n_oct - 1))))

    def stream(mat, c):
        for_chunks(mat, c, lambda cp: cp.wait())
        if mat < O:
            jobs = in_jobs(mat, c)
            jobs = jobs[:len(jobs) // 2], jobs[len(jobs) // 2:]
        else:
            first_products(2 * c)
            first_products(2 * c + 1)
            jobs = (in_jobs(K, jnp.minimum(c + 1, n_oct - 1)),
                    out_jobs(jnp.where(c == 0, n_oct, c - 1), jnp.maximum(c - 1, 0)))
        for k in range(2):
            for u in range(2):
                prod = pltpu.bitcast(_dot(ly_ref[k], w_in(6 + k, mat - 1, 2 * c + u)), U32)
                for j in range(n_per):
                    i, n = u * n_per + j, len(jobs[k])
                    for job in jobs[k][i * n // (2 * n_per):(i + 1) * n // (2 * n_per)]:
                        job()
                    ref, rs = ahead(mat - 1, k, 2 * c + u, j * R)
                    ref[rs, :] = prod[j * R:(j + 1) * R]
        for_chunks(mat, c + 2, lambda cp: cp.start())

    def stream_body(i, carry):
        for mat in (Q, V, O):
            pl.when(i % 3 == mat - 1)(functools.partial(stream, mat, i // 3))
        return carry

    w_copy(K, 0).wait()
    for job in in_jobs(K, 0):
        job()
    lax.fori_loop(0, 3 * n_oct, stream_body, 0)
    for cp in rest_copies + ffn_copies:
        cp.start()
    w_copy(O, n_oct - 1).wait()
    for job in out_jobs(n_oct - 1, n_oct - 1):
        job()

    def attend(ops, halves, t0, it, direct, o_dst, o_row, tail, jobs=()):
        nd = direct[0].shape[0]
        dl = [_direct_left(ops, direct[t], direct[2 + t]) for t in range(2)]
        tl = token_left(halves, t0)
        tiles = {i: [_feed(*[x[:, t * LANES:(t + 1) * LANES] for x in tl[i]], dl[t][i]) for t in range(2)]
                 for i in ops}
        lhs = {i: _cols(*tiles[i]) for i in ops}
        qi = lax.broadcasted_iota(jnp.int32, (L, L), 0)
        ki = lax.broadcasted_iota(jnp.int32, (L, L), 1)
        visible = (qi >= seg) | (ki >= seg) | (qi >= ki)
        qkv, e, inv, o_mem = {}, {}, {}, {}

        def first_units(i, t):
            w = _cols(*[w_in(i, K, g, t * LANES // 2, LANES // 2) for g in range(2)])
            return _dot(tiles[i][t], w)

        early = {i: first_units(i, 0) for i in ops}
        early = {i: first_units(i, 1) + early[i] for i in ops}
        clock, due = [0], {}

        def tick():
            clock[0] += 1
            for job in due.pop(clock[0], ()):
                job()

        def later(rounds, job, g):
            due.setdefault(clock[0] + rounds, []).append(functools.partial(job, g))

        for rounds, job, arg in jobs:
            later(rounds, job, arg)

        def project(mat, g):
            prod = {}
            for i in ops:
                if mat == K and g < 2:
                    prod[i] = early[i][:, g * UW:(g + 1) * UW]
                else:
                    prod[i] = _dot(lhs[i], w_in(i, mat, g))
                    tick()
            pair = _direct_out(ops, {i: prod[i][-nd:] for i in ops})
            own = in_tokens(ops, mat, g, {i: split(halves[i], prod[i]) for i in ops}, it)
            if own is not None:
                pair = [_rows(t, d) for t, d in zip(own, pair)]
            for p, x in enumerate(pair):
                x = x if mat == Q else x.astype(BF16)
                for j in range(2):
                    qkv[mat, g, p, j] = x[:, j * Dh:(j + 1) * Dh]

        heads = [(p, j) for p in range(2) for j in range(2)]

        def scores(g):
            for p, j in heads:
                sc = lax.dot_general(qkv[Q, g, p, j], qkv[K, g, p, j], (((1,), (1,)), ((), ())),
                                     preferred_element_type=F32)
                sc = jnp.where(visible, sc * scale, -1e9)
                w = jnp.exp(sc - jnp.max(sc, axis=-1, keepdims=True))
                e[g, p, j] = w
                inv[g, p, j] = pl.reciprocal(jnp.sum(w, axis=-1, keepdims=True), approx=True)
            later(VALUES_AFTER[g], values, g)

        def values(g):
            for p, j in heads:
                o = _dot(e[g, p, j], qkv[V, g, p, j]) * inv[g, p, j]
                o_dst[p, o_row:o_row + seg, (2 * g + j) * Dh:(2 * g + j + 1) * Dh] = o[:seg]
                o_mem[p, 2 * g + j] = o[seg:]

        project(K, 0)
        project(K, 1)
        for g in range(G):
            project(Q, g)
            later(SCORES_AFTER[g], scores, g)
            project(V, g)
            if g + 2 < G:
                project(K, g + 2)
        return tail(o_mem, tick)

    def project_out(ops, with_tokens, direct, tick=lambda: None):
        n_k = hp // 4
        lhs, acc = {}, {}

        def run(n, kk):
            c = slice(kk * 4 * Dh, (kk + 1) * 4 * Dh)
            if kk not in lhs:
                dl = _direct_left(ops, *direct(kk))
                block = lambda r: (o_ref[0, r * R:(r + 1) * R, c], o_ref[1, r * R:(r + 1) * R, c])
                used = "".join(HALVES[ops].values()) if with_tokens else ""
                blocks = {h: block(r) + block(r + 1) for h, r in (("y", 0), ("x", 2)) if h in used}
                lhs[kk] = {i: _rows(dl[i], *[_left(i, *blocks[h]) for h in HALVES[ops][i] if h in used])
                           for i in ops}
            for i in ops:
                w = wo_ref[pl.ds((i - 1) * op_rows + kk * 2 * Dh, 2 * Dh), n * LANES:(n + 1) * LANES]
                t = _dot(lhs[kk][i], pltpu.bitcast(w, BF16))
                acc[i, n] = t + acc[i, n] if kk else t
                tick()

        for n, kk in OUT_ORDER:
            run(n, kk)
        prod = {i: _cols(*[acc[i, n] for n in range(HD // LANES)]) for i in ops}
        nd = direct(0)[0].shape[0]
        res = [_direct_out(ops, {i: acc[i, n][:nd] for i in ops}) for n in range(HD // LANES)]
        res = tuple(r[p] for p in range(2) for r in res)
        return res, {i: split(HALVES[ops][i], prod[i][nd:]) for i in ops} if with_tokens else None

    def mem_rows(o_mem):
        return lambda kk: tuple(_cols(*[o_mem[p, 4 * kk + t] for t in range(4)]) for p in range(2))

    def router(n):
        return _rnd(jnp.sum(n * _rows(*[wr_ref[...]] * (n.shape[0] // 8)), axis=-1, keepdims=True))

    def finish(row, a, best, more=True):
        rows = a.shape[0]
        src = pl.ds(pl.multiple_of(jnp.maximum(row, 0), 16), rows)
        rs = pl.ds(pl.multiple_of(jnp.where(row < 0, S, row), 16), rows)
        x1 = _rnd(xr_ref[src, :].astype(F32) + a)
        n1 = _layernorm(x1, True)
        x2 = _rnd(x1 + n1)
        xm_ref[0, rs, :] = x1.astype(BF16)
        xm_ref[1, rs, :] = n1.astype(BF16)
        xr_ref[rs, :] = x2.astype(BF16)
        n_ref[rs, :] = _layernorm(x2) if more else x2
        r = jnp.where(row < 0, -jnp.inf, jnp.broadcast_to(router(n1), (rows, LANES)))
        best_r, best_i = best
        sub = lax.broadcasted_iota(jnp.int32, (8, LANES), 0)
        for b in range(0, rows, 8):
            better = r[b:b + 8] > best_r
            best_r = jnp.where(better, r[b:b + 8], best_r)
            best_i = jnp.where(better, sub + (row + b), best_i)
        return best_r, best_i

    def riders(l, ops):
        return {i: hs[0] if l == 0 else hs for i, hs in HALVES[ops].items()}

    n_early = (n_seg - 7) * seg
    early_copy = pltpu.make_async_copy(xr_ref.at[pl.ds(0, n_early)], out_hbm.at[pl.ds(0, n_early)], sems.at[0])
    late_copy = pltpu.make_async_copy(xr_ref.at[pl.ds(n_early, S - n_early)],
                                      out_hbm.at[pl.ds(n_early, S - n_early)], sems.at[1])

    def period(l, it, carry):
        mem, best = carry
        if l == 1:
            pl.when(it == n_per - 1)(early_copy.start)
        t0 = seg + it * P
        t1 = jnp.where(it == n_per - 1, seg, t0 + P)
        o_ref[:, :seg, :] = onext_ref[...]
        m, best = {}, [best]

        def finish_rows(r):
            best[0] = finish((it - 1) * P + r, a_ref[r:r + P // len(FINISH_STEP[l]), :], best[0], l == 0)

        def normalize_rows(_):
            rs = pl.ds(pl.multiple_of(jnp.where(it < n_per - 2, t0 + 2 * P, seg), seg), 2 * R)
            n_ref[rs, :] = _layernorm(xr_ref[rs, :].astype(F32))

        for u, (ops_in, t, ops_out, dst, row) in enumerate(((SET_B, t0, SET_C, o_ref, seg),
                                                           (SET_C, t0, SET_B, o_ref, 2 * seg),
                                                           (SET_A, t1, SET_A, onext_ref, 0))):
            jobs = [(1, normalize_rows, 0)] if l == 0 and u == REST_STEP else []
            jobs += [(88, finish_rows, b * P // len(FINISH_STEP[l])) for b, v in enumerate(FINISH_STEP[l]) if v == u]
            mem, prods = attend(
                ops_in, riders(l, ops_in), t, it, mem, dst, row,
                lambda o_mem, tick: project_out(ops_out, True, mem_rows(o_mem), tick), jobs)
            for i in ops_out:
                for h, x in prods[i].items():
                    m[i, h] = x
        for t, h in enumerate("yx"):
            top = _cols(m[1, h] + m[4, h] - m[5, h] + m[7, h], m[3, h] + m[5, h])
            bottom = _cols(m[2, h] + m[4, h], m[1, h] - m[2, h] + m[3, h] + m[6, h])
            a_ref[2 * t * R:2 * (t + 1) * R, :] = _rnd(_rows(top, bottom))
        return mem, best[0]

    def arg_max(best):
        best_r, best_i = best
        top = jnp.max(best_r, axis=0, keepdims=True)
        return jnp.min(jnp.where(best_r == top, best_i, S - 1)), top

    def patch_rows(idx):
        return pl.ds(pl.multiple_of(jnp.clip(idx // 16 * 16, 0, S - 16), 16), 16)

    def feed_forward(idx, top):
        rs = patch_rows(idx)
        n1 = xm_ref[1, rs, :]
        gate = _rnd(_dot(n1, wg_ref[...]))
        gate = _rnd(gate * jax.nn.sigmoid(gate))
        up = _rnd(_dot(n1, wu_ref[...]))
        y = _rnd(_dot((gate * up).astype(BF16), wd_ref[...]))
        y = _rnd(y * _cols(*[_rnd(jax.nn.sigmoid(top))] * (D // LANES)))
        chosen = lax.broadcasted_iota(jnp.int32, (16, D), 0) == idx - rs.start
        update = _rnd(n1.astype(F32) + jnp.where(chosen, y, 0.0))
        patch_ref[...] = (xm_ref[0, rs, :].astype(F32) + update).astype(BF16)

    def layer(l, routed):
        @pl.when((routed >= seg) & (routed < seg + 2 * R))
        def _():
            pl.loop(0, G)(first_products)

        mem = attend(SET_A, {i: hs[1:] for i, hs in HALVES[SET_A].items()}, seg, None,
                     jnp.split(_rows(n_ref[:seg, :], mem0_ref[...].astype(F32)), D // LANES, axis=1), onext_ref, 0,
                     lambda o_mem, tick: project_out(SET_C, False, mem_rows(o_mem), tick)[0])

        @pl.when(l == 0)
        def _():
            for cp in rest_copies:
                cp.wait()

        best = (jnp.full((8, LANES), -jnp.inf, F32), lax.broadcasted_iota(jnp.int32, (8, LANES), 0))
        carry = lax.fori_loop(0, (1 - l) * n_per, functools.partial(period, 0), (mem, best))
        _, best = lax.fori_loop(0, l * n_per, functools.partial(period, 1), carry)

        @pl.when(l == 0)
        def _():
            for cp in ffn_copies:
                cp.wait()

        last, _ = project_out(SET_C, False, lambda kk: tuple(
            onext_ref[p, :, kk * 4 * Dh:(kk + 1) * 4 * Dh] for p in range(2)))
        best = finish(S - seg - P, a_ref[...], best)
        leader = arg_max(best)
        feed_forward(*leader)
        winner = arg_max(finish(S - seg, _rnd(_cols(*last)), best))
        pl.when(l == 1)(late_copy.start)
        pl.when(winner[0] != leader[0])(lambda: feed_forward(*winner))

        @pl.when(l == 0)
        def _():
            xr_ref[patch_rows(winner[0]), :] = patch_ref[...]
            n_ref[patch_rows(winner[0]), :] = _layernorm(patch_ref[...].astype(F32))

        return winner[0]

    routed = lax.fori_loop(0, 2, layer, jnp.int32(0))
    early_copy.wait()
    late_copy.wait()
    patch_copy = pltpu.make_async_copy(patch_ref, out_hbm.at[patch_rows(routed)], sems.at[0])
    patch_copy.start()
    patch_copy.wait()


@functools.partial(jax.jit, static_argnames=("A_seg_len",))
def pallas_interleave_layers__memory_aug_recurrent_mem_tr__moe_arch_mod__prompt_kernel(
    A_x, A_mem0, A_Wq, A_Wk, A_Wv, A_Wo, A_seg_len, B_x, B_w_r, B_w_gate, B_w_up, B_w_down,
):
    del B_x
    B, S, D = A_x.shape
    _, H, Dh = A_Wq.shape
    M = A_mem0.shape[1]
    F = B_w_gate.shape[1]
    seg = int(A_seg_len)
    assert B == 1 and Dh == LANES and D == 4 * LANES and H % 8 == 0 and M % 8 == 0
    assert seg % 32 == 0 and S % seg == 0 and (S // seg) % 9 == 1 and S // seg > 7
    half = H * Dh // 2
    R = 3 * seg // 4
    hbm = pl.BlockSpec(memory_space=pl.ANY)

    def octets(w):
        return w.reshape(D, H // 8, 8, Dh).transpose(0, 2, 1, 3).reshape(8 * D, H // 8 * Dh)

    out = pl.pallas_call(
        functools.partial(_kernel, seg=seg, n_heads=H),
        out_shape=jax.ShapeDtypeStruct((S, D), A_x.dtype),
        in_specs=[hbm] * 10,
        out_specs=hbm,
        scratch_shapes=[
            pltpu.VMEM((3, H // 8, 8 * D + 16, Dh), BF16),
            pltpu.VMEM((H // 8 + 1, 8 * Dh, D), BF16),
            *[pltpu.VMEM((7 * half // 2 + n * H // 4 * (S - seg) // 4, UW), U32) for n in (1, 2, 2, 1)],
            pltpu.VMEM((D, F), BF16),
            pltpu.VMEM((D, F), BF16),
            pltpu.VMEM((F, D), BF16),
            pltpu.VMEM((S + 3 * seg, D), BF16),
            pltpu.VMEM((2, S + 3 * seg, D), BF16),
            pltpu.VMEM((S + 3 * seg, D), F32),
            pltpu.VMEM((2, (S - seg) // 4, D // 2), F32),
            pltpu.VMEM((4, 3, H // 4, R, UW), F32),
            pltpu.VMEM((2, 3, H // 4, R, UW), F32),
            pltpu.VMEM((2, 3, H // 4, seg, UW), F32),
            pltpu.VMEM((2, 3 * seg, half), F32),
            pltpu.VMEM((2, seg, half), F32),
            pltpu.VMEM((3 * seg, D), F32),
            pltpu.VMEM((16, D), BF16),
            pltpu.VMEM((M, D), BF16),
            pltpu.VMEM((D,), BF16),
            pltpu.VMEM((8, D), F32),
            pltpu.SemaphoreType.DMA((9 + H // 2,)),
        ],
        compiler_params=pltpu.CompilerParams(vmem_limit_bytes=110 * 1024 * 1024),
        name="rmt_mod",
    )(A_x.reshape(S, D), A_mem0.reshape(M, D), octets(A_Wq), octets(A_Wk),
      octets(A_Wv), A_Wo.reshape(H * Dh, D), B_w_r, B_w_gate, B_w_up, B_w_down)
    return out.reshape(B, S, D)
```

```python
import functools

import jax
import jax.numpy as jnp
from jax import lax
import jax.experimental.pallas as pl
import jax.experimental.pallas.tpu as pltpu

F32 = jnp.float32
BF16 = jnp.bfloat16
U32 = jnp.uint32
LANES = 128
FINISH_STEP = ((0, 1, 2), (0, 0, 1, 1, 2, 2))
REST_STEP = 2
SCORES_AFTER = (7, 7, 7, 7, 7, 7, 7, 11)
VALUES_AFTER = (8, 8, 8, 8, 8, 8, 8, 8)
OUT_ORDER = ((0, 0), (1, 0), (0, 1), (1, 1), (0, 2), (1, 2), (0, 3), (1, 3))
UW = 2 * LANES
EPS_BF16 = 1.0013580322265625e-05
K, Q, V, O = 0, 1, 2, 3


def _rnd(x):
    return x.astype(BF16).astype(F32)


def _layernorm(x, stepwise=False):
    inv_d = 1.0 / x.shape[-1]
    m = jnp.sum(x, axis=-1, keepdims=True) * inv_d
    c = x - m
    v = jnp.sum(c * c, axis=-1, keepdims=True) * inv_d
    if not stepwise:
        return c * lax.rsqrt(v + 1e-5)
    sd = _rnd(jnp.sqrt(_rnd(_rnd(v) + EPS_BF16)))
    return _rnd(_rnd(x - _rnd(m)) / sd)


def _aligned(i, n):
    return i if isinstance(i, int) else pl.multiple_of(i, n)


def _dot(a, b):
    return jnp.dot(a, b, preferred_element_type=F32)


def _rows(*xs):
    return xs[0] if len(xs) == 1 else jnp.concatenate(xs, axis=0)


def _feed(*xs):
    x = _rows(*xs)
    return x if x.shape[0] % 16 else x.astype(BF16)


def _cols(*xs):
    return jnp.concatenate(xs, axis=1)


def _right(b11, b12, b21, b22):
    return {1: b11 + b22, 2: b11, 3: b12 - b22, 4: b21 - b11, 5: b22, 6: b11 + b12, 7: b21 + b22}


def _left(i, a11, a12, a21, a22):
    return {1: lambda: a11 + a22, 2: lambda: a21 + a22, 3: lambda: a11, 4: lambda: a22,
            5: lambda: a11 + a12, 6: lambda: a21 - a11, 7: lambda: a12 - a22}[i]()


SET_A, SET_B, SET_C = (1, 3, 5, 7), (1, 2, 4, 6), (2, 3, 4, 5)
HALVES = {SET_A: {1: "x", 3: "x", 5: "x", 7: "xy"},
          SET_B: {1: "y", 2: "x", 4: "x", 6: "xy"},
          SET_C: {2: "y", 3: "y", 4: "y", 5: "y"}}


def _direct_left(ops, a1, a2):
    both = a1 + a2
    return {1: a1 if ops == SET_A else a2, 2: both, 3: a1, 4: a2, 5: both, 6: a1, 7: a2}


def _direct_out(ops, p):
    c1 = p[1] - p[5] + p[7] if ops == SET_A else p[2] + p[4]
    c2 = p[1] - p[2] + p[6] if ops == SET_B else p[3] + p[5]
    return c1, c2


def _kernel(x_hbm, mem0_hbm, wq_hbm, wk_hbm, wv_hbm, wo_hbm, wr_hbm, wg_hbm, wu_hbm, wd_hbm,
            out_hbm,
            raw_ref, words_ref, rawo_ref, wk_ref, wq_ref, wv_ref, wg_ref, wu_ref, wd_ref,
            xr_ref, xm_ref, n_ref, ly_ref, px_ref, py_ref, left_ref, o_ref, onext_ref, a_ref,
            patch_ref, mem0_ref, wr1_ref, wr_ref, sems,
            *, seg, n_heads):
    S, D = x_hbm.shape
    M = mem0_ref.shape[0]
    Dh = LANES
    n_seg = S // seg
    L = M + seg
    G = n_heads // 4
    HD = D // 2
    P = 3 * seg
    R = P // 4
    n_per = (n_seg - 1) // 3
    scale = Dh ** -0.5

    hp = n_heads // 2

    w_hbm = {Q: wq_hbm, K: wk_hbm, V: wv_hbm}
    w_ref = {Q: wq_ref, K: wk_ref, V: wv_ref}
    op_rows = G * HD // 2
    out_row = 7 * op_rows + 2 * G * n_per * R

    def ahead(mat, k, g, r):
        return w_ref[(mat + 1) % 3], pl.ds(pl.multiple_of(7 * op_rows + (k * G + g) * n_per * R + r, 8), R)

    n_oct = n_heads // 8

    def w_copy(mat, c):
        sem = sems.at[9 + 4 * c + mat]
        if mat == O:
            return pltpu.make_async_copy(wo_hbm.at[pl.ds(c * 8 * Dh, 8 * Dh)], rawo_ref.at[c], sem)
        col = c * Dh if isinstance(c, int) else pl.multiple_of(c * Dh, Dh)
        return pltpu.make_async_copy(w_hbm[mat].at[:, pl.ds(col, Dh)], raw_ref.at[mat, c], sem)

    def x_copy(row, rows, sem):
        rs = pl.ds(row if isinstance(row, int) else pl.multiple_of(row, 16), rows)
        return pltpu.make_async_copy(x_hbm.at[rs], xr_ref.at[rs], sems.at[sem])

    n_ln = n_per // 3
    y_copy = lambda j, group: x_copy(seg + j * P + 2 * R, 2 * R, 6 + group)
    rest_copies = [x_copy(seg + j * P, 2 * R, 0) for j in range(2, n_per)]
    ffn_copies = [pltpu.make_async_copy(src, dst, sems.at[1 + i])
                  for i, (src, dst) in enumerate(((wg_hbm, wg_ref), (wu_hbm, wu_ref), (wd_hbm, wd_ref)))]
    first_copies = [x_copy(0, seg + 2 * R, 0), x_copy(seg + P, 2 * R, 1),
                    pltpu.make_async_copy(mem0_hbm, mem0_ref, sems.at[4]),
                    pltpu.make_async_copy(wr_hbm, wr1_ref, sems.at[5])]
    for cp in first_copies:
        cp.start()
    for j in range(n_per):
        y_copy(j, j // n_ln).start()
    def arriving(mat, c):
        return [(mat, c)] if mat < O else [(K, c + 1), (O, c - 1)]

    w_copy(K, 0).start()
    for c in range(2):
        for mat in (Q, V, O):
            for chunk in arriving(mat, c):
                if chunk[1] >= 0:
                    w_copy(*chunk).start()

    a_ref[...] = jnp.zeros_like(a_ref)
    rawo_ref[n_oct] = jnp.zeros(rawo_ref.shape[1:], BF16)
    for cp in first_copies:
        cp.wait()
    wr_ref[...] = jnp.broadcast_to(wr1_ref[...].astype(F32).reshape(1, D), wr_ref.shape)
    for rs in (pl.ds(0, seg + 2 * R), pl.ds(seg + P, 2 * R)):
        n_ref[rs, :] = _layernorm(xr_ref[rs, :].astype(F32))

    def ln_body(group, carry):
        for u in range(n_ln):
            y_copy(group * n_ln + u, group).wait()
        for j in [group * n_ln + u for u in range(n_ln)]:
            rs = pl.ds(pl.multiple_of(seg + j * P + 2 * R, 16), 2 * R)
            n = _layernorm(xr_ref[rs, :].astype(F32))
            n_ref[rs, :] = n
            for t, i in enumerate((6, 7)):
                ly_ref[t, pl.ds(pl.multiple_of(j * R, 8), R), :] = _left(
                    i, n[:R, :HD], n[:R, HD:], n[R:, :HD], n[R:, HD:])
        return carry

    lax.fori_loop(0, 3, ln_body, 0)

    def pack(x):
        return pltpu.bitcast(x.astype(BF16), U32)

    def prep_in(mat, c, t):
        b, j = divmod(t, 4)
        dst = (2 * c + j // 2) * (HD // 2) + b * 8
        ds = [half * HD + b * 16 for half in range(2)]
        if j == 0:
            for d in ds:
                words_ref[pl.ds(4 * d, 64), :] = pltpu.bitcast(raw_ref[mat, c, pl.ds(8 * d, 128), :], U32)
        w1, w2 = (words_ref[pl.ds(4 * d + j, 16, stride=4), :] for d in ds)
        blocks = [pltpu.bitcast(w, F32) for w in (w1 << 16, w1 & U32(0xFFFF0000), w2 << 16, w2 & U32(0xFFFF0000))]
        for op, w in _right(*blocks).items():
            w_ref[mat][pl.ds(_aligned((op - 1) * op_rows + dst, 8), 8), pl.ds(j % 2 * Dh, Dh)] = pack(w)

    def prep_out(src, c, t):
        j, r = divmod(t * 16, Dh)
        even, odd = (rawo_ref[src, pl.ds(j * UW + p * Dh + r, 16), :].astype(F32) for p in range(2))
        dst = c * 2 * Dh + t * 8
        for op, w in _right(even[:, :HD], even[:, HD:], odd[:, :HD], odd[:, HD:]).items():
            wk_ref[pl.ds(_aligned(out_row + (op - 1) * op_rows + dst, 8), 8), :] = pack(w)

    def w_in(i, mat, g, r=0, rows=HD // 2):
        r = (i - 1) * op_rows + g * (HD // 2) + r
        return pltpu.bitcast(w_ref[mat][pl.ds(r if isinstance(r, int) else pl.multiple_of(r, 8), rows), :], BF16)

    def token_left(halves, t0):
        def block(r):
            t = n_ref[pl.ds(pl.multiple_of(t0 + r * R, 8), R), :]
            return t[:, :HD], t[:, HD:]

        used = "".join(halves.values())
        blocks = {h: block(r) + block(r + 1) for h, r in (("x", 0), ("y", 2)) if h in used}
        return {i: [_left(i, *blocks[h]) for h in hs] for i, hs in halves.items()}

    def split(hs, prod):
        return {h: prod[t * R:(t + 1) * R] for t, h in enumerate(hs)}

    def in_tokens(ops, mat, g, m, it):
        if ops == SET_A:
            if "x" in m[7]:
                px_ref[0, mat, g] = m[1]["x"] - m[5]["x"] + m[7]["x"]
                px_ref[1, mat, g] = m[3]["x"] + m[5]["x"]
                px_ref[2, mat, g] = m[1]["x"] + m[3]["x"]
            if "y" in m[7]:
                px_ref[3, mat, g] = m[7]["y"]
            return None if it is None else (left_ref[0, mat, g], left_ref[1, mat, g])
        if ops == SET_B:
            even = _rows(px_ref[0, mat, g] + m[4]["x"], m[2]["x"] + m[4]["x"])
            odd = _rows(px_ref[1, mat, g], px_ref[2, mat, g] - m[2]["x"] + m[6]["x"])
            if "y" in m[6]:
                m6, m7 = m[6]["y"], px_ref[3, mat, g]
            else:
                m6, m7 = (pltpu.bitcast(ref[rs, :], F32) for ref, rs in (ahead(mat, k, g, it * R) for k in range(2)))
            py_ref[0, mat, g] = m7 + m[1]["y"]
            py_ref[1, mat, g] = m[1]["y"] + m6
            left_ref[0, mat, g, :2 * R - seg] = even[seg:]
            left_ref[1, mat, g, :2 * R - seg] = odd[seg:]
            return even[:seg], odd[:seg]
        even = _rows(left_ref[0, mat, g, :2 * R - seg],
                     py_ref[0, mat, g] + m[4]["y"] - m[5]["y"], m[2]["y"] + m[4]["y"])
        odd = _rows(left_ref[1, mat, g, :2 * R - seg],
                    m[3]["y"] + m[5]["y"], py_ref[1, mat, g] - m[2]["y"] + m[3]["y"])
        left_ref[0, mat, g] = even[seg:]
        left_ref[1, mat, g] = odd[seg:]
        return even[:seg], odd[:seg]

    def first_products(g):
        tl = token_left({i: "x" for i in SET_A}, seg)
        for mat in (K, Q, V):
            in_tokens(SET_A, mat, g, {i: {"x": _dot(tl[i][0], w_in(i, mat, g))} for i in SET_A}, None)

    in_jobs = lambda mat, c: [functools.partial(prep_in, mat, c, t) for t in range(HD // 4)]
    out_jobs = lambda src, c: [functools.partial(prep_out, src, c, t) for t in range(Dh // 4)]

    def for_chunks(mat, c, action):
        for m, i in arriving(mat, c):
            pl.when((i >= 0) & (i < n_oct))(lambda: action(w_copy(m, jnp.clip(i, 0, n_oct - 1))))

    def stream(mat, c):
        for_chunks(mat, c, lambda cp: cp.wait())
        if mat < O:
            jobs = in_jobs(mat, c)
        else:
            first_products(2 * c)
            first_products(2 * c + 1)
            jobs = (in_jobs(K, jnp.minimum(c + 1, n_oct - 1))
                    + out_jobs(jnp.where(c == 0, n_oct, c - 1), jnp.maximum(c - 1, 0)))
        for k in range(2):
            for u in range(2):
                prod = pltpu.bitcast(_dot(ly_ref[k], w_in(6 + k, mat - 1, 2 * c + u)), U32)
                for j in range(n_per):
                    i = (2 * k + u) * n_per + j
                    for job in jobs[i * len(jobs) // (4 * n_per):(i + 1) * len(jobs) // (4 * n_per)]:
                        job()
                    ref, rs = ahead(mat - 1, k, 2 * c + u, j * R)
                    ref[rs, :] = prod[j * R:(j + 1) * R]
        for_chunks(mat, c + 2, lambda cp: cp.start())

    def stream_body(i, carry):
        for mat in (Q, V, O):
            pl.when(i % 3 == mat - 1)(functools.partial(stream, mat, i // 3))
        return carry

    w_copy(K, 0).wait()
    for job in in_jobs(K, 0):
        job()
    lax.fori_loop(0, 3 * n_oct, stream_body, 0)
    for cp in rest_copies + ffn_copies:
        cp.start()
    w_copy(O, n_oct - 1).wait()
    for job in out_jobs(n_oct - 1, n_oct - 1):
        job()

    def attend(ops, halves, t0, it, direct, o_dst, o_row, tail, jobs=()):
        nd = direct[0].shape[0]
        dl = [_direct_left(ops, direct[t], direct[2 + t]) for t in range(2)]
        tl = token_left(halves, t0)
        tiles = {i: [_feed(*[x[:, t * LANES:(t + 1) * LANES] for x in tl[i]], dl[t][i]) for t in range(2)]
                 for i in ops}
        lhs = {i: _cols(*tiles[i]) for i in ops}
        qi = lax.broadcasted_iota(jnp.int32, (L, L), 0)
        ki = lax.broadcasted_iota(jnp.int32, (L, L), 1)
        visible = (qi >= seg) | (ki >= seg) | (qi >= ki)
        qkv, e, inv, o_mem = {}, {}, {}, {}

        def first_units(i, t):
            w = _cols(*[w_in(i, K, g, t * LANES // 2, LANES // 2) for g in range(2)])
            return _dot(tiles[i][t], w)

        early = {i: first_units(i, 0) for i in ops}
        early = {i: first_units(i, 1) + early[i] for i in ops}
        clock, due = [0], {}

        def tick():
            clock[0] += 1
            for job in due.pop(clock[0], ()):
                job()

        def later(rounds, job, g):
            due.setdefault(clock[0] + rounds, []).append(functools.partial(job, g))

        for rounds, job, arg in jobs:
            later(rounds, job, arg)

        def project(mat, g):
            prod = {}
            for i in ops:
                if mat == K and g < 2:
                    prod[i] = early[i][:, g * UW:(g + 1) * UW]
                else:
                    prod[i] = _dot(lhs[i], w_in(i, mat, g))
                    tick()
            pair = _direct_out(ops, {i: prod[i][-nd:] for i in ops})
            own = in_tokens(ops, mat, g, {i: split(halves[i], prod[i]) for i in ops}, it)
            if own is not None:
                pair = [_rows(t, d) for t, d in zip(own, pair)]
            for p, x in enumerate(pair):
                x = x if mat == Q else x.astype(BF16)
                for j in range(2):
                    qkv[mat, g, p, j] = x[:, j * Dh:(j + 1) * Dh]

        heads = [(p, j) for p in range(2) for j in range(2)]

        def scores(g):
            for p, j in heads:
                sc = lax.dot_general(qkv[Q, g, p, j], qkv[K, g, p, j], (((1,), (1,)), ((), ())),
                                     preferred_element_type=F32)
                sc = jnp.where(visible, sc * scale, -1e9)
                w = jnp.exp(sc - jnp.max(sc, axis=-1, keepdims=True))
                e[g, p, j] = w
                inv[g, p, j] = pl.reciprocal(jnp.sum(w, axis=-1, keepdims=True), approx=True)
            later(VALUES_AFTER[g], values, g)

        def values(g):
            for p, j in heads:
                o = _dot(e[g, p, j], qkv[V, g, p, j]) * inv[g, p, j]
                o_dst[p, o_row:o_row + seg, (2 * g + j) * Dh:(2 * g + j + 1) * Dh] = o[:seg]
                o_mem[p, 2 * g + j] = o[seg:]

        project(K, 0)
        project(K, 1)
        for g in range(G):
            project(Q, g)
            later(SCORES_AFTER[g], scores, g)
            project(V, g)
            if g + 2 < G:
                project(K, g + 2)
        return tail(o_mem, tick)

    def project_out(ops, with_tokens, direct, tick=lambda: None):
        n_k = hp // 4
        lhs, acc = {}, {}

        def run(n, kk):
            c = slice(kk * 4 * Dh, (kk + 1) * 4 * Dh)
            if kk not in lhs:
                dl = _direct_left(ops, *direct(kk))
                block = lambda r: (o_ref[0, r * R:(r + 1) * R, c], o_ref[1, r * R:(r + 1) * R, c])
                used = "".join(HALVES[ops].values()) if with_tokens else ""
                blocks = {h: block(r) + block(r + 1) for h, r in (("y", 0), ("x", 2)) if h in used}
                lhs[kk] = {i: _rows(dl[i], *[_left(i, *blocks[h]) for h in HALVES[ops][i] if h in used])
                           for i in ops}
            for i in ops:
                w = wk_ref[pl.ds(out_row + (i - 1) * op_rows + kk * 2 * Dh, 2 * Dh), n * LANES:(n + 1) * LANES]
                t = _dot(lhs[kk][i], pltpu.bitcast(w, BF16))
                acc[i, n] = t + acc[i, n] if kk else t
                tick()

        for n, kk in OUT_ORDER:
            run(n, kk)
        prod = {i: _cols(*[acc[i, n] for n in range(HD // LANES)]) for i in ops}
        nd = direct(0)[0].shape[0]
        res = [_direct_out(ops, {i: acc[i, n][:nd] for i in ops}) for n in range(HD // LANES)]
        res = tuple(r[p] for p in range(2) for r in res)
        return res, {i: split(HALVES[ops][i], prod[i][nd:]) for i in ops} if with_tokens else None

    def mem_rows(o_mem):
        return lambda kk: tuple(_cols(*[o_mem[p, 4 * kk + t] for t in range(4)]) for p in range(2))

    def router(n):
        return _rnd(jnp.sum(n * _rows(*[wr_ref[...]] * (n.shape[0] // 8)), axis=-1, keepdims=True))

    def finish(row, a, best, more=True):
        rows = a.shape[0]
        src = pl.ds(pl.multiple_of(jnp.maximum(row, 0), 16), rows)
        rs = pl.ds(pl.multiple_of(jnp.where(row < 0, S, row), 16), rows)
        x1 = _rnd(xr_ref[src, :].astype(F32) + a)
        n1 = _layernorm(x1, True)
        x2 = _rnd(x1 + n1)
        xm_ref[0, rs, :] = x1.astype(BF16)
        xm_ref[1, rs, :] = n1.astype(BF16)
        xr_ref[rs, :] = x2.astype(BF16)
        n_ref[rs, :] = _layernorm(x2) if more else x2
        r = jnp.where(row < 0, -jnp.inf, jnp.broadcast_to(router(n1), (rows, LANES)))
        best_r, best_i = best
        sub = lax.broadcasted_iota(jnp.int32, (8, LANES), 0)
        for b in range(0, rows, 8):
            better = r[b:b + 8] > best_r
            best_r = jnp.where(better, r[b:b + 8], best_r)
            best_i = jnp.where(better, sub + (row + b), best_i)
        return best_r, best_i

    def riders(l, ops):
        return {i: hs[0] if l == 0 else hs for i, hs in HALVES[ops].items()}

    n_early = (n_seg - 7) * seg
    early_copy = pltpu.make_async_copy(xr_ref.at[pl.ds(0, n_early)], out_hbm.at[pl.ds(0, n_early)], sems.at[0])
    late_copy = pltpu.make_async_copy(xr_ref.at[pl.ds(n_early, S - n_early)],
                                      out_hbm.at[pl.ds(n_early, S - n_early)], sems.at[1])

    def period(l, it, carry):
        mem, best = carry
        if l == 1:
            pl.when(it == n_per - 1)(early_copy.start)
        t0 = seg + it * P
        t1 = jnp.where(it == n_per - 1, seg, t0 + P)
        o_ref[:, :seg, :] = onext_ref[...]
        m, best = {}, [best]

        def finish_rows(r):
            best[0] = finish((it - 1) * P + r, a_ref[r:r + P // len(FINISH_STEP[l]), :], best[0], l == 0)

        def normalize_rows(_):
            rs = pl.ds(pl.multiple_of(jnp.where(it < n_per - 2, t0 + 2 * P, seg), seg), 2 * R)
            n_ref[rs, :] = _layernorm(xr_ref[rs, :].astype(F32))

        for u, (ops_in, t, ops_out, dst, row) in enumerate(((SET_B, t0, SET_C, o_ref, seg),
                                                           (SET_C, t0, SET_B, o_ref, 2 * seg),
                                                           (SET_A, t1, SET_A, onext_ref, 0))):
            jobs = [(1, normalize_rows, 0)] if l == 0 and u == REST_STEP else []
            jobs += [(88, finish_rows, b * P // len(FINISH_STEP[l])) for b, v in enumerate(FINISH_STEP[l]) if v == u]
            mem, prods = attend(
                ops_in, riders(l, ops_in), t, it, mem, dst, row,
                lambda o_mem, tick: project_out(ops_out, True, mem_rows(o_mem), tick), jobs)
            for i in ops_out:
                for h, x in prods[i].items():
                    m[i, h] = x
        for t, h in enumerate("yx"):
            top = _cols(m[1, h] + m[4, h] - m[5, h] + m[7, h], m[3, h] + m[5, h])
            bottom = _cols(m[2, h] + m[4, h], m[1, h] - m[2, h] + m[3, h] + m[6, h])
            a_ref[2 * t * R:2 * (t + 1) * R, :] = _rnd(_rows(top, bottom))
        return mem, best[0]

    def arg_max(best):
        best_r, best_i = best
        top = jnp.max(best_r, axis=0, keepdims=True)
        return jnp.min(jnp.where(best_r == top, best_i, S - 1)), top

    def patch_rows(idx):
        return pl.ds(pl.multiple_of(jnp.clip(idx // 16 * 16, 0, S - 16), 16), 16)

    def feed_forward(idx, top):
        rs = patch_rows(idx)
        n1 = xm_ref[1, rs, :]
        gate = _rnd(_dot(n1, wg_ref[...]))
        gate = _rnd(gate * jax.nn.sigmoid(gate))
        up = _rnd(_dot(n1, wu_ref[...]))
        y = _rnd(_dot((gate * up).astype(BF16), wd_ref[...]))
        y = _rnd(y * _cols(*[_rnd(jax.nn.sigmoid(top))] * (D // LANES)))
        chosen = lax.broadcasted_iota(jnp.int32, (16, D), 0) == idx - rs.start
        update = _rnd(n1.astype(F32) + jnp.where(chosen, y, 0.0))
        patch_ref[...] = (xm_ref[0, rs, :].astype(F32) + update).astype(BF16)

    def layer(l, routed):
        @pl.when((routed >= seg) & (routed < seg + 2 * R))
        def _():
            pl.loop(0, G)(first_products)

        mem = attend(SET_A, {i: hs[1:] for i, hs in HALVES[SET_A].items()}, seg, None,
                     jnp.split(_rows(n_ref[:seg, :], mem0_ref[...].astype(F32)), D // LANES, axis=1), onext_ref, 0,
                     lambda o_mem, tick: project_out(SET_C, False, mem_rows(o_mem), tick)[0])

        @pl.when(l == 0)
        def _():
            for cp in rest_copies:
                cp.wait()

        best = (jnp.full((8, LANES), -jnp.inf, F32), lax.broadcasted_iota(jnp.int32, (8, LANES), 0))
        carry = lax.fori_loop(0, (1 - l) * n_per, functools.partial(period, 0), (mem, best))
        _, best = lax.fori_loop(0, l * n_per, functools.partial(period, 1), carry)

        @pl.when(l == 0)
        def _():
            for cp in ffn_copies:
                cp.wait()

        last, _ = project_out(SET_C, False, lambda kk: tuple(
            onext_ref[p, :, kk * 4 * Dh:(kk + 1) * 4 * Dh] for p in range(2)))
        best = finish(S - seg - P, a_ref[...], best)
        leader = arg_max(best)
        feed_forward(*leader)
        winner = arg_max(finish(S - seg, _rnd(_cols(*last)), best))
        pl.when(l == 1)(late_copy.start)
        pl.when(winner[0] != leader[0])(lambda: feed_forward(*winner))

        @pl.when(l == 0)
        def _():
            xr_ref[patch_rows(winner[0]), :] = patch_ref[...]
            n_ref[patch_rows(winner[0]), :] = _layernorm(patch_ref[...].astype(F32))

        return winner[0]

    routed = lax.fori_loop(0, 2, layer, jnp.int32(0))
    early_copy.wait()
    late_copy.wait()
    patch_copy = pltpu.make_async_copy(patch_ref, out_hbm.at[patch_rows(routed)], sems.at[0])
    patch_copy.start()
    patch_copy.wait()


@functools.partial(jax.jit, static_argnames=("A_seg_len",))
def pallas_interleave_layers__memory_aug_recurrent_mem_tr__moe_arch_mod__prompt_kernel(
    A_x, A_mem0, A_Wq, A_Wk, A_Wv, A_Wo, A_seg_len, B_x, B_w_r, B_w_gate, B_w_up, B_w_down,
):
    del B_x
    B, S, D = A_x.shape
    _, H, Dh = A_Wq.shape
    M = A_mem0.shape[1]
    F = B_w_gate.shape[1]
    seg = int(A_seg_len)
    assert B == 1 and Dh == LANES and D == 4 * LANES and H % 8 == 0 and M % 8 == 0
    assert seg % 32 == 0 and S % seg == 0 and (S // seg) % 9 == 1 and S // seg > 7
    half = H * Dh // 2
    R = 3 * seg // 4
    hbm = pl.BlockSpec(memory_space=pl.ANY)

    def octets(w):
        return w.reshape(D, H // 8, 8, Dh).transpose(0, 2, 1, 3).reshape(8 * D, H // 8 * Dh)

    out = pl.pallas_call(
        functools.partial(_kernel, seg=seg, n_heads=H),
        out_shape=jax.ShapeDtypeStruct((S, D), A_x.dtype),
        in_specs=[hbm] * 10,
        out_specs=hbm,
        scratch_shapes=[
            pltpu.VMEM((3, H // 8, 8 * D, Dh), BF16),
            pltpu.VMEM((4 * D + 32, Dh), U32),
            pltpu.VMEM((H // 8 + 1, 8 * Dh, D), BF16),
            *[pltpu.VMEM((n * 7 * half // 2 + H // 2 * (S - seg) // 4, UW), U32) for n in (2, 1, 1)],
            pltpu.VMEM((D, F), BF16),
            pltpu.VMEM((D, F), BF16),
            pltpu.VMEM((F, D), BF16),
            pltpu.VMEM((S + 3 * seg, D), BF16),
            pltpu.VMEM((2, S + 3 * seg, D), BF16),
            pltpu.VMEM((S + 3 * seg, D), F32),
            pltpu.VMEM((2, (S - seg) // 4, D // 2), F32),
            pltpu.VMEM((4, 3, H // 4, R, UW), F32),
            pltpu.VMEM((2, 3, H // 4, R, UW), F32),
            pltpu.VMEM((2, 3, H // 4, seg, UW), F32),
            pltpu.VMEM((2, 3 * seg, half), F32),
            pltpu.VMEM((2, seg, half), F32),
            pltpu.VMEM((3 * seg, D), F32),
            pltpu.VMEM((16, D), BF16),
            pltpu.VMEM((M, D), BF16),
            pltpu.VMEM((D,), BF16),
            pltpu.VMEM((8, D), F32),
            pltpu.SemaphoreType.DMA((9 + H // 2,)),
        ],
        compiler_params=pltpu.CompilerParams(vmem_limit_bytes=110 * 1024 * 1024),
        name="rmt_mod",
    )(A_x.reshape(S, D), A_mem0.reshape(M, D), octets(A_Wq), octets(A_Wk),
      octets(A_Wv), A_Wo.reshape(H * Dh, D), B_w_r, B_w_gate, B_w_up, B_w_down)
    return out.reshape(B, S, D)
```

```python
import functools

import jax
import jax.numpy as jnp
from jax import lax
import jax.experimental.pallas as pl
import jax.experimental.pallas.tpu as pltpu

F32 = jnp.float32
BF16 = jnp.bfloat16
U32 = jnp.uint32
LANES = 128
UNIT = 2 * LANES
EPS = 1e-5
EPS_BF16 = 1.0013580322265625e-05
K, Q, V, O = 0, 1, 2, 3

SCORES_AFTER = (7, 7, 7, 7, 7, 7, 7, 11)
VALUES_AFTER = 8
FINISH_AFTER = 88
FINISH_STEP = ((0, 1, 2), (0, 0, 1, 1, 2, 2))


def _rnd(x):
    return x.astype(BF16).astype(F32)


def _layernorm(x, stepwise=False):
    inv_d = 1.0 / x.shape[-1]
    m = jnp.sum(x, axis=-1, keepdims=True) * inv_d
    c = x - m
    v = jnp.sum(c * c, axis=-1, keepdims=True) * inv_d
    if not stepwise:
        return c * lax.rsqrt(v + EPS)
    sd = _rnd(jnp.sqrt(_rnd(_rnd(v) + EPS_BF16)))
    return _rnd(_rnd(x - _rnd(m)) / sd)


def _ds(start, size, align):
    return pl.ds(start if isinstance(start, int) else pl.multiple_of(start, align), size)


def _dot(a, b):
    return jnp.dot(a, b, preferred_element_type=F32)


def _rows(*xs):
    return xs[0] if len(xs) == 1 else jnp.concatenate(xs, axis=0)


def _cols(*xs):
    return jnp.concatenate(xs, axis=1)


def _feed(*xs):
    x = _rows(*xs)
    return x if x.shape[0] % 16 else x.astype(BF16)


def _right(b11, b12, b21, b22):
    return {1: b11 + b22, 2: b11, 3: b12 - b22, 4: b21 - b11, 5: b22, 6: b11 + b12, 7: b21 + b22}


def _left(i, a11, a12, a21, a22):
    return {1: lambda: a11 + a22, 2: lambda: a21 + a22, 3: lambda: a11, 4: lambda: a22,
            5: lambda: a11 + a12, 6: lambda: a21 - a11, 7: lambda: a12 - a22}[i]()


SET_A, SET_B, SET_C = (1, 3, 5, 7), (1, 2, 4, 6), (2, 3, 4, 5)


def _direct_left(ops, a1, a2):
    both = a1 + a2
    return {1: a1 if ops == SET_A else a2, 2: both, 3: a1, 4: a2, 5: both, 6: a1, 7: a2}


def _direct_out(ops, p):
    c1 = p[1] - p[5] + p[7] if ops == SET_A else p[2] + p[4]
    c2 = p[1] - p[2] + p[6] if ops == SET_B else p[3] + p[5]
    return c1, c2


HALVES = {SET_A: {1: "x", 3: "x", 5: "x", 7: "xy"},
          SET_B: {1: "y", 2: "x", 4: "x", 6: "xy"},
          SET_C: {2: "y", 3: "y", 4: "y", 5: "y"}}


def _kernel(x_hbm, mem0_hbm, wq_hbm, wk_hbm, wv_hbm, wo_hbm, wr_hbm, wg_hbm, wu_hbm, wd_hbm,
            out_hbm,
            raw_ref, words_ref, rawo_ref, wk_ref, wq_ref, wv_ref, wg_ref, wu_ref, wd_ref,
            xr_ref, xm_ref, n_ref, ly_ref, px_ref, py_ref, left_ref, o_ref, onext_ref, a_ref,
            patch_ref, mem0_ref, wr1_ref, wr_ref, sems,
            *, seg, n_heads):
    S, D = x_hbm.shape
    Dh = LANES
    L = mem0_ref.shape[0] + seg
    HD = D // 2
    P = 3 * seg
    R = P // 4
    n_per = (S - seg) // P
    n_unit = n_heads // 4
    n_oct = n_heads // 8
    scale = Dh ** -0.5

    w_ref = {K: wk_ref, Q: wq_ref, V: wv_ref}
    op_rows = n_unit * HD // 2
    out_row = 7 * op_rows + 2 * n_unit * n_per * R

    def w_in(i, mat, g, r=0, rows=HD // 2):
        return pltpu.bitcast(w_ref[mat][_ds((i - 1) * op_rows + g * (HD // 2) + r, rows, 8), :], BF16)

    def ahead(mat, k, g, r):
        return w_ref[(mat + 1) % 3], _ds(7 * op_rows + (k * n_unit + g) * n_per * R + r, R, 8)

    def w_copy(mat, c):
        sem = sems.at[9 + 4 * c + mat]
        if mat == O:
            return pltpu.make_async_copy(wo_hbm.at[pl.ds(c * 8 * Dh, 8 * Dh)], rawo_ref.at[c], sem)
        src = {K: wk_hbm, Q: wq_hbm, V: wv_hbm}[mat]
        return pltpu.make_async_copy(src.at[:, _ds(c * Dh, Dh, Dh)], raw_ref.at[mat, c], sem)

    def arriving(mat, c):
        return [(mat, c)] if mat < O else [(K, c + 1), (O, c - 1)]

    def x_copy(row, rows, sem):
        rs = _ds(row, rows, 16)
        return pltpu.make_async_copy(x_hbm.at[rs], xr_ref.at[rs], sems.at[sem])

    def y_copy(j, group):
        return x_copy(seg + j * P + 2 * R, 2 * R, 6 + group)

    n_ln = n_per // 3
    rest_copies = [x_copy(seg + j * P, 2 * R, 0) for j in range(2, n_per)]
    ffn_copies = [pltpu.make_async_copy(src, dst, sems.at[1 + i])
                  for i, (src, dst) in enumerate(((wg_hbm, wg_ref), (wu_hbm, wu_ref), (wd_hbm, wd_ref)))]
    first_copies = [x_copy(0, seg + 2 * R, 0), x_copy(seg + P, 2 * R, 1),
                    pltpu.make_async_copy(mem0_hbm, mem0_ref, sems.at[4]),
                    pltpu.make_async_copy(wr_hbm, wr1_ref, sems.at[5])]
    for cp in first_copies:
        cp.start()
    for j in range(n_per):
        y_copy(j, j // n_ln).start()
    w_copy(K, 0).start()
    for c in range(2):
        for mat in (Q, V, O):
            for chunk in arriving(mat, c):
                if chunk[1] >= 0:
                    w_copy(*chunk).start()

    a_ref[...] = jnp.zeros_like(a_ref)
    rawo_ref[n_oct] = jnp.zeros(rawo_ref.shape[1:], BF16)
    for cp in first_copies:
        cp.wait()
    wr_ref[...] = jnp.broadcast_to(wr1_ref[...].astype(F32).reshape(1, D), wr_ref.shape)
    for rs in (pl.ds(0, seg + 2 * R), pl.ds(seg + P, 2 * R)):
        n_ref[rs, :] = _layernorm(xr_ref[rs, :].astype(F32))

    def normalize_group(group, carry):
        periods = [group * n_ln + u for u in range(n_ln)]
        for j in periods:
            y_copy(j, group).wait()
        for j in periods:
            rs = _ds(seg + j * P + 2 * R, 2 * R, 16)
            n = _layernorm(xr_ref[rs, :].astype(F32))
            n_ref[rs, :] = n
            for k in range(2):
                ly_ref[k, _ds(j * R, R, 8), :] = _left(6 + k, n[:R, :HD], n[:R, HD:], n[R:, :HD], n[R:, HD:])
        return carry

    lax.fori_loop(0, 3, normalize_group, 0)

    def pack(x):
        return pltpu.bitcast(x.astype(BF16), U32)

    def prep_in(mat, c, t):
        b, j = divmod(t, 4)
        dst = (2 * c + j // 2) * (HD // 2) + b * 8
        ds = [half * HD + b * 16 for half in range(2)]
        if j == 0:
            for d in ds:
                words_ref[pl.ds(4 * d, 64), :] = pltpu.bitcast(raw_ref[mat, c, pl.ds(8 * d, 128), :], U32)
        w1, w2 = (words_ref[pl.ds(4 * d + j, 16, stride=4), :] for d in ds)
        blocks = [pltpu.bitcast(w, F32) for w in (w1 << 16, w1 & U32(0xFFFF0000), w2 << 16, w2 & U32(0xFFFF0000))]
        for i, w in _right(*blocks).items():
            w_ref[mat][_ds((i - 1) * op_rows + dst, 8, 8), pl.ds(j % 2 * Dh, Dh)] = pack(w)

    def prep_out(src, c, t):
        j, r = divmod(t * 16, Dh)
        even, odd = (rawo_ref[src, pl.ds(j * UNIT + p * Dh + r, 16), :].astype(F32) for p in range(2))
        dst = c * 2 * Dh + t * 8
        for i, w in _right(even[:, :HD], even[:, HD:], odd[:, :HD], odd[:, HD:]).items():
            wk_ref[_ds(out_row + (i - 1) * op_rows + dst, 8, 8), :] = pack(w)

    def in_jobs(mat, c):
        return [functools.partial(prep_in, mat, c, t) for t in range(HD // 4)]

    def out_jobs(src, c):
        return [functools.partial(prep_out, src, c, t) for t in range(Dh // 4)]

    def token_left(halves, t0):
        def block(r):
            t = n_ref[_ds(t0 + r * R, R, 8), :]
            return t[:, :HD], t[:, HD:]

        used = "".join(halves.values())
        blocks = {h: block(r) + block(r + 1) for h, r in (("x", 0), ("y", 2)) if h in used}
        return {i: [_left(i, *blocks[h]) for h in hs] for i, hs in halves.items()}

    def split(hs, prod):
        return {h: prod[t * R:(t + 1) * R] for t, h in enumerate(hs)}

    def in_tokens(ops, mat, g, m, it):
        if ops == SET_A:
            if "x" in m[7]:
                px_ref[0, mat, g] = m[1]["x"] - m[5]["x"] + m[7]["x"]
                px_ref[1, mat, g] = m[3]["x"] + m[5]["x"]
                px_ref[2, mat, g] = m[1]["x"] + m[3]["x"]
            if "y" in m[7]:
                px_ref[3, mat, g] = m[7]["y"]
            return None if it is None else (left_ref[0, mat, g], left_ref[1, mat, g])
        if ops == SET_B:
            even = _rows(px_ref[0, mat, g] + m[4]["x"], m[2]["x"] + m[4]["x"])
            odd = _rows(px_ref[1, mat, g], px_ref[2, mat, g] - m[2]["x"] + m[6]["x"])
            if "y" in m[6]:
                m6, m7 = m[6]["y"], px_ref[3, mat, g]
            else:
                m6, m7 = (pltpu.bitcast(ref[rs, :], F32) for ref, rs in (ahead(mat, k, g, it * R) for k in range(2)))
            py_ref[0, mat, g] = m7 + m[1]["y"]
            py_ref[1, mat, g] = m[1]["y"] + m6
            left_ref[0, mat, g, :2 * R - seg] = even[seg:]
            left_ref[1, mat, g, :2 * R - seg] = odd[seg:]
            return even[:seg], odd[:seg]
        even = _rows(left_ref[0, mat, g, :2 * R - seg],
                     py_ref[0, mat, g] + m[4]["y"] - m[5]["y"], m[2]["y"] + m[4]["y"])
        odd = _rows(left_ref[1, mat, g, :2 * R - seg],
                    m[3]["y"] + m[5]["y"], py_ref[1, mat, g] - m[2]["y"] + m[3]["y"])
        left_ref[0, mat, g] = even[seg:]
        left_ref[1, mat, g] = odd[seg:]
        return even[:seg], odd[:seg]

    def first_products(g):
        tl = token_left({i: "x" for i in SET_A}, seg)
        for mat in (K, Q, V):
            in_tokens(SET_A, mat, g, {i: {"x": _dot(tl[i][0], w_in(i, mat, g))} for i in SET_A}, None)

    def for_chunks(mat, c, action):
        for m, i in arriving(mat, c):
            pl.when((i >= 0) & (i < n_oct))(lambda m=m, i=i: action(w_copy(m, jnp.clip(i, 0, n_oct - 1))))

    def stream(mat, c):
        for_chunks(mat, c, lambda cp: cp.wait())
        if mat < O:
            jobs = in_jobs(mat, c)
        else:
            first_products(2 * c)
            first_products(2 * c + 1)
            jobs = (in_jobs(K, jnp.minimum(c + 1, n_oct - 1))
                    + out_jobs(jnp.where(c == 0, n_oct, c - 1), jnp.maximum(c - 1, 0)))
        for k in range(2):
            for u in range(2):
                prod = pltpu.bitcast(_dot(ly_ref[k], w_in(6 + k, mat - 1, 2 * c + u)), U32)
                for j in range(n_per):
                    i = (2 * k + u) * n_per + j
                    for job in jobs[i * len(jobs) // (4 * n_per):(i + 1) * len(jobs) // (4 * n_per)]:
                        job()
                    ref, rs = ahead(mat - 1, k, 2 * c + u, j * R)
                    ref[rs, :] = prod[j * R:(j + 1) * R]
        for_chunks(mat, c + 2, lambda cp: cp.start())

    def stream_round(i, carry):
        for mat in (Q, V, O):
            pl.when(i % 3 == mat - 1)(functools.partial(stream, mat, i // 3))
        return carry

    w_copy(K, 0).wait()
    for job in in_jobs(K, 0):
        job()
    lax.fori_loop(0, 3 * n_oct, stream_round, 0)
    for cp in rest_copies + ffn_copies:
        cp.start()
    w_copy(O, n_oct - 1).wait()
    for job in out_jobs(n_oct - 1, n_oct - 1):
        job()

    def project_out(ops, with_tokens, direct, tick=lambda: None):
        acc = {}
        used = "".join(HALVES[ops].values()) if with_tokens else ""
        for c in range(n_oct):
            cs = slice(c * 4 * Dh, (c + 1) * 4 * Dh)
            dl = _direct_left(ops, *(_cols(*[direct(p, 4 * c + t) for t in range(4)]) for p in range(2)))
            blocks = {h: [o_ref[p, b * R:(b + 1) * R, cs] for b in (r, r + 1) for p in range(2)]
                      for h, r in (("y", 0), ("x", 2)) if h in used}
            lhs = {i: _rows(dl[i], *[_left(i, *blocks[h]) for h in HALVES[ops][i] if h in used]) for i in ops}
            for n in range(2):
                for i in ops:
                    w = wk_ref[pl.ds(out_row + (i - 1) * op_rows + c * 2 * Dh, 2 * Dh), n * LANES:(n + 1) * LANES]
                    t = _dot(lhs[i], pltpu.bitcast(w, BF16))
                    acc[i, n] = t + acc[i, n] if c else t
                    tick()
        nd = dl[2].shape[0]
        res = [_direct_out(ops, {i: acc[i, n][:nd] for i in ops}) for n in range(2)]
        prods = {i: split(HALVES[ops][i], _cols(acc[i, 0], acc[i, 1])[nd:]) for i in ops if with_tokens}
        return tuple(r[p] for p in range(2) for r in res), prods

    def attend(ops, halves, t0, it, direct, o_dst, o_row, ops_out, jobs=()):
        nd = direct[0].shape[0]
        dl = [_direct_left(ops, direct[t], direct[2 + t]) for t in range(2)]
        tl = token_left(halves, t0)
        tiles = {i: [_feed(*[x[:, t * LANES:(t + 1) * LANES] for x in tl[i]], dl[t][i]) for t in range(2)]
                 for i in ops}
        lhs = {i: _cols(*tiles[i]) for i in ops}
        qi = lax.broadcasted_iota(jnp.int32, (L, L), 0)
        ki = lax.broadcasted_iota(jnp.int32, (L, L), 1)
        visible = (qi >= seg) | (ki >= seg) | (qi >= ki)
        heads = [(p, j) for p in range(2) for j in range(2)]
        qkv, e, inv, o_mem = {}, {}, {}, {}
        clock, due = [0], {}

        def tick():
            clock[0] += 1
            for job in due.pop(clock[0], ()):
                job()

        def later(rounds, job, *args):
            due.setdefault(clock[0] + rounds, []).append(functools.partial(job, *args))

        for job in jobs:
            later(*job)

        def first_units(i, t):
            return _dot(tiles[i][t], _cols(*[w_in(i, K, g, t * LANES // 2, LANES // 2) for g in range(2)]))

        early = {i: first_units(i, 0) for i in ops}
        early = {i: first_units(i, 1) + early[i] for i in ops}

        def project(mat, g):
            prod = {}
            for i in ops:
                if mat == K and g < 2:
                    prod[i] = early[i][:, g * UNIT:(g + 1) * UNIT]
                else:
                    prod[i] = _dot(lhs[i], w_in(i, mat, g))
                    tick()
            pair = _direct_out(ops, {i: prod[i][-nd:] for i in ops})
            own = in_tokens(ops, mat, g, {i: split(halves[i], prod[i]) for i in ops}, it)
            if own is not None:
                pair = [_rows(t, d) for t, d in zip(own, pair)]
            for p, x in enumerate(pair):
                x = x if mat == Q else x.astype(BF16)
                for j in range(2):
                    qkv[mat, g, p, j] = x[:, j * Dh:(j + 1) * Dh]

        def scores(g):
            for p, j in heads:
                sc = lax.dot_general(qkv[Q, g, p, j], qkv[K, g, p, j], (((1,), (1,)), ((), ())),
                                     preferred_element_type=F32)
                sc = jnp.where(visible, sc * scale, -1e9)
                e[g, p, j] = jnp.exp(sc - jnp.max(sc, axis=-1, keepdims=True))
                inv[g, p, j] = pl.reciprocal(jnp.sum(e[g, p, j], axis=-1, keepdims=True), approx=True)
            later(VALUES_AFTER, values, g)

        def values(g):
            for p, j in heads:
                o = _dot(e[g, p, j], qkv[V, g, p, j]) * inv[g, p, j]
                o_dst[p, o_row:o_row + seg, (2 * g + j) * Dh:(2 * g + j + 1) * Dh] = o[:seg]
                o_mem[p, 2 * g + j] = o[seg:]

        project(K, 0)
        project(K, 1)
        for g in range(n_unit):
            project(Q, g)
            later(SCORES_AFTER[g], scores, g)
            project(V, g)
            if g + 2 < n_unit:
                project(K, g + 2)
        res = project_out(ops_out, it is not None, lambda p, j: o_mem[p, j], tick)
        assert not due
        return res

    def finish(row, a, best, more=True):
        rows = a.shape[0]
        rs = _ds(jnp.where(row < 0, S, row), rows, 16)
        x1 = _rnd(xr_ref[_ds(jnp.maximum(row, 0), rows, 16), :].astype(F32) + a)
        n1 = _layernorm(x1, True)
        x2 = _rnd(x1 + n1)
        xm_ref[0, rs, :] = x1.astype(BF16)
        xm_ref[1, rs, :] = n1.astype(BF16)
        xr_ref[rs, :] = x2.astype(BF16)
        n_ref[rs, :] = _layernorm(x2) if more else x2
        r = _rnd(jnp.sum(n1 * _rows(*[wr_ref[...]] * (rows // 8)), axis=-1, keepdims=True))
        r = jnp.where(row < 0, -jnp.inf, jnp.broadcast_to(r, (rows, LANES)))
        best_r, best_i = best
        sub = lax.broadcasted_iota(jnp.int32, (8, LANES), 0)
        for b in range(0, rows, 8):
            better = r[b:b + 8] > best_r
            best_r = jnp.where(better, r[b:b + 8], best_r)
            best_i = jnp.where(better, sub + (row + b), best_i)
        return best_r, best_i

    n_early = S - seg - 2 * P
    early_copy, late_copy = (pltpu.make_async_copy(xr_ref.at[rs], out_hbm.at[rs], sems.at[i])
                             for i, rs in enumerate((pl.ds(0, n_early), pl.ds(n_early, S - n_early))))

    def period(l, it, carry):
        mem, best = carry
        if l == 1:
            pl.when(it == n_per - 1)(early_copy.start)
        t0 = seg + it * P
        t1 = jnp.where(it == n_per - 1, seg, t0 + P)
        o_ref[:, :seg, :] = onext_ref[...]
        m, best = {}, [best]
        piece = P // len(FINISH_STEP[l])

        def finish_rows(r):
            best[0] = finish((it - 1) * P + r, a_ref[r:r + piece, :], best[0], l == 0)

        def normalize_rest():
            rs = _ds(jnp.where(it < n_per - 2, t0 + 2 * P, seg), 2 * R, seg)
            n_ref[rs, :] = _layernorm(xr_ref[rs, :].astype(F32))

        for u, (ops_in, t, ops_out, dst, row) in enumerate(((SET_B, t0, SET_C, o_ref, seg),
                                                           (SET_C, t0, SET_B, o_ref, 2 * seg),
                                                           (SET_A, t1, SET_A, onext_ref, 0))):
            jobs = [(1, normalize_rest)] if l == 0 and u == 2 else []
            jobs += [(FINISH_AFTER, finish_rows, b * piece) for b, v in enumerate(FINISH_STEP[l]) if v == u]
            halves = {i: hs if l else hs[0] for i, hs in HALVES[ops_in].items()}
            mem, prods = attend(ops_in, halves, t, it, mem, dst, row, ops_out, jobs)
            for i in ops_out:
                for h, x in prods[i].items():
                    m[i, h] = x
        for t, h in enumerate("yx"):
            top = _cols(m[1, h] + m[4, h] - m[5, h] + m[7, h], m[3, h] + m[5, h])
            bottom = _cols(m[2, h] + m[4, h], m[1, h] - m[2, h] + m[3, h] + m[6, h])
            a_ref[2 * t * R:2 * (t + 1) * R, :] = _rnd(_rows(top, bottom))
        return mem, best[0]

    def arg_max(best):
        best_r, best_i = best
        top = jnp.max(best_r, axis=0, keepdims=True)
        return jnp.min(jnp.where(best_r == top, best_i, S - 1)), top

    def patch_rows(idx):
        return _ds(jnp.clip(idx // 16 * 16, 0, S - 16), 16, 16)

    def feed_forward(idx, top):
        rs = patch_rows(idx)
        n1 = xm_ref[1, rs, :]
        gate = _rnd(_dot(n1, wg_ref[...]))
        gate = _rnd(gate * jax.nn.sigmoid(gate))
        up = _rnd(_dot(n1, wu_ref[...]))
        y = _rnd(_dot((gate * up).astype(BF16), wd_ref[...]))
        y = _rnd(y * _cols(*[_rnd(jax.nn.sigmoid(top))] * (D // LANES)))
        chosen = lax.broadcasted_iota(jnp.int32, (16, D), 0) == idx - rs.start
        update = _rnd(n1.astype(F32) + jnp.where(chosen, y, 0.0))
        patch_ref[...] = (xm_ref[0, rs, :].astype(F32) + update).astype(BF16)

    def layer(l, routed):
        @pl.when((routed >= seg) & (routed < seg + 2 * R))
        def _():
            pl.loop(0, n_unit)(first_products)

        first = jnp.split(_rows(n_ref[:seg, :], mem0_ref[...].astype(F32)), D // LANES, axis=1)
        mem, _ = attend(SET_A, {i: hs[1:] for i, hs in HALVES[SET_A].items()}, seg, None, first,
                        onext_ref, 0, SET_C)

        @pl.when(l == 0)
        def _():
            for cp in rest_copies:
                cp.wait()

        best = (jnp.full((8, LANES), -jnp.inf, F32), lax.broadcasted_iota(jnp.int32, (8, LANES), 0))
        carry = lax.fori_loop(0, (1 - l) * n_per, functools.partial(period, 0), (mem, best))
        _, best = lax.fori_loop(0, l * n_per, functools.partial(period, 1), carry)

        @pl.when(l == 0)
        def _():
            for cp in ffn_copies:
                cp.wait()

        last, _ = project_out(SET_C, False, lambda p, j: onext_ref[p, :, j * Dh:(j + 1) * Dh])
        best = finish(S - seg - P, a_ref[...], best)
        leader = arg_max(best)
        feed_forward(*leader)
        winner = arg_max(finish(S - seg, _rnd(_cols(*last)), best))
        pl.when(l == 1)(late_copy.start)
        pl.when(winner[0] != leader[0])(lambda: feed_forward(*winner))

        @pl.when(l == 0)
        def _():
            xr_ref[patch_rows(winner[0]), :] = patch_ref[...]
            n_ref[patch_rows(winner[0]), :] = _layernorm(patch_ref[...].astype(F32))

        return winner[0]

    routed = lax.fori_loop(0, 2, layer, jnp.int32(0))
    early_copy.wait()
    late_copy.wait()
    patch_copy = pltpu.make_async_copy(patch_ref, out_hbm.at[patch_rows(routed)], sems.at[0])
    patch_copy.start()
    patch_copy.wait()


@functools.partial(jax.jit, static_argnames=("A_seg_len",))
def pallas_interleave_layers__memory_aug_recurrent_mem_tr__moe_arch_mod__prompt_kernel(
    A_x, A_mem0, A_Wq, A_Wk, A_Wv, A_Wo, A_seg_len, B_x, B_w_r, B_w_gate, B_w_up, B_w_down,
):
    del B_x
    B, S, D = A_x.shape
    _, H, Dh = A_Wq.shape
    M = A_mem0.shape[1]
    F = B_w_gate.shape[1]
    seg = int(A_seg_len)
    assert B == 1 and Dh == LANES and D == 4 * LANES and H == 4 * len(SCORES_AFTER) and M % 8 == 0
    assert seg % 32 == 0 and S % seg == 0 and (S // seg) % 9 == 1 and S // seg > 10
    half = H * Dh // 2
    R = 3 * seg // 4

    def octets(w):
        return w.reshape(D, H // 8, 8, Dh).transpose(0, 2, 1, 3).reshape(8 * D, H // 8 * Dh)

    out = pl.pallas_call(
        functools.partial(_kernel, seg=seg, n_heads=H),
        out_shape=jax.ShapeDtypeStruct((S, D), A_x.dtype),
        in_specs=[pl.BlockSpec(memory_space=pl.ANY)] * 10,
        out_specs=pl.BlockSpec(memory_space=pl.ANY),
        scratch_shapes=[
            pltpu.VMEM((3, H // 8, 8 * D, Dh), BF16),
            pltpu.VMEM((4 * D + 32, Dh), U32),
            pltpu.VMEM((H // 8 + 1, 8 * Dh, D), BF16),
            *[pltpu.VMEM((n * 7 * half // 2 + H // 2 * (S - seg) // 4, UNIT), U32) for n in (2, 1, 1)],
            pltpu.VMEM((D, F), BF16),
            pltpu.VMEM((D, F), BF16),
            pltpu.VMEM((F, D), BF16),
            pltpu.VMEM((S + 3 * seg, D), BF16),
            pltpu.VMEM((2, S + 3 * seg, D), BF16),
            pltpu.VMEM((S + 3 * seg, D), F32),
            pltpu.VMEM((2, (S - seg) // 4, D // 2), F32),
            pltpu.VMEM((4, 3, H // 4, R, UNIT), F32),
            pltpu.VMEM((2, 3, H // 4, R, UNIT), F32),
            pltpu.VMEM((2, 3, H // 4, seg, UNIT), F32),
            pltpu.VMEM((2, 3 * seg, half), F32),
            pltpu.VMEM((2, seg, half), F32),
            pltpu.VMEM((3 * seg, D), F32),
            pltpu.VMEM((16, D), BF16),
            pltpu.VMEM((M, D), BF16),
            pltpu.VMEM((D,), BF16),
            pltpu.VMEM((8, D), F32),
            pltpu.SemaphoreType.DMA((9 + H // 2,)),
        ],
        compiler_params=pltpu.CompilerParams(vmem_limit_bytes=110 * 1024 * 1024),
        name="rmt_mod",
    )(A_x.reshape(S, D), A_mem0.reshape(M, D), octets(A_Wq), octets(A_Wk), octets(A_Wv),
      A_Wo.reshape(H * Dh, D), B_w_r, B_w_gate, B_w_up, B_w_down)
    return out.reshape(B, S, D)
```
